```python
import jax
import jax.numpy as jnp

def _softmax(x, axis=-1):
    return jax.nn.softmax(x, axis=axis)
def _gelu(x):
    return jax.nn.gelu(x, approximate=True)
def _silu(x):
    return jax.nn.silu(x)
def _sigmoid(x):
    return jax.nn.sigmoid(x)
def _layernorm(x, axis=-1, eps=1e-5):
    m = jnp.mean(x, axis=axis, keepdims=True)
    v = jnp.var(x, axis=axis, keepdims=True)
    return (x - m) / jnp.sqrt(v + eps)
def _scatter_add(tgt, idx, src, axis=0):
    return tgt.at[idx].add(src)
def _segment_sum(src, seg, n):
    return jax.ops.segment_sum(src, seg, n)
class _Rng:
    def __init__(self, key):
        self._k = key
    def _next(self):
        self._k, sub = jax.random.split(self._k)
        return sub
    def normal(self, shape):
        return jax.random.normal(self._next(), shape, dtype=jnp.bfloat16)
    def randint(self, lo, hi, shape):
        return jax.random.randint(self._next(), shape, lo, hi, dtype=jnp.int32)
    def uniform(self, shape, lo=0.0, hi=1.0):
        return jax.random.uniform(self._next(), shape, jnp.bfloat16, lo, hi)
    def permutation(self, n):
        return jax.random.permutation(self._next(), n)


kernel_name = 'concat_heads__compressed_kv_cla__sliding_local_dilated__prompt'

def setup_inputs():
    _rng = _Rng(jax.random.key(int.from_bytes(__import__("os").urandom(4), "little")))
    _w = (lambda a: (lambda t: t.astype(jnp.bfloat16) if jnp.issubdtype(t.dtype, jnp.floating) else t)(jnp.asarray(a)))
    def _A_setup():
        B, H, Sq, Sk, D, M = 1, 32, 2048, 2048, 128, 1024
        Dc = 4 * D
        return {
            "x": _w((lambda *s: _rng.normal(s) * 0.05)(B, Sq, M)),
            "c_kv": _w((lambda *s: _rng.normal(s) * 0.05)(B, Sk, Dc)),
            "w_q": _w((lambda *s: _rng.normal(s) * 0.05)(M, H, D) * (M ** -0.5)),
            "w_uk": _w((lambda *s: _rng.normal(s) * 0.05)(Dc, H, D) * (Dc ** -0.5)),
            "w_uv": _w((lambda *s: _rng.normal(s) * 0.05)(Dc, H, D) * (Dc ** -0.5)),
            "w_o": _w((lambda *s: _rng.normal(s) * 0.05)(H, D, M) * ((H * D) ** -0.5)),
        }
    _A_in = _A_setup()

    def _B_setup():
        B, S, D = 1, 2048, 1024
        return {
            "x": _w((lambda *s: _rng.normal(s) * 0.05)(B, S, D)),
            "wqkv": _w((lambda *s: _rng.normal(s) * 0.05)(D, 3 * D)),
            "wo": _w((lambda *s: _rng.normal(s) * 0.05)(D, D)),
        }
    _B_in = _B_setup()

    return {
        "A_x": _A_in["x"],
        "A_c_kv": _A_in["c_kv"],
        "A_w_q": _A_in["w_q"],
        "A_w_uk": _A_in["w_uk"],
        "A_w_uv": _A_in["w_uv"],
        "A_w_o": _A_in["w_o"],
        "B_x": _B_in["x"],
        "B_wqkv": _B_in["wqkv"],
        "B_wo": _B_in["wo"],
    }

def reference(A_x, A_c_kv, A_w_q, A_w_uk, A_w_uv, A_w_o, B_x, B_wqkv, B_wo):
    def _A_ref(x, c_kv, w_q, w_uk, w_uv, w_o):
        B, Sq, M = x.shape[0], x.shape[1], x.shape[2]
        Sk = c_kv.shape[1]
        H, D = w_q.shape[1], w_q.shape[2]
        q = jnp.einsum("bqm,mhd->bhqd", x, w_q)
        k = jnp.einsum("bkc,chd->bhkd", c_kv, w_uk)
        v = jnp.einsum("bkc,chd->bhkd", c_kv, w_uv)
        scores = jnp.einsum("bhqd,bhkd->bhqk", q, k) * (D ** -0.5)
        off = Sk - Sq
        qi = jnp.arange(Sq)[:, None]
        kj = jnp.arange(Sk)[None, :]
        cmask = kj <= (qi + off)
        scores = jnp.where(cmask[None, None], scores, -1e9)
        p = _softmax(scores, axis=-1)
        ctx = jnp.einsum("bhqk,bhkd->bhqd", p, v)
        return jnp.einsum("bhqd,hdm->bqm", ctx, w_o)

    def _B_ref(x, wqkv, wo):
        B, S, D = x.shape
        H = 32; Dh = D // H
        W, dil = 8, 2
        qkv = (lambda x, *d: x.transpose(*d))((x @ wqkv).reshape(B, S, 3, H, Dh), 2, 0, 3, 1, 4)
        q, k, v = qkv[0], qkv[1], qkv[2]
        scale = Dh ** -0.5
        pos = jnp.arange(S)
        off = jnp.arange(W) * dil
        idx = pos[:, None] - off[None, :]
        mask = idx >= 0
        idx_c = jnp.where(mask, idx, 0).reshape(-1)
        kg = k[:, :, idx_c, :].reshape(B, H, S, W, Dh)
        vg = v[:, :, idx_c, :].reshape(B, H, S, W, Dh)
        logits = jnp.einsum("bhsd,bhswd->bhsw", q, kg) * scale
        logits = jnp.where(mask[None, None, :, :], logits, -1e9)
        attn = _softmax(logits, axis=-1)
        o = jnp.einsum("bhsw,bhswd->bhsd", attn, vg)
        return (lambda x, *d: x.transpose(*d))(o, 0, 2, 1, 3).reshape(B, S, D) @ wo

    a = _A_ref(A_x, A_c_kv, A_w_q, A_w_uk, A_w_uv, A_w_o)
    b = _B_ref(B_x, B_wqkv, B_wo)
    return jnp.concatenate([a, b], axis=-1)
```

```python
import functools
import math

import jax
import jax.numpy as jnp
from jax import lax
import jax.experimental.pallas as pl
import jax.experimental.pallas.tpu as pltpu

CFG = dict(BQ=256, RB=256, do_a=True, do_b=True, lag_out=2)

S = 2048
M = 1024
H = 32
D = 128
DC = 512
DH = 32
W = 8
DIL = 2
HALO = 16
LOG2E = math.log2(math.e)
NEG = -1e9 * LOG2E

F32 = jnp.float32
BF16 = jnp.bfloat16
NT = (((1,), (1,)), ((), ()))


def _dot(a, b):
    return jnp.dot(a, b, preferred_element_type=F32)


def _dot_nt(a, b):
    return lax.dot_general(a, b, NT, preferred_element_type=F32)


def _unpack_pair(w):
    lo = pltpu.bitcast(w << 16, F32)
    hi = pltpu.bitcast(w & jnp.uint32(0xFFFF0000), F32)
    return lo, hi


def _kernel(x_hbm, c_hbm, wq_hbm, wuk_hbm, wuv_hbm, wo_hbm, bx_hbm, wqkv_hbm, bwo_hbm,
            out_hbm,
            x_v, c_v, wq_v, wuk_v, wuv_v, wo_v, wq2, wkv2, q_s, k_s, v_s, ctx_s, acc,
            bx_v, wqkv_v, bwo_v, wt, bwo_p, qb, kb, vb, ob, outa, outb,
            sems, osems):
    BQ = CFG["BQ"]
    RB = CFG["RB"]
    NQ = S // BQ

    cps = [
        pltpu.make_async_copy(c_hbm, c_v, sems.at[0]),
        pltpu.make_async_copy(wuk_hbm.bitcast(jnp.uint32), wuk_v, sems.at[1]),
        pltpu.make_async_copy(wuv_hbm.bitcast(jnp.uint32), wuv_v, sems.at[2]),
        pltpu.make_async_copy(wq_hbm.bitcast(jnp.uint32), wq_v, sems.at[3]),
        pltpu.make_async_copy(x_hbm, x_v, sems.at[4]),
        pltpu.make_async_copy(wo_hbm, wo_v, sems.at[5]),
        pltpu.make_async_copy(bx_hbm, bx_v, sems.at[6]),
        pltpu.make_async_copy(wqkv_hbm, wqkv_v, sems.at[7]),
    ]
    bwo_cps = [
        pltpu.make_async_copy(bwo_hbm.at[:, pl.ds(128 * j, 128)], bwo_v.at[j], sems.at[8 + j])
        for j in range(8)
    ]
    for cp in cps + bwo_cps:
        cp.start()

    acc[...] = jnp.zeros(acc.shape, F32)
    for cp in cps[:6]:
        cp.wait()

    wq32, wuk32, wuv32 = wq_v, wuk_v, wuv_v

    def prep(t):
        for j, w32 in enumerate((wuk32, wuv32)):
            lo, hi = _unpack_pair(w32[pl.ds(t, DC, stride=H // 2), :])
            wkv2[:, 256 * j:256 * j + 128] = lo.astype(BF16)
            wkv2[:, 256 * j + 128:256 * j + 256] = hi.astype(BF16)
        lo, hi = _unpack_pair(wq32[pl.ds(t, M, stride=H // 2), :])
        wq2[:, 0:128] = lo.astype(BF16)
        wq2[:, 128:256] = hi.astype(BF16)

    qscale = (D ** -0.5) * LOG2E

    def pair_body(t, carry):
        row = lax.broadcasted_iota(jnp.int32, (128, 128), 0)
        col = lax.broadcasted_iota(jnp.int32, (128, 128), 1)
        tri = col <= row

        def proj(i):
            r = slice(i * BQ, (i + 1) * BQ)
            kv = _dot(c_v[r, :], wkv2[...]).astype(BF16)
            for h in range(2):
                k_s[h, r, :] = kv[:, 128 * h:128 * h + 128]
                v_s[h, r, :] = kv[:, 256 + 128 * h:256 + 128 * h + 128]
            q_s[r, :] = (_dot(x_v[r, :], wq2[...]) * qscale).astype(BF16)

        def qk(i, h):
            r0 = i * BQ
            nsub = BQ // 128
            q = q_s[r0:r0 + BQ, 128 * h:128 * h + 128]
            parts = [[] for _ in range(nsub)]
            full = r0 + 128
            s = _dot_nt(q, k_s[h, 0:full, :])
            for a in range(nsub):
                parts[a].append(s[128 * a:128 * a + 128])
            for d in range(1, nsub):
                s = _dot_nt(q[128 * d:], k_s[h, r0 + 128 * d:r0 + 128 * d + 128, :])
                for a in range(d, nsub):
                    parts[a].append(s[128 * (a - d):128 * (a - d) + 128])
            out = []
            for a in range(nsub):
                s = jnp.concatenate(parts[a], axis=1)
                n = s.shape[1]
                diag = jnp.where(tri, s[:, n - 128:], NEG)
                s = jnp.concatenate([s[:, :n - 128], diag], axis=1) if n > 128 else diag
                out.append((s, jnp.max(s, axis=-1, keepdims=True)))
            return out

        def pv(i, h, sc):
            r0 = i * BQ
            nsub = BQ // 128
            ps, ls = [], []
            for s, m in sc:
                p = jnp.exp2(s - m)
                ls.append(jnp.sum(p, axis=-1, keepdims=True))
                ps.append(p.astype(BF16))
            full = r0 + 128
            o = _dot(jnp.concatenate([p[:, :full] for p in ps], axis=0), v_s[h, 0:full, :])
            os_ = [o[128 * a:128 * a + 128] for a in range(nsub)]
            for d in range(1, nsub):
                c0 = r0 + 128 * d
                o = _dot(jnp.concatenate([p[:, c0:c0 + 128] for p in ps[d:]], axis=0),
                         v_s[h, c0:c0 + 128, :])
                for a in range(d, nsub):
                    os_[a] = os_[a] + o[128 * (a - d):128 * (a - d) + 128]
            for a in range(nsub):
                ctx_s[r0 + 128 * a:r0 + 128 * a + 128, 128 * h:128 * h + 128] = (
                    os_[a] * (1.0 / ls[a])).astype(BF16)

        def outp(i):
            r = slice(i * BQ, (i + 1) * BQ)
            acc[r, :] += _dot(ctx_s[r, :], wo_v[pl.ds(pl.multiple_of(t * 256, 256), 256), :])

        lag = CFG["lag_out"]
        proj(0)
        sc = {}
        for i in range(NQ):
            if i + 1 < NQ:
                proj(i + 1)
            sc[i, 0] = qk(i, 0)
            if i >= 1:
                pv(i - 1, 1, sc.pop((i - 1, 1)))
            sc[i, 1] = qk(i, 1)
            if i - lag >= 0:
                outp(i - lag)
            pv(i, 0, sc.pop((i, 0)))
            if i == NQ - 2:
                prep(jnp.minimum(t + 1, H // 2 - 1))
        pv(NQ - 1, 1, sc.pop((NQ - 1, 1)))
        for i in range(NQ - lag, NQ):
            outp(i)
        return carry

    if CFG["do_a"]:
        prep(0)
        lax.fori_loop(0, H // 2, pair_body, 0)

    outa[...] = acc[...].astype(BF16)
    oa = pltpu.make_async_copy(outa, out_hbm.at[:, pl.ds(0, M)], osems.at[0])
    oa.start()

    for cp in cps[6:] + bwo_cps:
        cp.wait()

    def wt_body(mb, carry):
        r = pl.ds(pl.multiple_of(mb * 128, 128), 128)
        for part in range(3):
            for cb in range(8):
                n0 = part * M + cb * 128
                tt = wqkv_v[r, n0:n0 + 128].astype(F32).T
                for hl in range(4):
                    wt[mb, pl.ds(part * M + 4 * cb + hl, DH, stride=H), :] = tt[32 * hl:32 * hl + 32]
        return carry

    bwo32 = bwo_v.bitcast(jnp.uint32)

    if CFG["do_b"]:
        lax.fori_loop(0, 8, wt_body, 0)
        for cb in range(8):
            for j in range(DH // 2):
                lo, hi = _unpack_pair(bwo32[cb, pl.ds(j, H, stride=DH // 2), :])
                bwo_p[64 * j:64 * j + 32, 128 * cb:128 * cb + 128] = lo.astype(BF16)
                bwo_p[64 * j + 32:64 * j + 64, 128 * cb:128 * cb + 128] = hi.astype(BF16)

    bscale = (DH ** -0.5) * LOG2E
    kb[:, RB:RB + HALO, :] = jnp.zeros((8, HALO, 128), F32)
    vb[:, RB:RB + HALO, :] = jnp.zeros((8, HALO, 128), F32)

    def b_copy(i):
        r = pl.ds(pl.multiple_of(i * RB, RB), RB)
        return pltpu.make_async_copy(outb.at[r, :], out_hbm.at[r, pl.ds(M, M)], osems.at[1 + i])

    def b_body(i, carry):
        r = pl.ds(pl.multiple_of(i * RB, RB), RB)
        xb = bx_v[r, :]

        def wpart(part):
            return jnp.concatenate(
                [wt[mb, part * M:(part + 1) * M, :] for mb in range(8)], axis=1).astype(BF16)

        kb[:, 0:HALO, :] = kb[:, RB:RB + HALO, :]
        vb[:, 0:HALO, :] = vb[:, RB:RB + HALO, :]
        qb[...] = _dot_nt(xb, wpart(0)) * bscale
        kk = _dot_nt(xb, wpart(1))
        for cb in range(8):
            kb[cb, HALO:HALO + RB, :] = kk[:, 128 * cb:128 * cb + 128]
        vv = _dot_nt(xb, wpart(2))
        for cb in range(8):
            vb[cb, HALO:HALO + RB, :] = vv[:, 128 * cb:128 * cb + 128]

        G = 16
        for g in range(RB // G):
            r0 = g * G
            qs = [qb[r0:r0 + G, 128 * cb:128 * cb + 128] for cb in range(8)]
            lg = []
            for w in range(W):
                o = HALO + r0 - DIL * w
                a = qs[0] * kb[0, o:o + G, :]
                for cb in range(1, 8):
                    a = a + qs[cb] * kb[cb, o:o + G, :]
                a = a + pltpu.roll(a, 64, 1)
                a = a + pltpu.roll(a, 32, 1)
                if r0 < DIL * w:
                    pos = i * RB + r0 + lax.broadcasted_iota(jnp.int32, (G, 128), 0)
                    a = jnp.where(pos >= DIL * w, a, NEG)
                lg.append(a)
            m = functools.reduce(jnp.maximum, lg)
            ps = [jnp.exp2(a - m) for a in lg]
            inv = 1.0 / functools.reduce(jnp.add, ps)
            ps = [p * inv for p in ps]
            for cb in range(8):
                a = None
                for w in range(W):
                    o = HALO + r0 - DIL * w
                    term = ps[w] * vb[cb, o:o + G, :]
                    a = term if a is None else a + term
                ob[r0:r0 + G, 128 * cb:128 * cb + 128] = a.astype(BF16)
        outb[r, :] = _dot(ob[...], bwo_p[...]).astype(BF16)
        b_copy(i).start()
        return carry

    if CFG["do_b"]:
        lax.fori_loop(0, S // RB, b_body, 0)
        for i in range(S // RB):
            b_copy(i).wait()
    oa.wait()


@jax.jit
def pallas_concat_heads__compressed_kv_cla__sliding_local_dilated__prompt_kernel(
    A_x: jax.Array,
    A_c_kv: jax.Array,
    A_w_q: jax.Array,
    A_w_uk: jax.Array,
    A_w_uv: jax.Array,
    A_w_o: jax.Array,
    B_x: jax.Array,
    B_wqkv: jax.Array,
    B_wo: jax.Array,
):
    RB = CFG["RB"]
    vm = pltpu.VMEM
    scratch = [
        vm((S, M), BF16), vm((S, DC), BF16),
        vm((M * H // 2, D), jnp.uint32), vm((DC * H // 2, D), jnp.uint32), vm((DC * H // 2, D), jnp.uint32),
        vm((H * D, M), BF16),
        vm((M, 2 * D), BF16), vm((DC, 4 * D), BF16),
        vm((S, 2 * D), BF16), vm((2, S, D), BF16), vm((2, S, D), BF16), vm((S, 2 * D), BF16),
        vm((S, M), F32),
        vm((S, M), BF16), vm((M, 3 * M), BF16), vm((8, M, 128), BF16),
        vm((8, 3 * M, 128), F32), vm((M, M), BF16),
        vm((RB, M), F32), vm((8, HALO + RB, 128), F32), vm((8, HALO + RB, 128), F32),
        vm((RB, M), BF16), vm((S, M), BF16), vm((S, M), BF16),
        pltpu.SemaphoreType.DMA((16,)), pltpu.SemaphoreType.DMA((1 + S // RB,)),
    ]
    out = pl.pallas_call(
        _kernel,
        out_shape=jax.ShapeDtypeStruct((S, 2 * M), BF16),
        in_specs=[pl.BlockSpec(memory_space=pl.ANY)] * 9,
        out_specs=pl.BlockSpec(memory_space=pl.ANY),
        scratch_shapes=scratch,
        compiler_params=pltpu.CompilerParams(vmem_limit_bytes=120 * 1024 * 1024),
        name="fused_ab",
    )(
        A_x.reshape(S, M), A_c_kv.reshape(S, DC),
        A_w_q.reshape(M * H, D), A_w_uk.reshape(DC * H, D), A_w_uv.reshape(DC * H, D),
        A_w_o.reshape(H * D, M),
        B_x.reshape(S, M), B_wqkv, B_wo,
    )
    return out.reshape(1, S, 2 * M)
```

```python
import functools
import math

import jax
import jax.numpy as jnp
from jax import lax
import jax.experimental.pallas as pl
import jax.experimental.pallas.tpu as pltpu

CFG = dict(na=16, R0=256, R1=512, R2=256, delay=400, lead=200, period=64, UT=2, nout=3, PR=32,
           mincost=256, flags=None, bperiod=128, LAG=2, G=16, do_b=True, n0=None, scopes=False)

S = 2048
M = 1024
H = 32
D = 128
DC = 512
DH = 32
W = 8
DIL = 2
HALO = 16
BQ = 256
NQ = S // BQ
WPITCH = DH // 2 + 1
LOG2E = math.log2(math.e)
NEG = -1e9 * LOG2E

F32 = jnp.float32
BF16 = jnp.bfloat16
U32 = jnp.uint32
NT = (((1,), (1,)), ((), ()))


def _dot(a, b):
    return jnp.dot(a, b, preferred_element_type=F32)


def _dot_nt(a, b):
    return lax.dot_general(a, b, NT, preferred_element_type=F32)


def _words(x):
    return pltpu.bitcast(x.astype(BF16), U32)


def _halves(w):
    return pltpu.bitcast(w, BF16)


def _unpack_pair(w):
    lo = pltpu.bitcast(w << 16, F32)
    hi = pltpu.bitcast(w & jnp.uint32(0xFFFF0000), F32)
    return lo, hi


def _recip(x):
    r = pl.reciprocal(x, approx=True)
    return r * (2.0 - x * r)


import contextlib
def _scope(name):
    return jax.named_scope(name) if CFG["scopes"] else contextlib.nullcontext()


def _rows(r0, n):
    return slice(r0 // 2, (r0 + n) // 2)


class _Interleaver:
    def __init__(self, zero, never):
        self.zero, self.never = zero, never
        self.steps = []
        self.side = []

    def mxu(self, cost, lhs, fn, name):
        self.steps.append((cost, lhs, fn, name))

    def vpu(self, after, before, buf, fns, until=None):
        self.side.append((after, before, buf, fns, until))

    def _tie(self, words, buf):
        token = buf[pl.ds(self.zero, 8), 0:128]
        return jnp.where(self.never, pltpu.bitcast(token, U32), words)

    def emit(self, delay, lead, period):
        start, end, starts, t = {}, {"begin": -delay}, [], 0
        for cost, _, _, name in self.steps:
            starts.append(t)
            start.setdefault(name, t)
            t += cost
            end[name] = t
        start["end"] = t
        todo = []
        for after, before, buf, fns, until in self.side:
            hi = start[before]
            lo = min(end[after] + delay, hi)
            hi = max(hi - lead, lo)
            if until is not None:
                hi = min(hi, end[until] + delay)
            total, done = sum(w for w, _ in fns), 0
            for w, fn in fns:
                done += w
                todo.append((lo + (hi - lo) * done / total, len(todo), fn, buf, start[before]))
        todo.sort(key=lambda e: e[:2])
        k = 0
        for (cost, lhs, fn, _), t0 in zip(self.steps, starts):
            while k < len(todo) and todo[k][4] <= t0:
                todo[k][2]()
                k += 1
            words = lhs()
            n = words.shape[0] // 8
            slabs = [words[8 * u:8 * u + 8] for u in range(n)]
            nslot = max(cost // period, 1) if cost >= CFG["mincost"] else 0
            for slot in range(nslot):
                bufs = []
                while k < len(todo) and todo[k][0] < t0 + cost * (slot + 1) / nslot:
                    todo[k][2]()
                    if not any(todo[k][3] is b for b in bufs):
                        bufs.append(todo[k][3])
                    k += 1
                u = (slot + 1) * n // nslot - 1
                for buf in bufs:
                    head = self._tie(slabs[u][:, 0:128], buf)
                    slabs[u] = (jnp.concatenate([head, slabs[u][:, 128:]], axis=1)
                                if words.shape[1] > 128 else head)
            fn(_halves(jnp.concatenate(slabs, axis=0)))
        for e in todo[k:]:
            e[2]()


def _weight_steps(t, wq_v, wuk_v, wuv_v, wq2, wk2, wv2):
    PR = CFG["PR"]
    held = []

    def gather(src, r0):
        return src[pl.ds(t + r0 * (H // 2), PR, stride=H // 2), :]

    def k_step(r0):
        held.append(gather(wuk_v, r0))
        if (r0 + PR) % 128 == 0:
            lo, hi = _unpack_pair(jnp.concatenate(held, axis=0).T)
            held.clear()
            c = slice(r0 + PR - 128, r0 + PR)
            wk2[0:64, c] = _words(lo)
            wk2[64:128, c] = _words(hi)

    def plain_step(src, dst, r0):
        lo, hi = _unpack_pair(gather(src, r0))
        dst[_rows(r0, PR), 0:128] = _words(lo)
        dst[_rows(r0, PR), 128:256] = _words(hi)

    return ([(wuk_v, functools.partial(k_step, r)) for r in range(0, DC, PR)]
            + [(wuv_v, functools.partial(plain_step, wuv_v, wv2, r)) for r in range(0, DC, PR)]
            + [(wq_v, functools.partial(plain_step, wq_v, wq2, r)) for r in range(0, M, PR)])


def _head_pair(t, x_v, c_v, wq_v, wuk_v, wuv_v, wo_v, wq2, wk2, wv2, q_s, k_s, v_s,
               ctx_a, ctx_b, s_s, p_s, acc):
    UT = CFG["UT"]
    qscale = (D ** -0.5) * LOG2E
    row = lax.broadcasted_iota(jnp.int32, (128, 128), 0)
    col = lax.broadcasted_iota(jnp.int32, (128, 128), 1)
    tri = col <= row
    st = {}
    zero = pl.multiple_of((t >> 8) * 8, 8)
    il = _Interleaver(zero, t < 0)

    def ctx(i):
        return ctx_a if i < NQ - 1 else ctx_b

    def normalizer(i, h, a, anchor):
        l = p_s[i % 2][pl.ds(zero + a, 64), S + 128 * h:S + 128 * h + 128]
        l = jnp.where(il.never, anchor, pltpu.bitcast(l, F32))
        st["inv", h, a] = _recip(jnp.sum(l, axis=-1, keepdims=True))

    def proj_k(i):
        def step(j, w):
            k_s[:, 128 * j:128 * j + 128] = _words(
                _dot_nt(w, _halves(c_v[_rows(128 * j, 128), :])))

        for j in range(2 * i, 2 * i + 2):
            il.mxu(256, lambda: wk2[...], functools.partial(step, j), ("proj", i))

    def proj_v(i, h):
        r, c = _rows(i * BQ, BQ), slice(128 * h, 128 * h + 128)

        def step(cc):
            y = _dot(cc, _halves(wv2[:, c]))
            v_s[r, c] = _words(y)
            if i >= 1:
                for a in range(0, BQ, 64):
                    normalizer(i - 1, h, a, y[a:a + 64])

        il.mxu(256, lambda: c_v[r, :], step, ("v", i))

    def proj_q(i, h):
        r, c = _rows(i * BQ, BQ), slice(128 * h, 128 * h + 128)

        def first(xx):
            st["q"] = _dot(xx, _halves(wq2[0:256, c]))

        def second(xx):
            q_s[r, c] = _words((st.pop("q") + _dot(xx, _halves(wq2[256:512, c]))) * qscale)

        il.mxu(256, lambda: x_v[r, 0:512], first, ("proj", i))
        il.mxu(256, lambda: x_v[r, 512:1024], second, ("proj", i))

    def pieces(i):
        n = 2 * i
        body = [(h, j, 4, 0, BQ) for h in range(2) for j in range(0, n - 3, 4)]
        if n % 4:
            body += [(h, n - 2, 2, 0, BQ) for h in range(2)]
        diag = ([(h, n, 1, 0, BQ) for h in range(2)]
                + [(h, n + 1, 1, 128, 128) for h in range(2)])
        return body, diag

    def qk(i):
        left = {}

        def piece(h, j, n, a0, nr, q):
            s = _dot(q, _halves(k_s[64 * h:64 * h + 64, 128 * j:128 * (j + n)]))
            for a in range(a0, a0 + nr, 64):
                m = st.get(("m", i, h, a))
                for u in range(n):
                    tile = s[a - a0:a - a0 + 64, 128 * u:128 * u + 128]
                    if j + u == 2 * i + a // 128:
                        tile = jnp.where(tri[a % 128:a % 128 + 64], tile, NEG)
                    s_s[i % 2][BQ * h + a:BQ * h + a + 64,
                               128 * (j + u):128 * (j + u + 1)] = tile
                    m = tile if m is None else jnp.maximum(m, tile)
                left[h, a] -= n
                if left[h, a] == 0:
                    m = jnp.broadcast_to(jnp.max(m, axis=-1, keepdims=True), (64, 128))
                st["m", i, h, a] = m

        body, diag = pieces(i)
        for h, j, n, a0, nr in diag + body[::-1]:
            for a in range(a0, a0 + nr, 64):
                left[h, a] = left.get((h, a), 0) + n
            il.mxu(nr * n // 4,
                   lambda h=h, a0=a0, nr=nr: q_s[_rows(i * BQ + a0, nr), 128 * h:128 * h + 128],
                   functools.partial(piece, h, j, n, a0, nr), ("qk", i))

    def softmax(i):
        sb, pb = s_s[i % 2], p_s[i % 2]

        def unit(h, r0, j0, j1, last):
            a = r0 // 64 * 64
            m = st["m", i, h, a][r0 - a:r0 - a + 16]
            l = st.pop(("l", i), None)
            r = BQ * h + r0
            for j in range(j0, j1):
                p = jnp.exp2(sb[pl.ds(zero + r, 16), 128 * j:128 * j + 128] - m)
                l = p if l is None else l + p
                pb[_rows(r, 16), 128 * j:128 * j + 128] = _words(p)
            if last:
                pb[r0:r0 + 16, S + 128 * h:S + 128 * h + 128] = pltpu.bitcast(l, U32)
            else:
                st["l", i] = l

        fns = []
        for h in (1, 0):
            for r0 in range(0, BQ, 16):
                n = 2 * i + 1 + r0 // 128
                for j0 in range(0, n, UT):
                    j1 = min(j0 + UT, n)
                    fns.append((j1 - j0, functools.partial(unit, h, r0, j0, j1, j1 == n)))
        if i < NQ - 1:
            il.vpu(("qk", i), ("v", i + 1), pb, fns, until=("qk", i + 1) if i else None)
        else:
            il.vpu(("qk", i), ("pv", i), pb, fns)

    def pv(i):
        pb = p_s[i % 2]
        left = {}

        def piece(h, j, n, a0, nr, p):
            c = slice(128 * h, 128 * h + 128)
            o = _dot(p, _halves(v_s[_rows(128 * j, 128 * n), c]))
            for a in range(a0, a0 + nr, 64):
                part = o[a - a0:a - a0 + 64]
                prev = st.pop(("o", h, a), None)
                if prev is None and i == NQ - 1:
                    normalizer(i, h, a, part)
                part = part if prev is None else prev + part
                left[h, a] -= n
                if left[h, a] == 0:
                    ctx(i)[_rows(i * BQ + a, 64), c] = _words(part * st.pop(("inv", h, a)))
                else:
                    st["o", h, a] = part

        body, diag = pieces(i)
        for h, j, n, a0, nr in (diag + body[::-1] if i == NQ - 1 else body + diag):
            for a in range(a0, a0 + nr, 64):
                left[h, a] = left.get((h, a), 0) + n
            il.mxu(nr * n // 4,
                   lambda h=h, j=j, n=n, a0=a0, nr=nr: pb[
                       pl.ds(zero + (BQ * h + a0) // 2, nr // 2), 128 * j:128 * (j + n)],
                   functools.partial(piece, h, j, n, a0, nr), ("pv", i))
        if i < NQ - 1:
            il.vpu(("pv", i), ("out", i), ctx(i), [(1, lambda: None)], until=("pv", i))

    upcoming = _weight_steps(jnp.minimum(t + 1, H // 2 - 1), wq_v, wuk_v, wuv_v, wq2, wk2, wv2)

    def outp(i):
        def piece(n0, cx):
            c = slice(n0, n0 + 256)
            wo = wo_v[pl.ds(pl.multiple_of(t * 128, 128), 128), c]
            y = _dot(cx, _halves(wo))
            acc[i * BQ:(i + 1) * BQ, c] += y
            for r0 in range(0, BQ, 2 * CFG["PR"]):
                if i >= NQ - 5 and upcoming:
                    src, fn = upcoming.pop(0)
                    src[src.shape[0] - 8:, :] = pltpu.bitcast(y[r0:r0 + 8, 0:128], U32)
                    fn()

        for n0 in range(0, M, 256):
            il.mxu(256, lambda: ctx(i)[pl.ds(zero + i * BQ // 2, BQ // 2), :],
                   functools.partial(piece, n0), ("out", i))

    for i in range(2):
        proj_k(i)
        proj_q(i, 0)
        proj_q(i, 1)
    proj_v(0, 0)
    proj_v(0, 1)
    qk(0)
    softmax(0)
    for i in range(1, NQ):
        qk(i)
        softmax(i)
        if i + 1 < NQ:
            proj_k(i + 1)
            proj_q(i + 1, 0)
            proj_q(i + 1, 1)
        proj_v(i, 0)
        proj_v(i, 1)
        if i + 1 == NQ:
            for n in range(CFG["nout"]):
                outp(n)
        pv(i - 1)
    pv(NQ - 1)
    for i in range(CFG["nout"], NQ):
        outp(i)
    il.emit(CFG["delay"], CFG["lead"], CFG["period"])
    assert not upcoming


def _wt_steps(part, w_v, wt):
    def step(mb, cb):
        n0 = part * M + 128 * cb
        tt = pltpu.bitcast(_halves(w_v[64 * mb:64 * mb + 64, n0:n0 + 128]).T, U32)
        for hl in range(4):
            r = (4 * cb + hl) * WPITCH
            wt[part, mb, r:r + 16, :] = tt[16 * hl:16 * hl + 16]

    return [functools.partial(step, mb, cb) for mb in range(8) for cb in range(8)]


def _bwo_steps(bwo_v, bwo_p):
    def step(cb, j):
        bwo_p[H * j:H * j + H, 128 * cb:128 * cb + 128] = bwo_v[cb, pl.ds(j, H, stride=DH // 2), :]

    return [functools.partial(step, cb, j) for cb in range(8) for j in range(DH // 2)]


def _b_project(il, bx_v, wt, part, row0, nrows, store, name):
    st = {}

    def rhs(cb, half):
        return _halves(jnp.concatenate(
            [jnp.concatenate([wt[part, mb, pl.ds(j, H, stride=WPITCH), :]
                              for j in (2 * cb, 2 * cb + 1)], axis=0)
             for mb in range(4 * half, 4 * half + 4)], axis=1))

    def first(cb, xx):
        st["y"] = _dot_nt(xx, rhs(cb, 0))

    def second(cb, r, xx):
        store(cb, r, st.pop("y") + _dot_nt(xx, rhs(cb, 1)))

    for r in range(0, nrows, 256):
        rr = pl.ds(pl.multiple_of((row0 + r) // 2, 128), 128)
        for cb in range(8):
            il.mxu(256, lambda rr=rr: bx_v[rr, 0:512], functools.partial(first, cb), name)
            il.mxu(256, lambda rr=rr: bx_v[rr, 512:1024], functools.partial(second, cb, r), name)


def _b_prob_steps(row0, nrows, cur, k_f, prob):
    G = CFG["G"]
    st = {}
    even = lax.broadcasted_iota(jnp.int32, (G, 128), 1) % 2 == 0

    def products(r0):
        qs = [cur[cb, HALO + r0:HALO + r0 + G, :] for cb in range(8)]
        out = []
        for w in range(W):
            r = pl.ds(row0 + (HALO + r0 - DIL * w), G)
            a = qs[0] * k_f[0, r, :]
            for cb in range(1, 8):
                a = a + qs[cb] * k_f[cb, r, :]
            out.append(a + pltpu.roll(a, 64, 1))
        st[r0] = out

    def finish(r0):
        lg = []
        for w, a in enumerate(st.pop(r0)):
            a = a + jnp.where(even, pltpu.roll(a, 127, 1), pltpu.roll(a, 1, 1))
            if r0 < DIL * w:
                pos = row0 + r0 + lax.broadcasted_iota(jnp.int32, (G, 128), 0)
                a = jnp.where(pos >= DIL * w, a, NEG)
            lg.append(a)
        m = functools.reduce(jnp.maximum, lg)
        ps = [jnp.exp2(a - m) for a in lg]
        inv = _recip(functools.reduce(jnp.add, ps))
        for w in range(W):
            prob[pl.ds(pl.multiple_of(row0 + r0, G), G), 128 * w:128 * w + 128] = ps[w] * inv

    starts = list(range(0, nrows, G))
    fns = []
    for n in range(len(starts) + CFG["LAG"]):
        if n < len(starts):
            fns.append((1, functools.partial(products, starts[n])))
        if n >= CFG["LAG"]:
            fns.append((1, functools.partial(finish, starts[n - CFG["LAG"]])))
    return fns


def _b_mix_steps(row0, nrows, cur, prob, o_s):
    def step(r0):
        r = pl.multiple_of(row0 + r0, 16)
        ps = [prob[pl.ds(r, 16), 128 * w:128 * w + 128] for w in range(W)]
        for cb in range(8):
            a = None
            for w in range(W):
                o = HALO + r0 - DIL * w
                term = ps[w] * cur[cb, o:o + 16, :]
                a = term if a is None else a + term
            o_s[pl.ds(pl.multiple_of(r // 2, 8), 8), 128 * cb:128 * cb + 128] = _words(a)

    return [(1, functools.partial(step, r0)) for r0 in range(0, nrows, 16)]


def _kernel(x_hbm, c_hbm, wq_hbm, wuk_hbm, wuv_hbm, wo_hbm, bx_hbm, wqkv_hbm, bwo_hbm,
            out_hbm,
            x_v, c_v, wq_v, wuk_v, wuv_v, wo_v, wq2, wk2, wv2, q_s, k_s, v_s, ctx_a, ctx_b,
            s_a, s_b, p_a, p_b, acc,
            bx_v, wqkv_v, bwo_v, wt, bwo_p, k_f, cur, nxt, prob, o_s, o_l, out_v,
            a_sems, b_sems, x_sems, o_sems):
    R0, R1, R2 = CFG["R0"], CFG["R1"], CFG["R2"]
    bscale = (DH ** -0.5) * LOG2E

    a_copies = [
        pltpu.make_async_copy(src.bitcast(U32), dst, a_sems.at[n])
        for n, (src, dst) in enumerate((
            (wuk_hbm, wuk_v.at[pl.ds(0, DC * H // 2)]),
            (wuv_hbm, wuv_v.at[pl.ds(0, DC * H // 2)]),
            (wq_hbm, wq_v.at[pl.ds(0, M * H // 2)]),
            (c_hbm, c_v), (x_hbm, x_v), (wo_hbm, wo_v)))]
    w_copies = [
        pltpu.make_async_copy(wqkv_hbm.bitcast(U32).at[:, pl.ds(n * M, M)],
                              wqkv_v.at[:, pl.ds(n * M, M)], b_sems.at[n])
        for n in range(3)]
    bwo_copies = [
        pltpu.make_async_copy(bwo_hbm.bitcast(U32).at[:, pl.ds(128 * j, 128)], bwo_v.at[j],
                              b_sems.at[3 + j])
        for j in range(8)]

    def bx_copy(c):
        r = pl.ds(pl.multiple_of(c * (R0 // 2), R0 // 2), R0 // 2)
        return pltpu.make_async_copy(bx_hbm.bitcast(U32).at[r, :], bx_v.at[r, :], x_sems.at[c])

    def out_copy(c, half):
        r = pl.ds(pl.multiple_of(c * (R2 // 2), R2 // 2), R2 // 2)
        cols = pl.ds(half * M, M)
        return pltpu.make_async_copy(out_v.at[r, cols], out_hbm.bitcast(U32).at[r, cols],
                                     o_sems.at[2 * c + half])

    def interleaver(c):
        return _Interleaver(pl.multiple_of((c >> 8) * 8, 8), c < 0)

    w_copies[1].start()
    bx_copy(0).start()
    acc[...] = jnp.zeros(acc.shape, F32)
    k_f[:, 0:HALO, :] = jnp.zeros((8, HALO, 128), F32)
    prob[0:8, 0:128] = jnp.zeros((8, 128), F32)
    o_s[0:8, 0:128] = jnp.zeros((8, 128), U32)
    o_l[0:8, 0:128] = jnp.zeros((8, 128), U32)
    with _scope('w0'):
        w_copies[1].wait()
    for c in range(1, S // R0):
        bx_copy(c).start()
    for cp in [w_copies[0], w_copies[2]] + bwo_copies + a_copies:
        cp.start()
    for fn in _wt_steps(1, wqkv_v, wt):
        fn()

    def key_rows(c, carry):
        bx_copy(c).wait()
        il = interleaver(c)
        row0 = pl.multiple_of(c * R0, R0)

        def store(cb, r, y):
            k_f[cb, pl.ds(pl.multiple_of(row0 + (HALO + r), 8), 256), :] = y * bscale

        _b_project(il, bx_v, wt, 1, row0, R0, store, "k")
        il.emit(0, 0, 256)
        return carry

    with _scope('L0'):
        lax.fori_loop(0, S // R0, key_rows, 0)

    with _scope('w1'):
        for cp in [w_copies[0], w_copies[2]] + bwo_copies:
            cp.wait()
    for fn in _wt_steps(0, wqkv_v, wt) + _wt_steps(2, wqkv_v, wt) + _bwo_steps(bwo_v, bwo_p):
        fn()

    def store_into(buf):
        def store(cb, r, y):
            buf[cb, HALO + r:HALO + r + 256, :] = y
        return store

    n1 = S // R1

    def first_rows(c, carry):
        il = interleaver(c)
        _b_project(il, bx_v, wt, 0, 0, R1, store_into(cur), "q")
        il.emit(0, 0, 256)
        return carry

    lax.fori_loop(0, 1, first_rows, 0)

    def prob_rows(c, carry):
        il = interleaver(c)
        last = c == n1 - 1
        _b_project(il, bx_v, wt, jnp.where(last, 2, 0), jnp.where(last, 0, (c + 1) * R1), R1,
                   store_into(nxt), "q")
        il.vpu("begin", "end", prob,
               _b_prob_steps(pl.multiple_of(c * R1, R1), R1, cur, k_f, prob))
        il.emit(0, 300, CFG["bperiod"])
        cur[:, HALO:, :] = nxt[:, HALO:, :]
        return carry

    with _scope('L1'):
        lax.fori_loop(0, n1, prob_rows, 0)
    cur[:, 0:HALO, :] = jnp.zeros((8, HALO, 128), F32)

    def mix_rows(c, carry):
        il = interleaver(c)
        _b_project(il, bx_v, wt, 2, (c + 1) * R1, R1, store_into(nxt), "v")
        il.vpu("begin", "end", o_s,
               _b_mix_steps(pl.multiple_of(c * R1, R1), R1, cur, prob, o_s))
        il.emit(0, 300, CFG["bperiod"])
        cur[:, 0:HALO, :] = cur[:, R1:R1 + HALO, :]
        cur[:, HALO:, :] = nxt[:, HALO:, :]
        return carry

    with _scope('L2'):
        lax.fori_loop(0, n1 - 1, mix_rows, 0)

    with _scope('w2'):
        for cp in a_copies:
            cp.wait()
    for _, fn in _weight_steps(0, wq_v, wuk_v, wuv_v, wq2, wk2, wv2):
        fn()

    def head_pair(t, carry):
        _head_pair(t, x_v, c_v, wq_v, wuk_v, wuv_v, wo_v, wq2, wk2, wv2, q_s, k_s, v_s,
                   ctx_a, ctx_b, (s_a, s_b), (p_a, p_b), acc)
        return carry

    with _scope('LA'):
        lax.fori_loop(0, CFG["na"], head_pair, 0)

    def out_rows(c, with_mix):
        il = interleaver(c)
        rr = pl.ds(pl.multiple_of(c * (R2 // 2), R2 // 2), R2 // 2)
        out_v[rr, 0:M] = _words(acc[pl.ds(pl.multiple_of(c * R2, R2), R2), :])
        out_copy(c, 0).start()
        st = {}

        def first(n0, oo):
            st["y"] = _dot(oo, _halves(bwo_p[0:256, n0:n0 + 128]))

        def second(n0, r, oo):
            y = st.pop("y") + _dot(oo, _halves(bwo_p[256:512, n0:n0 + 128]))
            out_v[r, M + n0:M + n0 + 128] = _words(y)

        for r0 in range(0, R2, 256):
            r = pl.ds(pl.multiple_of((c * R2 + r0) // 2, 128), 128)
            for n0 in range(0, M, 128):
                il.mxu(256, lambda r=r: o_s[r, 0:512], functools.partial(first, n0), "o")
                il.mxu(256, lambda r=r: o_s[r, 512:1024], functools.partial(second, n0, r), "o")
        if with_mix:
            il.vpu("begin", "end", o_l, _b_mix_steps(0, R1, cur, prob.at[pl.ds(S - R1, R1)], o_l))
        il.emit(0, 300, CFG["bperiod"])
        if with_mix:
            o_s[_rows(S - R1, R1), :] = o_l[...]
        out_copy(c, 1).start()

    lax.fori_loop(0, 1, lambda c, carry: out_rows(c, True), None)
    with _scope('L3'):
        lax.fori_loop(1, S // R2, lambda c, carry: out_rows(c, False), None)
    with _scope('w3'):
        for c in range(S // R2):
            out_copy(c, 0).wait()
            out_copy(c, 1).wait()


@jax.jit
def pallas_concat_heads__compressed_kv_cla__sliding_local_dilated__prompt_kernel(
    A_x: jax.Array,
    A_c_kv: jax.Array,
    A_w_q: jax.Array,
    A_w_uk: jax.Array,
    A_w_uv: jax.Array,
    A_w_o: jax.Array,
    B_x: jax.Array,
    B_wqkv: jax.Array,
    B_wo: jax.Array,
):
    R0, R1, R2 = CFG["R0"], CFG["R1"], CFG["R2"]
    vm = pltpu.VMEM
    scratch = [
        vm((S // 2, M), U32), vm((S // 2, DC), U32),
        vm((M * H // 2 + 8, D), U32), vm((DC * H // 2 + 8, D), U32),
        vm((DC * H // 2 + 8, D), U32), vm((H * D // 2, M), U32),
        vm((M // 2, 2 * D), U32), vm((D, DC), U32), vm((DC // 2, 2 * D), U32),
        vm((S // 2, 2 * D), U32), vm((D, S), U32), vm((S // 2, 2 * D), U32),
        vm((S // 2, 2 * D), U32), vm((S // 2, 2 * D), U32),
        vm((2 * BQ, S), F32), vm((2 * BQ, S), F32),
        vm((BQ, S + 2 * D), U32), vm((BQ, S + 2 * D), U32),
        vm((S, M), F32),
        vm((S // 2, M), U32), vm((M // 2, 3 * M), U32), vm((8, M // 2, 128), U32),
        vm((3, 8, H * WPITCH, 128), U32), vm((M // 2, M), U32),
        vm((8, HALO + S, 128), F32), vm((8, HALO + R1, 128), F32), vm((8, HALO + R1, 128), F32),
        vm((S, W * 128), F32), vm((S // 2, M), U32), vm((R1 // 2, M), U32),
        vm((S // 2, 2 * M), U32),
        pltpu.SemaphoreType.DMA((6,)), pltpu.SemaphoreType.DMA((11,)),
        pltpu.SemaphoreType.DMA((S // R0,)), pltpu.SemaphoreType.DMA((2 * S // R2,)),
    ]
    out = pl.pallas_call(
        _kernel,
        out_shape=jax.ShapeDtypeStruct((S, 2 * M), BF16),
        in_specs=[pl.BlockSpec(memory_space=pl.ANY)] * 9,
        out_specs=pl.BlockSpec(memory_space=pl.ANY),
        scratch_shapes=scratch,
        compiler_params=pltpu.CompilerParams(vmem_limit_bytes=124 * 1024 * 1024,
                                             flags=CFG["flags"]),
        name="fused_ab",
    )(
        A_x.reshape(S, M), A_c_kv.reshape(S, DC),
        A_w_q.reshape(M * H, D), A_w_uk.reshape(DC * H, D), A_w_uv.reshape(DC * H, D),
        A_w_o.reshape(H * D, M),
        B_x.reshape(S, M), B_wqkv, B_wo,
    )
    return out.reshape(1, S, 2 * M)
```

```python
import functools
import math

import jax
import jax.numpy as jnp
from jax import lax
import jax.experimental.pallas as pl
import jax.experimental.pallas.tpu as pltpu

CFG = dict(na=16, R0=256, R1=256, R2=256, fw=3, NS=1, bdelay=0, only=None, R3=256, ahead=256, prep_after=('v', 7), spad=0, ppad=0, PN=2, late_v=0, btie=1, blead=300, delay=400, lead=200, period=32, UT=1, nout=3, PR=32,
           mincost=256, flags=None, bperiod=32, LAG=1, G=16, do_b=True, n0=None, scopes=False)

S = 2048
M = 1024
H = 32
D = 128
DC = 512
DH = 32
W = 8
DIL = 2
HALO = 16
BQ = 256
NQ = S // BQ
WPITCH = DH // 2 + 1
LOG2E = math.log2(math.e)
NEG = -1e9 * LOG2E

F32 = jnp.float32
BF16 = jnp.bfloat16
U32 = jnp.uint32
NT = (((1,), (1,)), ((), ()))


def _dot(a, b):
    return jnp.dot(a, b, preferred_element_type=F32)


def _dot_nt(a, b):
    return lax.dot_general(a, b, NT, preferred_element_type=F32)


def _words(x):
    return pltpu.bitcast(x.astype(BF16), U32)


def _halves(w):
    return pltpu.bitcast(w, BF16)


def _unpack_pair(w):
    lo = pltpu.bitcast(w << 16, F32)
    hi = pltpu.bitcast(w & jnp.uint32(0xFFFF0000), F32)
    return lo, hi


def _recip(x):
    r = pl.reciprocal(x, approx=True)
    return r * (2.0 - x * r)


import contextlib
def _scope(name):
    return jax.named_scope(name) if CFG["scopes"] else contextlib.nullcontext()


def _rows(r0, n):
    return slice(r0 // 2, (r0 + n) // 2)


class _Interleaver:
    def __init__(self, never):
        self.never = never
        self.steps = []
        self.side = []

    def mxu(self, cost, lhs, fn, name):
        self.steps.append((cost, lhs, fn, name))

    def vpu(self, after, before, fns, token, until=None):
        self.side.append((after, before, fns, until, token))

    def emit(self, delay, lead, period):
        start, end, starts, t = {}, {"begin": -delay}, [], 0
        for cost, _, _, name in self.steps:
            starts.append(t)
            start.setdefault(name, t)
            t += cost
            end[name] = t
        start["end"] = t
        slots = [t0 + cost * (s + 1) / (cost // period)
                 for (cost, _, _, _), t0 in zip(self.steps, starts)
                 if cost >= CFG["mincost"] for s in range(cost // period)]
        todo = []
        for after, before, fns, until, token in self.side:
            hi = start[before]
            lo = min(end[after] + delay, hi)
            hi = max(hi - lead, lo)
            if until is not None:
                hi = min(hi, end[until] + delay)
            mine = [s for s in slots if lo <= s <= hi] or [lo]
            total, done = sum(w for w, _ in fns), 0
            for w, fn in fns:
                when = mine[min(int(len(mine) * (done + w / 2) / total), len(mine) - 1)]
                todo.append((when, len(todo), fn, start[before], token))
                done += w
        todo.sort(key=lambda e: e[:2])
        k = 0
        results = []

        def hold(now):
            past = [y for t, y in results if t <= now - CFG["ahead"]]
            if not past or not CFG["ahead"]:
                return lambda x: x
            return lambda x: jnp.where(
                self.never, jnp.concatenate([past[-1]] * (x.shape[0] // 8), axis=0), x)

        for (cost, lhs, fn, _), t0 in zip(self.steps, starts):
            while k < len(todo) and todo[k][3] <= t0:
                todo[k][2](hold(t0))
                k += 1
            words = lhs()
            n = words.shape[0] // 8
            slabs = [words[8 * u:8 * u + 8] for u in range(n)]
            nslot = cost // period if cost >= CFG["mincost"] else 0
            for slot in range(nslot):
                tokens = []
                t1 = t0 + cost * (slot + 1) / nslot
                while k < len(todo) and todo[k][0] <= t1:
                    todo[k][2](hold(t1))
                    if todo[k][4] is not None and todo[k][4] not in tokens:
                        tokens.append(todo[k][4])
                    k += 1
                u = (slot + 1) * n // nslot - 1
                for token in tokens:
                    head = jnp.where(self.never, token(), slabs[u][:, 0:128])
                    slabs[u] = (jnp.concatenate([head, slabs[u][:, 128:]], axis=1)
                                if words.shape[1] > 128 else head)
            y = fn(_halves(jnp.concatenate(slabs, axis=0)))
            if cost == 256:
                results += [(t0 + cost * (u + 1) / n, y[16 * u:16 * u + 8, 0:128])
                            for u in range(n)]
        for e in todo[k:]:
            e[2](hold(t))


def _read_back(buf, zero):
    return lambda: pltpu.bitcast(buf[pl.ds(zero, 8), 0:128], U32)


def _fence(buf, zero):
    buf[pl.ds(zero + (buf.shape[0] - 8), 8), 0:128] = jnp.zeros((8, 128), buf.dtype)


def _weight_steps(t, wq_v, wuk_v, wuv_v, wq2, wk2, wv2):
    PR = CFG["PR"]
    held = []

    def gather(src, r0):
        return src[pl.ds(t + r0 * (H // 2), PR, stride=H // 2), :]

    def k_step(r0):
        held.append(gather(wuk_v, r0))
        if (r0 + PR) % 128 == 0:
            lo, hi = _unpack_pair(jnp.concatenate(held, axis=0).T)
            held.clear()
            c = slice(r0 + PR - 128, r0 + PR)
            wk2[0:64, c] = _words(lo)
            wk2[64:128, c] = _words(hi)

    def plain_step(src, dst, r0):
        lo, hi = _unpack_pair(gather(src, r0))
        dst[_rows(r0, PR), 0:128] = _words(lo)
        dst[_rows(r0, PR), 128:256] = _words(hi)

    return ([(wuk_v, functools.partial(k_step, r)) for r in range(0, DC, PR)]
            + [(wq_v, functools.partial(plain_step, wq_v, wq2, r)) for r in range(0, M, PR)]
            + [(wuv_v, functools.partial(plain_step, wuv_v, wv2, r)) for r in range(0, DC, PR)])


def _head_pair(t, x_v, c_v, wq_v, wuk_v, wuv_v, wq2, wk2, wv2, q_s, k_s, v_s, s_s, p_s, ctx):
    UT = CFG["UT"]
    qscale = (D ** -0.5) * LOG2E
    row = lax.broadcasted_iota(jnp.int32, (128, 128), 0)
    col = lax.broadcasted_iota(jnp.int32, (128, 128), 1)
    tri = col <= row
    zero = pl.multiple_of((t >> 8) * 8, 8)
    ctx_row = pl.multiple_of(t * (S // 2), S // 2)
    st = {}
    il = _Interleaver(t < 0)
    upcoming = _weight_steps(jnp.minimum(t + 1, H // 2 - 1), wq_v, wuk_v, wuv_v, wq2, wk2, wv2)

    def normalizer(i, h, a, anchor):
        l = p_s[i % 3][a:a + 64, S + 128 * h:S + 128 * h + 128]
        l = jnp.where(il.never, anchor, pltpu.bitcast(l, F32))
        st["inv", i, h, a] = _recip(jnp.sum(l, axis=-1, keepdims=True))

    def proj_k(i):
        def step(j, w):
            y = _dot_nt(w, _halves(c_v[_rows(128 * j, 128), :]))
            k_s[:, 128 * j:128 * j + 128] = _words(y)
            return y

        for j in range(2 * i, 2 * i + 2):
            il.mxu(256, lambda: wk2[...], functools.partial(step, j), ("proj", i))

    def proj_v(i, h, n):
        def step(cc):
            y = _dot(cc, _halves(wv2[:, 128 * h:128 * h + 128]))
            v_s[_rows(i * BQ, BQ), 128 * h:128 * h + 128] = _words(y)
            if n is not None:
                for a in range(0, BQ, 64):
                    normalizer(n, h, a, y[a:a + 64])
            return y

        il.mxu(256, lambda: c_v[_rows(i * BQ, BQ), :], step, ("v", i))

    def proj_q(i, h):
        r, c = _rows(i * BQ, BQ), slice(128 * h, 128 * h + 128)

        def first(xx):
            st["q"] = _dot(xx, _halves(wq2[0:256, c]))
            return st["q"]

        def second(xx):
            y = _dot(xx, _halves(wq2[256:512, c]))
            q_s[r, c] = _words((st.pop("q") + y) * qscale)
            return y

        il.mxu(256, lambda: x_v[r, 0:512], first, ("proj", i))
        il.mxu(256, lambda: x_v[r, 512:1024], second, ("proj", i))

    def pieces(i):
        n = 2 * i
        body = [(h, j, 4, 0, BQ) for h in range(2) for j in range(0, n - 3, 4)]
        if n % 4:
            body += [(h, n - 2, 2, 0, BQ) for h in range(2)]
        diag = ([(h, n, 1, 0, BQ) for h in range(2)]
                + [(h, n + 1, 1, 128, 128) for h in range(2)])
        return body, diag

    def qk(i, diag_first):
        left = {}

        def piece(h, j, n, a0, nr, q):
            s = _dot(q, _halves(k_s[64 * h:64 * h + 64, 128 * j:128 * (j + n)]))
            for a in range(a0, a0 + nr, 64):
                m = st.get(("m", i, h, a))
                for u in range(n):
                    tile = s[a - a0:a - a0 + 64, 128 * u:128 * u + 128]
                    if j + u == 2 * i + a // 128:
                        tile = jnp.where(tri[a % 128:a % 128 + 64], tile, NEG)
                    s_s[i % 2][BQ * h + a:BQ * h + a + 64,
                               128 * (j + u):128 * (j + u + 1)] = tile
                    m = tile if m is None else jnp.maximum(m, tile)
                left[h, a] -= n
                if left[h, a] == 0:
                    m = jnp.broadcast_to(jnp.max(m, axis=-1, keepdims=True), (64, 128))
                st["m", i, h, a] = m
            if not any(left[h, a] for a in range(0, BQ, 64)):
                _fence(s_s[i % 2], zero)
            return s

        body, diag = pieces(i)
        for h, j, n, a0, nr in (diag + body[::-1] if diag_first else body[::-1] + diag):
            for a in range(a0, a0 + nr, 64):
                left[h, a] = left.get((h, a), 0) + n
            il.mxu(nr * n // 4,
                   lambda h=h, a0=a0, nr=nr: q_s[_rows(i * BQ + a0, nr), 128 * h:128 * h + 128],
                   functools.partial(piece, h, j, n, a0, nr), ("qk", i))

    def softmax(i, before, until):
        sb, pb = s_s[i % 2], p_s[i % 3]

        def unit(h, r0, j0, j1, last, hold):
            a = r0 // 64 * 64
            m = hold(st["m", i, h, a][r0 - a:r0 - a + 16])
            l = st.pop(("l", i), None)
            r = BQ * h + r0
            for j in range(j0, j1):
                p = jnp.exp2(sb[r:r + 16, 128 * j:128 * j + 128] - m)
                l = p if l is None else l + p
                pb[_rows(r, 16), 128 * j:128 * j + 128] = _words(p)
            if last:
                pb[r0:r0 + 16, S + 128 * h:S + 128 * h + 128] = pltpu.bitcast(l, U32)
                if r0 + 16 == BQ and h == 0:
                    _fence(pb, zero)
            else:
                st["l", i] = l

        fns = []
        for h in (1, 0):
            for r0 in range(0, BQ, 16):
                n = 2 * i + 1 + r0 // 128
                for j0 in range(0, n, UT):
                    j1 = min(j0 + UT, n)
                    fns.append((j1 - j0, functools.partial(unit, h, r0, j0, j1, j1 == n)))
        il.vpu(("qk", i), before, fns, _read_back(pb, zero + BQ // 2), until)

    def pv(i, diag_first):
        left = {}

        def probs(h, j, n, a0, nr):
            return p_s[i % 3][_rows(BQ * h + a0, nr), 128 * j:128 * (j + n)]

        def piece(h, j, n, a0, nr, p):
            o = _dot(p, _halves(v_s[_rows(128 * j, 128 * n), 128 * h:128 * h + 128]))
            for a in range(a0, a0 + nr, 64):
                part = o[a - a0:a - a0 + 64]
                if ("inv", i, h, a) not in st:
                    normalizer(i, h, a, part)
                prev = st.pop(("o", h, a), None)
                part = part if prev is None else prev + part
                left[h, a] -= n
                if left[h, a] == 0:
                    ctx[pl.ds(ctx_row + (i * BQ + a) // 2, 32), 128 * h:128 * h + 128] = _words(
                        part * st.pop(("inv", i, h, a)))
                else:
                    st["o", h, a] = part
            return o

        body, diag = pieces(i)
        for h, j, n, a0, nr in (diag + body[::-1] if diag_first else body + diag):
            for a in range(a0, a0 + nr, 64):
                left[h, a] = left.get((h, a), 0) + n
            il.mxu(nr * n // 4, functools.partial(probs, h, j, n, a0, nr),
                   functools.partial(piece, h, j, n, a0, nr), ("pv", i))
        if i < NQ - 1:
            il.vpu(("pv", i), "end", [(1, lambda hold: None)], _read_back(ctx, ctx_row + zero),
                   until=("pv", i))

    def gather(src, fn, hold):
        src[src.shape[0] - 8:, :] = pltpu.bitcast(hold(jnp.zeros((8, 128), F32)), U32)
        fn()

    for i in range(2):
        proj_k(i)
        proj_q(i, 0)
        proj_q(i, 1)
    proj_v(0, 0, None)
    proj_v(0, 1, None)
    qk(0, True)
    softmax(0, ("v", 1), None)
    for i in range(1, NQ - 1):
        qk(i, True)
        softmax(i, ("v", i + 1), ("qk", i + 1))
        proj_k(i + 1)
        proj_q(i + 1, 0)
        proj_q(i + 1, 1)
        proj_v(i, 0, i - 1)
        proj_v(i, 1, i - 1)
        if i < NQ - 2:
            pv(i - 1, False)
    qk(NQ - 1, False)
    softmax(NQ - 1, ("pv", NQ - 1), None)
    pv(NQ - 3, True)
    proj_v(NQ - 1, 0, NQ - 2)
    proj_v(NQ - 1, 1, NQ - 2)
    pv(NQ - 2, False)
    pv(NQ - 1, True)
    il.vpu(CFG["prep_after"], "end", [(1, functools.partial(gather, *e)) for e in upcoming], None)
    il.emit(CFG["delay"], CFG["lead"], CFG["period"])


def _wt_steps(part, w_v, wt):
    def step(mb, cb):
        n0 = part * M + 128 * cb
        tt = pltpu.bitcast(_halves(w_v[64 * mb:64 * mb + 64, n0:n0 + 128]).T, U32)
        for hl in range(4):
            r = (4 * cb + hl) * WPITCH
            wt[part, mb, r:r + 16, :] = tt[16 * hl:16 * hl + 16]

    return [functools.partial(step, mb, cb) for mb in range(8) for cb in range(8)]


def _bwo_steps(bwo_v, bwo_p):
    def step(cb, j):
        bwo_p[H * j:H * j + H, 128 * cb:128 * cb + 128] = bwo_v[cb, pl.ds(j, H, stride=DH // 2), :]

    return [functools.partial(step, cb, j) for cb in range(8) for j in range(DH // 2)]


def _b_project(il, bx_v, wt, part, row0, nrows, store):
    st = {}

    def rhs(cb, half):
        return _halves(jnp.concatenate(
            [jnp.concatenate([wt[part, mb, pl.ds(j, H, stride=WPITCH), :]
                              for j in (2 * cb, 2 * cb + 1)], axis=0)
             for mb in range(4 * half, 4 * half + 4)], axis=1))

    def first(cb, xx):
        st["y"] = _dot_nt(xx, rhs(cb, 0))
        return st["y"]

    def second(cb, r, xx):
        y = _dot_nt(xx, rhs(cb, 1))
        store(cb, r, st.pop("y") + y)
        return y

    for r in range(0, nrows, 256):
        rr = pl.ds(_half(row0 + r), 128)
        for cb in range(8):
            il.mxu(256, lambda rr=rr: bx_v[rr, 0:512], functools.partial(first, cb), 'p')
            il.mxu(256, lambda rr=rr: bx_v[rr, 512:1024], functools.partial(second, cb, r), 'p')


def _window(buf, cb, row, n):
    half = W // 2
    back = DIL * half
    out = [None] * W
    for w in range(half):
        x = buf[cb, pl.ds(row + (HALO - back - DIL * w), n + back), :]
        out[w], out[w + half] = x[back:], x[:n]
    return out


def _b_prob_steps(row0, nrows, qk_f, prob):
    G = CFG["G"]
    st = {}
    even = lax.broadcasted_iota(jnp.int32, (G, 128), 1) % 2 == 0

    def products(r0, cb, hold):
        q = hold(qk_f[cb, pl.ds(pl.multiple_of(row0 + (HALO + r0), 8), G), :])
        sums = st.get(r0)
        sums = [q * k if cb == 0 else sums[w] + q * k
                for w, k in enumerate(_window(qk_f, 8 + cb, row0 + r0, G))]
        st[r0] = [a + pltpu.roll(a, 64, 1) for a in sums] if cb == 7 else sums

    def finish(r0, hold):
        lg = []
        for w, a in enumerate(st.pop(r0)):
            a = a + jnp.where(even, pltpu.roll(a, 127, 1), pltpu.roll(a, 1, 1))
            if r0 < DIL * w:
                pos = row0 + r0 + lax.broadcasted_iota(jnp.int32, (G, 128), 0)
                a = jnp.where(pos >= DIL * w, a, NEG)
            lg.append(a)
        m = functools.reduce(jnp.maximum, lg)
        ps = [jnp.exp2(a - m) for a in lg]
        inv = _recip(functools.reduce(jnp.add, ps))
        for w in range(W):
            prob[pl.ds(pl.multiple_of(row0 + r0, G), G), 128 * w:128 * w + 128] = ps[w] * inv

    starts = list(range(0, nrows, G))
    fns = []
    for n in range(len(starts) + CFG["LAG"]):
        if n < len(starts):
            fns += [(1, functools.partial(products, starts[n], cb)) for cb in range(8)]
        if n >= CFG["LAG"]:
            fns.append((CFG['fw'], functools.partial(finish, starts[n - CFG["LAG"]])))
    return fns


def _b_mix_steps(row0, nrows, v_f, prob, o_s, dst0):
    half = W // 2
    back = DIL * half
    st = {}

    def step(r0, w, cb, hold):
        if cb == 0:
            r = pl.ds(pl.multiple_of(row0 + r0, 16), 16)
            st["p"] = [hold(prob[r, 128 * u:128 * u + 128]) for u in (w, w + half)]
        v = v_f[cb, pl.ds(row0 + (r0 + HALO - back - DIL * w), 16 + back), :]
        a = st["p"][0] * v[back:] + st["p"][1] * v[:16]
        st[cb] = a if w == 0 else st[cb] + a
        if w == half - 1:
            o_s[pl.ds(_half(dst0 + r0), 8), 128 * cb:128 * cb + 128] = _words(st[cb])

    return [(1, functools.partial(step, r0, w, cb))
            for r0 in range(0, nrows, 16) for w in range(half) for cb in range(8)]


def _zero_of(c):
    return pl.multiple_of((c >> 8) * 8, 8)


def _half(r):
    return r // 2 if isinstance(r, int) else pl.multiple_of(r >> 1, 8)


def _branch_b(bx_hbm, wqkv_hbm, bwo_hbm, out_v, start_other_copies,
              bx_v, wqkv_v, bwo_v, wt, bwo_p, qk_f, v_f, prob, o_a, o_b, w_sems, x_sems):
    R0, R1, R2 = CFG["R0"], CFG["R1"], CFG["R2"]
    bscale = (DH ** -0.5) * LOG2E
    w_copies = [
        pltpu.make_async_copy(wqkv_hbm.bitcast(U32).at[:, pl.ds(n * M, M)],
                              wqkv_v.at[:, pl.ds(n * M, M)], w_sems.at[n])
        for n in range(3)]
    w_copies += [
        pltpu.make_async_copy(bwo_hbm.bitcast(U32).at[:, pl.ds(128 * j, 128)], bwo_v.at[j],
                              w_sems.at[3 + j])
        for j in range(8)]

    def bx_copy(c):
        r = pl.ds(pl.multiple_of(c * (R0 // 2), R0 // 2), R0 // 2)
        return pltpu.make_async_copy(bx_hbm.bitcast(U32).at[r, :], bx_v.at[r, :], x_sems.at[c])

    w_copies[0].start()
    bx_copy(0).start()
    qk_f[8:16, 0:HALO, :] = jnp.zeros((8, HALO, 128), F32)
    v_f[:, 0:HALO, :] = jnp.zeros((8, HALO, 128), F32)
    prob[0:8, 0:128] = jnp.zeros((8, 128), F32)
    with _scope('w0'):
        w_copies[0].wait()
    for c in range(1, S // R0):
        bx_copy(c).start()
    for cp in w_copies[1:]:
        cp.start()
    for fn in _wt_steps(0, wqkv_v, wt):
        fn()

    def store_into(buf, cb0, row0, scale=None):
        def store(cb, r, y):
            buf[cb0 + cb, pl.ds(pl.multiple_of(row0 + (HALO + r), 8), 256), :] = (
                y if scale is None else y * scale)
        return store

    def qk_rows(n, carry):
        part, c = n // (S // R0), n % (S // R0)

        @pl.when(part == 0)
        def _():
            bx_copy(c).wait()

        @pl.when(n == S // R0)
        def _():
            with _scope('w1'):
                for cp in w_copies[1:]:
                    cp.wait()
            start_other_copies()
            for fn in (_wt_steps(1, wqkv_v, wt) + _wt_steps(2, wqkv_v, wt)
                       + _bwo_steps(bwo_v, bwo_p)):
                fn()

        il = _Interleaver(None)
        row0 = pl.multiple_of(c * R0, R0)
        _b_project(il, bx_v, wt, part, row0, R0,
                   store_into(qk_f, 8 * part, row0, jnp.where(part == 0, bscale, 1.0)))
        il.emit(0, 0, 256)
        return carry

    with _scope('L0'):
        lax.fori_loop(0, 2 * (S // R0), qk_rows, 0)

    def prob_rows(c, carry):
        il = _Interleaver(c < 0)
        row0 = pl.multiple_of(c * R1, R1)
        _b_project(il, bx_v, wt, 2, row0, R1, store_into(v_f, 0, row0))
        il.vpu("begin", "end", _b_prob_steps(row0, R1, qk_f, prob), _read_back(prob, _zero_of(c)))
        il.emit(0, CFG["blead"], CFG["bperiod"])
        return carry

    with _scope('L1'):
        lax.fori_loop(0, S // R1, prob_rows, 0)

    def out_rows(c, carry):
        il = _Interleaver(c < 0)
        st = {}

        def first(n0, oo):
            st["y"] = _dot(oo, _halves(bwo_p[0:256, n0:n0 + 128]))
            return st["y"]

        def second(n0, r, oo):
            y = _dot(oo, _halves(bwo_p[256:512, n0:n0 + 128]))
            out_v[r, M + n0:M + n0 + 128] = _words(st.pop("y") + y)
            return y

        for n, (src, dst) in enumerate(((o_a, o_b), (o_b, o_a))):
            row0 = pl.multiple_of((2 * c + n) * 256, 256)
            for n0 in range(0, M, 128):
                il.mxu(256, lambda src=src: src[0:128, 0:512], functools.partial(first, n0), n)
                il.mxu(256, lambda src=src: src[0:128, 512:1024],
                       functools.partial(second, n0, pl.ds(_half(row0), 128)), n)
            fns = _b_mix_steps(pl.multiple_of(jnp.minimum(row0 + 256, S - 256), 256), 256,
                               v_f, prob, dst, 0)
            fns.append((0, lambda hold, dst=dst: _fence(dst, _zero_of(c))))
            il.vpu(0 if n else "begin", "end" if n else 1, fns, _read_back(dst, _zero_of(c)))
        il.emit(CFG["bdelay"], CFG["blead"], CFG["bperiod"])
        return carry

    def first_mix(c, carry):
        row0 = pl.multiple_of(c * 64, 64)
        for _, fn in _b_mix_steps(row0, 64, v_f, prob, o_a, row0):
            fn(lambda x: x)
        return carry

    with _scope('m0'):
        lax.fori_loop(0, 256 // 64, first_mix, 0)
    with _scope('L2'):
        lax.fori_loop(0, S // 512, out_rows, 0)


def _branch_a(x_v, c_v, wq_v, wuk_v, wuv_v, wo_v, out_v, wo_copy, out_copy,
              wq2, wk2, wv2, q_s, k_s, v_s, s_a, s_b, p_a, p_b, p_c, ctx):
    R3 = CFG["R3"]
    for _, fn in _weight_steps(0, wq_v, wuk_v, wuv_v, wq2, wk2, wv2):
        fn()

    def head_pair(t, carry):
        with _scope('it'):
            _head_pair(t, x_v, c_v, wq_v, wuk_v, wuv_v, wq2, wk2, wv2, q_s, k_s, v_s,
                       (s_a, s_b), (p_a, p_b, p_c), ctx)
        return carry

    with _scope('LA'):
        lax.fori_loop(0, CFG["na"], head_pair, 0)
    wo_copy.wait()

    NS = CFG["NS"]

    def out_rows(n, carry):
        c, side = n // NS, n % NS
        w0 = pl.multiple_of(c * (R3 // 2), 128)
        for n0 in range(0, M // NS, 128):
            cols = pl.ds(pl.multiple_of(side * (M // NS) + n0, 128), 128)
            y = None
            for t in range(0, H // 2, 2):
                lhs = jnp.concatenate([ctx[pl.ds(w0 + u * (S // 2), R3 // 2), :]
                                       for u in (t, t + 1)], axis=1)
                part = _dot(_halves(lhs), _halves(wo_v[128 * t:128 * t + 256, cols]))
                y = part if y is None else y + part
            out_v[pl.ds(w0, R3 // 2), cols] = _words(y)
        out_copy(n).start()
        return carry

    with _scope('L4'):
        lax.fori_loop(0, NS * S // R3, out_rows, 0)
    with _scope('w3'):
        for n in range(NS * S // R3):
            out_copy(n).wait()


def _kernel(x_hbm, c_hbm, wq_hbm, wuk_hbm, wuv_hbm, wo_hbm, bx_hbm, wqkv_hbm, bwo_hbm,
            out_hbm, x_v, c_v, wq_v, wuk_v, wuv_v, wo_v, out_v, a_sems, o_sems):
    R0, R3 = CFG["R0"], CFG["R3"]
    vm = pltpu.VMEM
    a_copies = [
        pltpu.make_async_copy(src.bitcast(U32), dst, a_sems.at[n])
        for n, (src, dst) in enumerate((
            (wuk_hbm, wuk_v.at[pl.ds(0, DC * H // 2)]),
            (wuv_hbm, wuv_v.at[pl.ds(0, DC * H // 2)]),
            (wq_hbm, wq_v.at[pl.ds(0, M * H // 2)]),
            (c_hbm, c_v), (x_hbm, x_v), (wo_hbm, wo_v)))]

    def out_copy(r, cols, n):
        return pltpu.make_async_copy(out_v.at[r, cols], out_hbm.bitcast(U32).at[r, cols],
                                     o_sems.at[n])

    def a_out_copy(n):
        NS = CFG["NS"]
        r = pl.ds(pl.multiple_of(n // NS * (R3 // 2), R3 // 2), R3 // 2)
        return out_copy(r, pl.ds(pl.multiple_of(n % NS * (M // NS), 128), M // NS), 1 + n)

    def start_a_copies():
        for cp in a_copies:
            cp.start()

    if CFG["only"] == "a": start_a_copies()
    else: pl.run_scoped(
        functools.partial(_branch_b, bx_hbm, wqkv_hbm, bwo_hbm, out_v, start_a_copies),
        vm((S // 2, M), U32), vm((M // 2, 3 * M), U32), vm((8, M // 2, 128), U32),
        vm((3, 8, H * WPITCH, 128), U32), vm((M // 2, M), U32),
        vm((16, HALO + S, 128), F32), vm((8, HALO + S, 128), F32),
        vm((S, W * 128), F32), vm((128 + 8, M), U32), vm((128 + 8, M), U32),
        pltpu.SemaphoreType.DMA((11,)), pltpu.SemaphoreType.DMA((S // R0,)))
    b_out_copy = out_copy(pl.ds(0, S // 2), pl.ds(M, M), 0)
    b_out_copy.start()
    with _scope('w2'):
        for cp in a_copies[:-1]:
            cp.wait()
    if CFG["only"] == "b": a_copies[-1].wait()
    else: pl.run_scoped(
        functools.partial(_branch_a, x_v, c_v, wq_v, wuk_v, wuv_v, wo_v, out_v, a_copies[-1],
                          a_out_copy),
        vm((M // 2, 2 * D), U32), vm((D, DC), U32), vm((DC // 2, 2 * D), U32),
        vm((S // 2, 2 * D), U32), vm((D, S), U32), vm((S // 2, 2 * D), U32),
        vm((2 * BQ + 8, S), F32), vm((2 * BQ + 8, S), F32),
        vm((BQ + 8, S + 2 * D), U32), vm((BQ + 8, S + 2 * D), U32),
        vm((BQ + 8, S + 2 * D), U32), vm((H // 2 * S // 2, 2 * D), U32))
    b_out_copy.wait()


@jax.jit
def pallas_concat_heads__compressed_kv_cla__sliding_local_dilated__prompt_kernel(
    A_x: jax.Array,
    A_c_kv: jax.Array,
    A_w_q: jax.Array,
    A_w_uk: jax.Array,
    A_w_uv: jax.Array,
    A_w_o: jax.Array,
    B_x: jax.Array,
    B_wqkv: jax.Array,
    B_wo: jax.Array,
):
    vm = pltpu.VMEM
    scratch = [
        vm((S // 2, M), U32), vm((S // 2, DC), U32),
        vm((M * H // 2 + 8, D), U32), vm((DC * H // 2 + 8, D), U32),
        vm((DC * H // 2 + 8, D), U32), vm((H * D // 2, M), U32),
        vm((S // 2, 2 * M), U32),
        pltpu.SemaphoreType.DMA((6,)), pltpu.SemaphoreType.DMA((1 + CFG["NS"] * S // CFG["R3"],)),
    ]
    out = pl.pallas_call(
        _kernel,
        out_shape=jax.ShapeDtypeStruct((S, 2 * M), BF16),
        in_specs=[pl.BlockSpec(memory_space=pl.ANY)] * 9,
        out_specs=pl.BlockSpec(memory_space=pl.ANY),
        scratch_shapes=scratch,
        compiler_params=pltpu.CompilerParams(vmem_limit_bytes=124 * 1024 * 1024,
                                             flags=CFG["flags"]),
        name="fused_ab",
    )(
        A_x.reshape(S, M), A_c_kv.reshape(S, DC),
        A_w_q.reshape(M * H, D), A_w_uk.reshape(DC * H, D), A_w_uv.reshape(DC * H, D),
        A_w_o.reshape(H * D, M),
        B_x.reshape(S, M), B_wqkv, B_wo,
    )
    return out.reshape(1, S, 2 * M)
```

```python
import functools
import math

import jax
import jax.numpy as jnp
from jax import lax
import jax.experimental.pallas as pl
import jax.experimental.pallas.tpu as pltpu

CFG = dict(na=16, R0=256, R1=256, R2=256, fw=3, nextra=192, nshift=500, NS=1, bdelay=0, only=None, R3=256, ahead=256, prep_after=('qk', 7), spad=0, ppad=0, PN=2, late_v=0, btie=1, blead=300, delay=400, lead=200, period=32, UT=1, nout=3, PR=16,
           mincost=256, flags=None, bperiod=32, LAG=1, G=16, do_b=True, n0=None, scopes=False)

S = 2048
M = 1024
H = 32
D = 128
DC = 512
DH = 32
W = 8
DIL = 2
HALO = 16
BQ = 256
NQ = S // BQ
WPITCH = DH // 2 + 1
LOG2E = math.log2(math.e)
NEG = -1e9 * LOG2E

F32 = jnp.float32
BF16 = jnp.bfloat16
U32 = jnp.uint32
NT = (((1,), (1,)), ((), ()))


def _dot(a, b):
    return jnp.dot(a, b, preferred_element_type=F32)


def _dot_nt(a, b):
    return lax.dot_general(a, b, NT, preferred_element_type=F32)


def _words(x):
    return pltpu.bitcast(x.astype(BF16), U32)


def _halves(w):
    return pltpu.bitcast(w, BF16)


def _unpack_pair(w):
    lo = pltpu.bitcast(w << 16, F32)
    hi = pltpu.bitcast(w & jnp.uint32(0xFFFF0000), F32)
    return lo, hi


def _recip(x):
    r = pl.reciprocal(x, approx=True)
    return r * (2.0 - x * r)


import contextlib
def _scope(name):
    return jax.named_scope(name) if CFG["scopes"] else contextlib.nullcontext()


def _rows(r0, n):
    return slice(r0 // 2, (r0 + n) // 2)


class _Interleaver:
    def __init__(self, never):
        self.never = never
        self.steps = []
        self.side = []

    def mxu(self, rows, tiles, lhs, fn, name):
        self.steps.append((rows, tiles, lhs, fn, name))

    def vpu(self, after, before, fns, token, until=None, shift=0):
        self.side.append((after, before, fns, until, token, shift))

    def emit(self, delay=0, lead=0, period=32):
        busy, starts, slots = [0] * 4, [], []
        start, end = {}, {"begin": -delay}
        for rows, tiles, _, _, name in self.steps:
            units = sorted(range(4), key=lambda u: busy[u])[:tiles]
            t0 = busy[units[0]]
            starts.append(t0)
            start.setdefault(name, t0)
            for u in units:
                busy[u] += rows
            end[name] = max([end.get(name, 0)] + [busy[u] for u in units])
            slots += [(t, len(starts) - 1) for t in range(t0 + period, t0 + rows + 1, period)
                      if not slots or t > slots[-1][0]]
        start["end"] = max(busy)
        todo = []
        for after, before, fns, until, token, shift in self.side:
            hi = start[before]
            lo = min(end[after] + delay, hi)
            hi = max(hi - lead, lo)
            if until is not None:
                hi = min(hi, end[until] + delay)
            total, done = sum(w for w, _ in fns), 0
            for w, fn in fns:
                when = lo + (hi - lo) * (done + w / 2) / total + shift
                todo.append((when, len(todo), fn, token, None if shift else before))
                done += w
        todo.sort(key=lambda e: e[:2])
        results = []

        def hold(now):
            def apply(x, extra=0):
                past = [y for t, y in results if t <= now - CFG["ahead"] - extra]
                if not past:
                    return x
                return jnp.where(
                    self.never, jnp.concatenate([past[-1]] * (x.shape[0] // 8), axis=0), x)

            return apply

        k = 0
        for n, ((rows, _, lhs, fn, name), t0) in enumerate(zip(self.steps, starts)):
            assert all(e[4] != name for e in todo[k:])
            words = lhs()
            slabs = [words[r:r + 8] for r in range(0, rows // 2, 8)]
            for t in [t for t, step in slots if step == n]:
                tokens = []
                while k < len(todo) and todo[k][0] < t + period:
                    todo[k][2](hold(t))
                    if todo[k][3] is not None and todo[k][3] not in tokens:
                        tokens.append(todo[k][3])
                    k += 1
                u = (t - t0) // 16 - 1
                for token in [x for x in (token() for token in tokens) if x is not None]:
                    head = jnp.where(self.never, token, slabs[u][:, 0:128])
                    slabs[u] = (jnp.concatenate([head, slabs[u][:, 128:]], axis=1)
                                if words.shape[1] > 128 else head)
            y = fn(_halves(jnp.concatenate(slabs, axis=0)))
            results += [(t0 + r + 16, y[r:r + 8, 0:128]) for r in range(0, rows, 16)
                        if not results or t0 + r + 16 > results[-1][0]]
        for e in todo[k:]:
            e[2](hold(start["end"]))


def _read_back(buf, zero):
    return lambda: pltpu.bitcast(buf[pl.ds(zero, 8), 0:128], U32)


def _fence(buf, zero):
    buf[pl.ds(zero + (buf.shape[0] - 8), 8), 0:128] = jnp.zeros((8, 128), buf.dtype)


def _weight_steps(t, wq_v, wuk_v, wuv_v, wq2, wk2, wv2):
    PR = CFG["PR"]
    held = []

    def gather(src, r0):
        return src[pl.ds(t + r0 * (H // 2), PR, stride=H // 2), :]

    def k_step(r0):
        held.append(gather(wuk_v, r0))
        if (r0 + PR) % 128 == 0:
            lo, hi = _unpack_pair(jnp.concatenate(held, axis=0).T)
            held.clear()
            c = slice(r0 + PR - 128, r0 + PR)
            wk2[0:64, c] = _words(lo)
            wk2[64:128, c] = _words(hi)

    def plain_step(src, dst, r0):
        lo, hi = _unpack_pair(gather(src, r0))
        dst[_rows(r0, PR), 0:128] = _words(lo)
        dst[_rows(r0, PR), 128:256] = _words(hi)

    return ([(wuk_v, functools.partial(k_step, r)) for r in range(0, DC, PR)]
            + [(wq_v, functools.partial(plain_step, wq_v, wq2, r)) for r in range(0, M, PR)]
            + [(wuv_v, functools.partial(plain_step, wuv_v, wv2, r)) for r in range(0, DC, PR)])


def _head_pair(t, x_v, c_v, wq_v, wuk_v, wuv_v, wq2, wk2, wv2, q_s, k_s, v_s, s_s, p_s, ctx):
    UT = CFG["UT"]
    qscale = (D ** -0.5) * LOG2E
    row = lax.broadcasted_iota(jnp.int32, (128, 128), 0)
    col = lax.broadcasted_iota(jnp.int32, (128, 128), 1)
    tri = col <= row
    zero = pl.multiple_of((t >> 8) * 8, 8)
    ctx_row = pl.multiple_of(t * (S // 2), S // 2)
    st = {}
    il = _Interleaver(t < 0)
    upcoming = _weight_steps(jnp.minimum(t + 1, H // 2 - 1), wq_v, wuk_v, wuv_v, wq2, wk2, wv2)

    def proj_k(i):
        def step(j, w):
            y = _dot_nt(w, _halves(c_v[_rows(128 * j, 128), :]))
            k_s[:, 128 * j:128 * j + 128] = _words(y)
            return y

        for j in range(2 * i, 2 * i + 2):
            il.mxu(256, 4, lambda: wk2[...], functools.partial(step, j), ("proj", i))

    def proj_v(i, h, n):
        def step(cc):
            y = _dot(cc, _halves(wv2[:, 128 * h:128 * h + 128]))
            v_s[_rows(i * BQ, BQ), 128 * h:128 * h + 128] = _words(y)
            return y

        il.mxu(256, 4, lambda: c_v[_rows(i * BQ, BQ), :], step, ("v", i))

    def proj_q(i, h):
        r, c = _rows(i * BQ, BQ), slice(128 * h, 128 * h + 128)

        def first(xx):
            st["q"] = _dot(xx, _halves(wq2[0:256, c]))
            return st["q"]

        def second(xx):
            y = _dot(xx, _halves(wq2[256:512, c]))
            q_s[r, c] = _words((st.pop("q") + y) * qscale)
            return y

        il.mxu(256, 4, lambda: x_v[r, 0:512], first, ("proj", i))
        il.mxu(256, 4, lambda: x_v[r, 512:1024], second, ("proj", i))

    def pieces(i):
        n = 2 * i
        body = [(h, j, 4, 0, BQ) for h in range(2) for j in range(0, n - 3, 4)]
        if n % 4:
            body += [(h, n - 2, 2, 0, BQ) for h in range(2)]
        diag = ([(h, n, 1, 0, BQ) for h in range(2)]
                + [(h, n + 1, 1, 128, 128) for h in range(2)])
        return body, diag

    def qk(i, diag_first):
        left = {}

        def piece(h, j, n, a0, nr, q):
            s = _dot(q, _halves(k_s[64 * h:64 * h + 64, 128 * j:128 * (j + n)]))
            for a in range(a0, a0 + nr, 64):
                m = st.get(("m", i, h, a))
                for u in range(n):
                    tile = s[a - a0:a - a0 + 64, 128 * u:128 * u + 128]
                    if j + u == 2 * i + a // 128:
                        tile = jnp.where(tri[a % 128:a % 128 + 64], tile, NEG)
                    s_s[i % 2][BQ * h + a:BQ * h + a + 64,
                               128 * (j + u):128 * (j + u + 1)] = tile
                    m = tile if m is None else jnp.maximum(m, tile)
                left[h, a] -= n
                if left[h, a] == 0:
                    m = jnp.broadcast_to(jnp.max(m, axis=-1, keepdims=True), (64, 128))
                st["m", i, h, a] = m
            if not any(left[h, a] for a in range(0, BQ, 64)):
                _fence(s_s[i % 2], zero)
            return s

        body, diag = pieces(i)
        for h, j, n, a0, nr in (diag + body[::-1] if diag_first else body[::-1] + diag):
            for a in range(a0, a0 + nr, 64):
                left[h, a] = left.get((h, a), 0) + n
            il.mxu(nr, n,
                   lambda h=h, a0=a0, nr=nr: q_s[_rows(i * BQ + a0, nr), 128 * h:128 * h + 128],
                   functools.partial(piece, h, j, n, a0, nr), ("qk", i))

    def softmax(i, before, until):
        sb, pb = s_s[i % 2], p_s[i % 3]

        def unit(h, r0, j0, j1, last, hold):
            a = r0 // 64 * 64
            m = hold(st["m", i, h, a][r0 - a:r0 - a + 16])
            l = st.pop(("l", i), None)
            r = BQ * h + r0
            for j in range(j0, j1):
                p = jnp.exp2(sb[r:r + 16, 128 * j:128 * j + 128] - m)
                l = p if l is None else l + p
                pb[_rows(r, 16), 128 * j:128 * j + 128] = _words(p)
            if last:
                pb[r0:r0 + 16, S + 128 * h:S + 128 * h + 128] = pltpu.bitcast(l, U32)
                st["sum", i, h, r0] = l
                if r0 + 16 == BQ and h == 0:
                    _fence(pb, zero)
            else:
                st["l", i] = l

        def normalizer(h, r0, hold):
            l = hold(st.pop(("sum", i, h, r0)), CFG["nextra"])
            st["inv", i, h, r0] = st["last", i] = jnp.broadcast_to(
                _recip(jnp.sum(l, axis=-1, keepdims=True)), (16, 128))

        fns, norms = [], []
        for h in (1, 0):
            for r0 in range(0, BQ, 16):
                n = 2 * i + 1 + r0 // 128
                norms += [(n, lambda hold: None), (0, functools.partial(normalizer, h, r0))]
                for j0 in range(0, n, UT):
                    j1 = min(j0 + UT, n)
                    fns.append((j1 - j0, functools.partial(unit, h, r0, j0, j1, j1 == n)))
        il.vpu(("qk", i), before, fns, _read_back(pb, zero + BQ // 2), until)
        il.vpu(("qk", i), before, norms,
               lambda: pltpu.bitcast(st.pop(("last", i))[8:], U32) if ("last", i) in st else None,
               until, CFG["nshift"])

    def pv(i, diag_first):
        left = {}

        def probs(h, j, n, a0, nr):
            return p_s[i % 3][_rows(BQ * h + a0, nr), 128 * j:128 * (j + n)]

        def piece(h, j, n, a0, nr, p):
            o = _dot(p, _halves(v_s[_rows(128 * j, 128 * n), 128 * h:128 * h + 128]))
            for a in range(a0, a0 + nr, 64):
                part = o[a - a0:a - a0 + 64]
                prev = st.pop(("o", h, a), None)
                part = part if prev is None else prev + part
                left[h, a] -= n
                if left[h, a] == 0:
                    ctx[pl.ds(ctx_row + (i * BQ + a) // 2, 32), 128 * h:128 * h + 128] = _words(
                        part * jnp.concatenate(
                            [st.pop(("inv", i, h, r0)) for r0 in range(a, a + 64, 16)], axis=0))
                else:
                    st["o", h, a] = part
            return o

        body, diag = pieces(i)
        for h, j, n, a0, nr in (diag + body[::-1] if diag_first else body + diag):
            for a in range(a0, a0 + nr, 64):
                left[h, a] = left.get((h, a), 0) + n
            il.mxu(nr, n, functools.partial(probs, h, j, n, a0, nr),
                   functools.partial(piece, h, j, n, a0, nr), ("pv", i))
        if i < NQ - 1:
            il.vpu(("pv", i), "end", [(1, lambda hold: None)], _read_back(ctx, ctx_row + zero),
                   until=("pv", i))

    def gather(src, fn, hold):
        src[src.shape[0] - 8:, :] = pltpu.bitcast(hold(jnp.zeros((8, 128), F32)), U32)
        fn()

    for i in range(2):
        proj_q(i, 0)
        proj_k(i)
        proj_q(i, 1)
    proj_v(0, 0, None)
    proj_v(0, 1, None)
    qk(0, True)
    softmax(0, ("v", 1), None)
    for i in range(1, NQ - 1):
        qk(i, True)
        softmax(i, ("v", i + 1), ("qk", i + 1))
        proj_k(i + 1)
        proj_q(i + 1, 0)
        proj_q(i + 1, 1)
        proj_v(i, 0, i - 1)
        proj_v(i, 1, i - 1)
        if i < NQ - 2:
            pv(i - 1, False)
    qk(NQ - 1, False)
    softmax(NQ - 1, ("pv", NQ - 1), None)
    pv(NQ - 3, True)
    proj_v(NQ - 1, 0, NQ - 2)
    proj_v(NQ - 1, 1, NQ - 2)
    pv(NQ - 2, False)
    pv(NQ - 1, True)
    il.vpu(CFG["prep_after"], "end", [(1, functools.partial(gather, *e)) for e in upcoming], None)
    il.emit(CFG["delay"], CFG["lead"], CFG["period"])


def _wt_steps(part, w_v, wt):
    def step(mb, cb):
        n0 = part * M + 128 * cb
        tt = pltpu.bitcast(_halves(w_v[64 * mb:64 * mb + 64, n0:n0 + 128]).T, U32)
        for hl in range(4):
            r = (4 * cb + hl) * WPITCH
            wt[part, mb, r:r + 16, :] = tt[16 * hl:16 * hl + 16]

    return [functools.partial(step, mb, cb) for mb in range(8) for cb in range(8)]


def _bwo_steps(bwo_v, bwo_p):
    def step(cb, j):
        bwo_p[H * j:H * j + H, 128 * cb:128 * cb + 128] = bwo_v[cb, pl.ds(j, H, stride=DH // 2), :]

    return [functools.partial(step, cb, j) for cb in range(8) for j in range(DH // 2)]


def _b_project(il, bx_v, wt, part, row0, nrows, store):
    st = {}

    def rhs(cb, half):
        return _halves(jnp.concatenate(
            [jnp.concatenate([wt[part, mb, pl.ds(j, H, stride=WPITCH), :]
                              for j in (2 * cb, 2 * cb + 1)], axis=0)
             for mb in range(4 * half, 4 * half + 4)], axis=1))

    def first(cb, xx):
        st["y"] = _dot_nt(xx, rhs(cb, 0))
        return st["y"]

    def second(cb, r, xx):
        y = _dot_nt(xx, rhs(cb, 1))
        store(cb, r, st.pop("y") + y)
        return y

    for r in range(0, nrows, 256):
        rr = pl.ds(_half(row0 + r), 128)
        for cb in range(8):
            il.mxu(256, 4, lambda rr=rr: bx_v[rr, 0:512], functools.partial(first, cb), 'p')
            il.mxu(256, 4, lambda rr=rr: bx_v[rr, 512:1024], functools.partial(second, cb, r), 'p')


def _window(buf, cb, row, n):
    half = W // 2
    back = DIL * half
    out = [None] * W
    for w in range(half):
        x = buf[cb, pl.ds(row + (HALO - back - DIL * w), n + back), :]
        out[w], out[w + half] = x[back:], x[:n]
    return out


def _b_prob_steps(row0, nrows, qk_f, prob):
    G = CFG["G"]
    st = {}
    even = lax.broadcasted_iota(jnp.int32, (G, 128), 1) % 2 == 0

    def products(r0, cb, hold):
        q = hold(qk_f[cb, pl.ds(pl.multiple_of(row0 + (HALO + r0), 8), G), :])
        sums = st.get(r0)
        sums = [q * k if cb == 0 else sums[w] + q * k
                for w, k in enumerate(_window(qk_f, 8 + cb, row0 + r0, G))]
        st[r0] = [a + pltpu.roll(a, 64, 1) for a in sums] if cb == 7 else sums

    def finish(r0, hold):
        lg = []
        for w, a in enumerate(st.pop(r0)):
            a = a + jnp.where(even, pltpu.roll(a, 127, 1), pltpu.roll(a, 1, 1))
            if r0 < DIL * w:
                pos = row0 + r0 + lax.broadcasted_iota(jnp.int32, (G, 128), 0)
                a = jnp.where(pos >= DIL * w, a, NEG)
            lg.append(a)
        m = functools.reduce(jnp.maximum, lg)
        ps = [jnp.exp2(a - m) for a in lg]
        inv = _recip(functools.reduce(jnp.add, ps))
        for w in range(W):
            prob[pl.ds(pl.multiple_of(row0 + r0, G), G), 128 * w:128 * w + 128] = ps[w] * inv

    starts = list(range(0, nrows, G))
    fns = []
    for n in range(len(starts) + CFG["LAG"]):
        if n < len(starts):
            fns += [(1, functools.partial(products, starts[n], cb)) for cb in range(8)]
        if n >= CFG["LAG"]:
            fns.append((CFG['fw'], functools.partial(finish, starts[n - CFG["LAG"]])))
    return fns


def _b_mix_steps(row0, nrows, v_f, prob, o_s, dst0):
    half = W // 2
    back = DIL * half
    st = {}

    def step(r0, w, cb, hold):
        if cb == 0:
            r = pl.ds(pl.multiple_of(row0 + r0, 16), 16)
            st["p"] = [hold(prob[r, 128 * u:128 * u + 128]) for u in (w, w + half)]
        v = v_f[cb, pl.ds(row0 + (r0 + HALO - back - DIL * w), 16 + back), :]
        a = st["p"][0] * v[back:] + st["p"][1] * v[:16]
        st[cb] = a if w == 0 else st[cb] + a
        if w == half - 1:
            o_s[pl.ds(_half(dst0 + r0), 8), 128 * cb:128 * cb + 128] = _words(st[cb])

    return [(1, functools.partial(step, r0, w, cb))
            for r0 in range(0, nrows, 16) for w in range(half) for cb in range(8)]


def _zero_of(c):
    return pl.multiple_of((c >> 8) * 8, 8)


def _half(r):
    return r // 2 if isinstance(r, int) else pl.multiple_of(r >> 1, 8)


def _branch_b(bx_hbm, wqkv_hbm, bwo_hbm, out_v, start_other_copies,
              bx_v, wqkv_v, bwo_v, wt, bwo_p, qk_f, v_f, prob, o_a, o_b, w_sems, x_sems):
    R0, R1, R2 = CFG["R0"], CFG["R1"], CFG["R2"]
    bscale = (DH ** -0.5) * LOG2E
    w_copies = [
        pltpu.make_async_copy(wqkv_hbm.bitcast(U32).at[:, pl.ds(n * M, M)],
                              wqkv_v.at[:, pl.ds(n * M, M)], w_sems.at[n])
        for n in range(3)]
    w_copies += [
        pltpu.make_async_copy(bwo_hbm.bitcast(U32).at[:, pl.ds(128 * j, 128)], bwo_v.at[j],
                              w_sems.at[3 + j])
        for j in range(8)]

    def bx_copy(c):
        r = pl.ds(pl.multiple_of(c * (R0 // 2), R0 // 2), R0 // 2)
        return pltpu.make_async_copy(bx_hbm.bitcast(U32).at[r, :], bx_v.at[r, :], x_sems.at[c])

    w_copies[0].start()
    bx_copy(0).start()
    qk_f[8:16, 0:HALO, :] = jnp.zeros((8, HALO, 128), F32)
    v_f[:, 0:HALO, :] = jnp.zeros((8, HALO, 128), F32)
    prob[0:8, 0:128] = jnp.zeros((8, 128), F32)
    with _scope('w0'):
        w_copies[0].wait()
    for c in range(1, S // R0):
        bx_copy(c).start()
    for cp in w_copies[1:]:
        cp.start()
    for fn in _wt_steps(0, wqkv_v, wt):
        fn()

    def store_into(buf, cb0, row0, scale=None):
        def store(cb, r, y):
            buf[cb0 + cb, pl.ds(pl.multiple_of(row0 + (HALO + r), 8), 256), :] = (
                y if scale is None else y * scale)
        return store

    def qk_rows(n, carry):
        part, c = n // (S // R0), n % (S // R0)

        @pl.when(part == 0)
        def _():
            bx_copy(c).wait()

        @pl.when(n == S // R0)
        def _():
            with _scope('w1'):
                for cp in w_copies[1:]:
                    cp.wait()
            start_other_copies()
            for fn in (_wt_steps(1, wqkv_v, wt) + _wt_steps(2, wqkv_v, wt)
                       + _bwo_steps(bwo_v, bwo_p)):
                fn()

        il = _Interleaver(None)
        row0 = pl.multiple_of(c * R0, R0)
        _b_project(il, bx_v, wt, part, row0, R0,
                   store_into(qk_f, 8 * part, row0, jnp.where(part == 0, bscale, 1.0)))
        il.emit()
        return carry

    with _scope('L0'):
        lax.fori_loop(0, 2 * (S // R0), qk_rows, 0)

    def prob_rows(c, carry):
        il = _Interleaver(c < 0)
        row0 = pl.multiple_of(c * R1, R1)
        _b_project(il, bx_v, wt, 2, row0, R1, store_into(v_f, 0, row0))
        il.vpu("begin", "end", _b_prob_steps(row0, R1, qk_f, prob), _read_back(prob, _zero_of(c)))
        il.emit(0, CFG["blead"], CFG["bperiod"])
        return carry

    with _scope('L1'):
        lax.fori_loop(0, S // R1, prob_rows, 0)

    def out_rows(c, carry):
        il = _Interleaver(c < 0)
        st = {}

        def first(n0, oo):
            st["y"] = _dot(oo, _halves(bwo_p[0:256, n0:n0 + 128]))
            return st["y"]

        def second(n0, r, oo):
            y = _dot(oo, _halves(bwo_p[256:512, n0:n0 + 128]))
            out_v[r, M + n0:M + n0 + 128] = _words(st.pop("y") + y)
            return y

        for n, (src, dst) in enumerate(((o_a, o_b), (o_b, o_a))):
            row0 = pl.multiple_of((2 * c + n) * 256, 256)
            for n0 in range(0, M, 128):
                il.mxu(256, 4, lambda src=src: src[0:128, 0:512], functools.partial(first, n0), n)
                il.mxu(256, 4, lambda src=src: src[0:128, 512:1024],
                       functools.partial(second, n0, pl.ds(_half(row0), 128)), n)
            fns = _b_mix_steps(pl.multiple_of(jnp.minimum(row0 + 256, S - 256), 256), 256,
                               v_f, prob, dst, 0)
            fns.append((0, lambda hold, dst=dst: _fence(dst, _zero_of(c))))
            il.vpu(0 if n else "begin", "end" if n else 1, fns, _read_back(dst, _zero_of(c)))
        il.emit(CFG["bdelay"], CFG["blead"], CFG["bperiod"])
        return carry

    def first_mix(c, carry):
        row0 = pl.multiple_of(c * 64, 64)
        for _, fn in _b_mix_steps(row0, 64, v_f, prob, o_a, row0):
            fn(lambda x: x)
        return carry

    with _scope('m0'):
        lax.fori_loop(0, 256 // 64, first_mix, 0)
    with _scope('L2'):
        lax.fori_loop(0, S // 512, out_rows, 0)


def _branch_a(x_v, c_v, wq_v, wuk_v, wuv_v, wo_v, out_v, wo_copy, out_copy,
              wq2, wk2, wv2, q_s, k_s, v_s, s_a, s_b, p_a, p_b, p_c, ctx):
    R3 = CFG["R3"]
    for _, fn in _weight_steps(0, wq_v, wuk_v, wuv_v, wq2, wk2, wv2):
        fn()

    def head_pair(t, carry):
        with _scope('it'):
            _head_pair(t, x_v, c_v, wq_v, wuk_v, wuv_v, wq2, wk2, wv2, q_s, k_s, v_s,
                       (s_a, s_b), (p_a, p_b, p_c), ctx)
        return carry

    with _scope('LA'):
        lax.fori_loop(0, CFG["na"], head_pair, 0)
    wo_copy.wait()

    NS = CFG["NS"]

    def out_rows(n, carry):
        c, side = n // NS, n % NS
        w0 = pl.multiple_of(c * (R3 // 2), 128)
        for n0 in range(0, M // NS, 128):
            cols = pl.ds(pl.multiple_of(side * (M // NS) + n0, 128), 128)
            y = None
            for t in range(0, H // 2, 2):
                lhs = jnp.concatenate([ctx[pl.ds(w0 + u * (S // 2), R3 // 2), :]
                                       for u in (t, t + 1)], axis=1)
                part = _dot(_halves(lhs), _halves(wo_v[128 * t:128 * t + 256, cols]))
                y = part if y is None else y + part
            out_v[pl.ds(w0, R3 // 2), cols] = _words(y)
        out_copy(n).start()
        return carry

    with _scope('L4'):
        lax.fori_loop(0, NS * S // R3, out_rows, 0)
    with _scope('w3'):
        for n in range(NS * S // R3):
            out_copy(n).wait()


def _kernel(x_hbm, c_hbm, wq_hbm, wuk_hbm, wuv_hbm, wo_hbm, bx_hbm, wqkv_hbm, bwo_hbm,
            out_hbm, x_v, c_v, wq_v, wuk_v, wuv_v, wo_v, out_v, a_sems, o_sems):
    R0, R3 = CFG["R0"], CFG["R3"]
    vm = pltpu.VMEM
    a_copies = [
        pltpu.make_async_copy(src.bitcast(U32), dst, a_sems.at[n])
        for n, (src, dst) in enumerate((
            (wuk_hbm, wuk_v.at[pl.ds(0, DC * H // 2)]),
            (wuv_hbm, wuv_v.at[pl.ds(0, DC * H // 2)]),
            (wq_hbm, wq_v.at[pl.ds(0, M * H // 2)]),
            (c_hbm, c_v), (x_hbm, x_v), (wo_hbm, wo_v)))]

    def out_copy(r, cols, n):
        return pltpu.make_async_copy(out_v.at[r, cols], out_hbm.bitcast(U32).at[r, cols],
                                     o_sems.at[n])

    def a_out_copy(n):
        NS = CFG["NS"]
        r = pl.ds(pl.multiple_of(n // NS * (R3 // 2), R3 // 2), R3 // 2)
        return out_copy(r, pl.ds(pl.multiple_of(n % NS * (M // NS), 128), M // NS), 1 + n)

    def start_a_copies():
        for cp in a_copies:
            cp.start()

    if CFG["only"] == "a": start_a_copies()
    else: pl.run_scoped(
        functools.partial(_branch_b, bx_hbm, wqkv_hbm, bwo_hbm, out_v, start_a_copies),
        vm((S // 2, M), U32), vm((M // 2, 3 * M), U32), vm((8, M // 2, 128), U32),
        vm((3, 8, H * WPITCH, 128), U32), vm((M // 2, M), U32),
        vm((16, HALO + S, 128), F32), vm((8, HALO + S, 128), F32),
        vm((S, W * 128), F32), vm((128 + 8, M), U32), vm((128 + 8, M), U32),
        pltpu.SemaphoreType.DMA((11,)), pltpu.SemaphoreType.DMA((S // R0,)))
    b_out_copy = out_copy(pl.ds(0, S // 2), pl.ds(M, M), 0)
    b_out_copy.start()
    with _scope('w2'):
        for cp in a_copies[:-1]:
            cp.wait()
    if CFG["only"] == "b": a_copies[-1].wait()
    else: pl.run_scoped(
        functools.partial(_branch_a, x_v, c_v, wq_v, wuk_v, wuv_v, wo_v, out_v, a_copies[-1],
                          a_out_copy),
        vm((M // 2, 2 * D), U32), vm((D, DC), U32), vm((DC // 2, 2 * D), U32),
        vm((S // 2, 2 * D), U32), vm((D, S), U32), vm((S // 2, 2 * D), U32),
        vm((2 * BQ + 8, S), F32), vm((2 * BQ + 8, S), F32),
        vm((BQ + 8, S + 2 * D), U32), vm((BQ + 8, S + 2 * D), U32),
        vm((BQ + 8, S + 2 * D), U32), vm((H // 2 * S // 2, 2 * D), U32))
    b_out_copy.wait()


@jax.jit
def pallas_concat_heads__compressed_kv_cla__sliding_local_dilated__prompt_kernel(
    A_x: jax.Array,
    A_c_kv: jax.Array,
    A_w_q: jax.Array,
    A_w_uk: jax.Array,
    A_w_uv: jax.Array,
    A_w_o: jax.Array,
    B_x: jax.Array,
    B_wqkv: jax.Array,
    B_wo: jax.Array,
):
    vm = pltpu.VMEM
    scratch = [
        vm((S // 2, M), U32), vm((S // 2, DC), U32),
        vm((M * H // 2 + 8, D), U32), vm((DC * H // 2 + 8, D), U32),
        vm((DC * H // 2 + 8, D), U32), vm((H * D // 2, M), U32),
        vm((S // 2, 2 * M), U32),
        pltpu.SemaphoreType.DMA((6,)), pltpu.SemaphoreType.DMA((1 + CFG["NS"] * S // CFG["R3"],)),
    ]
    out = pl.pallas_call(
        _kernel,
        out_shape=jax.ShapeDtypeStruct((S, 2 * M), BF16),
        in_specs=[pl.BlockSpec(memory_space=pl.ANY)] * 9,
        out_specs=pl.BlockSpec(memory_space=pl.ANY),
        scratch_shapes=scratch,
        compiler_params=pltpu.CompilerParams(vmem_limit_bytes=124 * 1024 * 1024,
                                             flags=CFG["flags"]),
        name="fused_ab",
    )(
        A_x.reshape(S, M), A_c_kv.reshape(S, DC),
        A_w_q.reshape(M * H, D), A_w_uk.reshape(DC * H, D), A_w_uv.reshape(DC * H, D),
        A_w_o.reshape(H * D, M),
        B_x.reshape(S, M), B_wqkv, B_wo,
    )
    return out.reshape(1, S, 2 * M)
```

```python
import functools
import math

import jax
import jax.numpy as jnp
from jax import lax
import jax.experimental.pallas as pl
import jax.experimental.pallas.tpu as pltpu

CFG = dict(na=16, R0=256, R1=256, R2=256, fw=3, pad=1, dmam=0, aprio=0, wunroll=1, astart=-1, nextra=192, nshift=500, NS=1, bdelay=0, only=None, R3=256, ahead=256, prep_after=('qk', 7), spad=0, ppad=0, PN=2, late_v=0, btie=1, blead=300, delay=400, lead=200, period=32, UT=1, nout=3, PR=16,
           mincost=256, flags=None, bperiod=32, LAG=1, G=16, do_b=True, n0=None, scopes=False)

S = 2048
M = 1024
H = 32
D = 128
DC = 512
DH = 32
W = 8
DIL = 2
HALO = 16
BQ = 256
NQ = S // BQ
WPITCH = DH // 2 + 1
LOG2E = math.log2(math.e)
NEG = -1e9 * LOG2E

F32 = jnp.float32
BF16 = jnp.bfloat16
U32 = jnp.uint32
NT = (((1,), (1,)), ((), ()))


def _dot(a, b):
    return jnp.dot(a, b, preferred_element_type=F32)


def _dot_nt(a, b):
    return lax.dot_general(a, b, NT, preferred_element_type=F32)


def _words(x):
    return pltpu.bitcast(x.astype(BF16), U32)


def _halves(w):
    return pltpu.bitcast(w, BF16)


def _unpack_pair(w):
    lo = pltpu.bitcast(w << 16, F32)
    hi = pltpu.bitcast(w & jnp.uint32(0xFFFF0000), F32)
    return lo, hi


def _recip(x):
    r = pl.reciprocal(x, approx=True)
    return r * (2.0 - x * r)


import contextlib
def _scope(name):
    return jax.named_scope(name) if CFG["scopes"] else contextlib.nullcontext()


def _rows(r0, n):
    return slice(r0 // 2, (r0 + n) // 2)


def _aligned(x, n):
    return x if isinstance(x, int) else pl.multiple_of(x, n)


def _half(r):
    return r // 2 if isinstance(r, int) else pl.multiple_of(r >> 1, 8)


def _zero_of(c):
    return pl.multiple_of((c >> 8) * 8, 8)


class _Interleaver:
    def __init__(self, never):
        self.never = never
        self.steps = []
        self.side = []

    def mxu(self, rows, tiles, lhs, fn, name):
        self.steps.append((rows, tiles, lhs, fn, name))

    def vpu(self, after, before, fns, token, until=None, shift=0):
        self.side.append((after, before, fns, until, token, shift))

    def emit(self, delay=0, lead=0, period=32):
        busy, starts, slots = [0] * 4, [], []
        start, end = {}, {"begin": -delay}
        for rows, tiles, _, _, name in self.steps:
            units = sorted(range(4), key=lambda u: busy[u])[:tiles]
            t0 = busy[units[0]]
            starts.append(t0)
            start.setdefault(name, t0)
            for u in units:
                busy[u] += rows
            end[name] = max([end.get(name, 0)] + [busy[u] for u in units])
            slots += [(t, len(starts) - 1) for t in range(t0 + period, t0 + rows + 1, period)
                      if not slots or t > slots[-1][0]]
        start["end"] = max(busy)
        todo = []
        for after, before, fns, until, token, shift in self.side:
            hi = start[before]
            lo = min(end[after] + delay, hi)
            hi = max(hi - lead, lo)
            if until is not None:
                hi = min(hi, end[until] + delay)
            total, done = sum(w for w, _ in fns), 0
            for w, fn in fns:
                when = lo + (hi - lo) * (done + w / 2) / total + shift
                todo.append((when, len(todo), fn, token, None if shift else before))
                done += w
        todo.sort(key=lambda e: e[:2])
        results = []

        def hold(now):
            def apply(x, extra=0):
                past = [y for t, y in results if t <= now - CFG["ahead"] - extra]
                if not past:
                    return x
                return jnp.where(
                    self.never, jnp.concatenate([past[-1]] * (x.shape[0] // 8), axis=0), x)

            return apply

        k = 0
        for n, ((rows, _, lhs, fn, name), t0) in enumerate(zip(self.steps, starts)):
            assert all(e[4] != name for e in todo[k:])
            words = lhs()
            slabs = [words[r:r + 8] for r in range(0, rows // 2, 8)]
            for t in [t for t, step in slots if step == n]:
                tokens = []
                while k < len(todo) and todo[k][0] < t + period:
                    todo[k][2](hold(t))
                    if todo[k][3] is not None and todo[k][3] not in tokens:
                        tokens.append(todo[k][3])
                    k += 1
                u = (t - t0) // 16 - 1
                for token in [x for x in (token() for token in tokens) if x is not None]:
                    head = jnp.where(self.never, token, slabs[u][:, 0:128])
                    slabs[u] = (jnp.concatenate([head, slabs[u][:, 128:]], axis=1)
                                if words.shape[1] > 128 else head)
            y = fn(_halves(jnp.concatenate(slabs, axis=0)))
            results += [(t0 + r + 16, y[r:r + 8, 0:128]) for r in range(0, rows, 16)
                        if not results or t0 + r + 16 > results[-1][0]]
        for e in todo[k:]:
            e[2](hold(start["end"]))


def _read_back(buf, zero):
    return lambda: pltpu.bitcast(buf[pl.ds(zero, 8), 0:128], U32)


def _fence(buf, zero):
    buf[pl.ds(zero + (buf.shape[0] - 8), 8), 0:128] = jnp.zeros((8, 128), buf.dtype)


def _regroup_steps(part, nparts, raw, by_head):
    def step(src, dst, r, hold):
        pitch = dst.shape[1] // (H // 2)
        r0 = _aligned(r * H, H)
        src[src.shape[0] - 8:, :] = pltpu.bitcast(hold(jnp.zeros((8, 128), F32)), U32)
        even, odd = src[pl.ds(r0, H // 2), :], src[pl.ds(r0 + H // 2, H // 2), :]
        o = pl.ds(r, H // 2, stride=pitch)
        dst[0, o, :] = (even & jnp.uint32(0xFFFF)) | (odd << 16)
        dst[1, o, :] = (even >> 16) | (odd & jnp.uint32(0xFFFF0000))

    fns = []
    for src, dst in zip(raw, by_head):
        n = (src.shape[0] - 8) // H // nparts
        fns += [(1, functools.partial(step, src, dst, part * n + r)) for r in range(n)]
    return fns


def _head_pair(t, x_v, c_v, wq_h, wk_h, wv_h, q_s, k_s, v_s, s_s, p_s, ctx):
    UT = CFG["UT"]
    qscale = (D ** -0.5) * LOG2E
    row = lax.broadcasted_iota(jnp.int32, (128, 128), 0)
    col = lax.broadcasted_iota(jnp.int32, (128, 128), 1)
    tri = col <= row
    zero = pl.multiple_of((t >> 8) * 8, 8)
    ctx_row = pl.multiple_of(t * (S // 2), S // 2)
    st = {}
    il = _Interleaver(t < 0)

    def weights(ref, h, r0):
        pitch = ref.shape[1] // (H // 2)
        return _halves(ref[h, pl.ds(t * pitch + r0, 256), :])

    def proj_kv(w, dst, name, i):
        def step(h, cc):
            y = _dot(cc, weights(w, h, 0))
            dst[_rows(i * BQ, BQ), 128 * h:128 * h + 128] = _words(y)
            return y

        for h in range(2):
            il.mxu(256, 4, lambda: c_v[_rows(i * BQ, BQ), :], functools.partial(step, h),
                   (name, i))

    proj_k = functools.partial(proj_kv, wk_h, k_s, "k")
    proj_v = functools.partial(proj_kv, wv_h, v_s, "v")

    def proj_q(i, h):
        r, c = _rows(i * BQ, BQ), slice(128 * h, 128 * h + 128)

        def first(xx):
            st["q"] = _dot(xx, weights(wq_h, h, 0))
            return st["q"]

        def second(xx):
            y = _dot(xx, weights(wq_h, h, 256))
            q_s[r, c] = _words((st.pop("q") + y) * qscale)
            return y

        il.mxu(256, 4, lambda: x_v[r, 0:512], first, ("proj", i))
        il.mxu(256, 4, lambda: x_v[r, 512:1024], second, ("proj", i))

    def pieces(i):
        n = 2 * i
        body = [(h, j, 4, 0, BQ) for h in range(2) for j in range(0, n - 3, 4)]
        if n % 4:
            body += [(h, n - 2, 2, 0, BQ) for h in range(2)]
        diag = ([(h, n, 1, 0, BQ) for h in range(2)]
                + [(h, n + 1, 1, 128, 128) for h in range(2)])
        return body, diag

    def qk(i, diag_first):
        left = {}

        def piece(h, j, n, a0, nr, q):
            s = _dot_nt(q, _halves(k_s[_rows(128 * j, 128 * n), 128 * h:128 * h + 128]))
            for a in range(a0, a0 + nr, 64):
                m = st.get(("m", i, h, a))
                for u in range(n):
                    tile = s[a - a0:a - a0 + 64, 128 * u:128 * u + 128]
                    if j + u == 2 * i + a // 128:
                        tile = jnp.where(tri[a % 128:a % 128 + 64], tile, NEG)
                    s_s[i % 2][BQ * h + a:BQ * h + a + 64,
                               128 * (j + u):128 * (j + u + 1)] = tile
                    m = tile if m is None else jnp.maximum(m, tile)
                left[h, a] -= n
                if left[h, a] == 0:
                    m = jnp.broadcast_to(jnp.max(m, axis=-1, keepdims=True), (64, 128))
                st["m", i, h, a] = m
            if not any(left[h, a] for a in range(0, BQ, 64)):
                _fence(s_s[i % 2], zero)
            return s

        body, diag = pieces(i)
        for h, j, n, a0, nr in (diag + body[::-1] if diag_first else body[::-1] + diag):
            for a in range(a0, a0 + nr, 64):
                left[h, a] = left.get((h, a), 0) + n
            il.mxu(nr, n,
                   lambda h=h, a0=a0, nr=nr: q_s[_rows(i * BQ + a0, nr), 128 * h:128 * h + 128],
                   functools.partial(piece, h, j, n, a0, nr), ("qk", i))

    def softmax(i, before, until):
        sb, pb = s_s[i % 2], p_s[i % 3]

        def unit(h, r0, j0, j1, last, hold):
            a = r0 // 64 * 64
            m = hold(st["m", i, h, a][r0 - a:r0 - a + 16])
            l = st.pop(("l", i), None)
            r = BQ * h + r0
            for j in range(j0, j1):
                p = jnp.exp2(sb[r:r + 16, 128 * j:128 * j + 128] - m)
                l = p if l is None else l + p
                pb[_rows(r, 16), 128 * j:128 * j + 128] = _words(p)
            if last:
                pb[r0:r0 + 16, S + 128 * h:S + 128 * h + 128] = pltpu.bitcast(l, U32)
                st["sum", i, h, r0] = l
                if r0 + 16 == BQ and h == 0:
                    _fence(pb, zero)
            else:
                st["l", i] = l

        def normalizer(h, r0, hold):
            l = hold(st.pop(("sum", i, h, r0)), CFG["nextra"])
            st["inv", i, h, r0] = st["last", i] = jnp.broadcast_to(
                _recip(jnp.sum(l, axis=-1, keepdims=True)), (16, 128))

        fns, norms = [], []
        for h in (1, 0):
            for r0 in range(0, BQ, 16):
                n = 2 * i + 1 + r0 // 128
                norms += [(n, lambda hold: None), (0, functools.partial(normalizer, h, r0))]
                for j0 in range(0, n, UT):
                    j1 = min(j0 + UT, n)
                    fns.append((j1 - j0, functools.partial(unit, h, r0, j0, j1, j1 == n)))
        il.vpu(("qk", i), before, fns, _read_back(pb, zero + BQ // 2), until)
        il.vpu(("qk", i), before, norms,
               lambda: pltpu.bitcast(st.pop(("last", i))[8:], U32) if ("last", i) in st else None,
               until, CFG["nshift"])

    def pv(i, diag_first):
        left = {}

        def probs(h, j, n, a0, nr):
            return p_s[i % 3][_rows(BQ * h + a0, nr), 128 * j:128 * (j + n)]

        def piece(h, j, n, a0, nr, p):
            o = _dot(p, _halves(v_s[_rows(128 * j, 128 * n), 128 * h:128 * h + 128]))
            for a in range(a0, a0 + nr, 64):
                part = o[a - a0:a - a0 + 64]
                prev = st.pop(("o", h, a), None)
                part = part if prev is None else prev + part
                left[h, a] -= n
                if left[h, a] == 0:
                    ctx[pl.ds(ctx_row + (i * BQ + a) // 2, 32), 128 * h:128 * h + 128] = _words(
                        part * jnp.concatenate(
                            [st.pop(("inv", i, h, r0)) for r0 in range(a, a + 64, 16)], axis=0))
                else:
                    st["o", h, a] = part
            return o

        body, diag = pieces(i)
        for h, j, n, a0, nr in (diag + body[::-1] if diag_first else body + diag):
            for a in range(a0, a0 + nr, 64):
                left[h, a] = left.get((h, a), 0) + n
            il.mxu(nr, n, functools.partial(probs, h, j, n, a0, nr),
                   functools.partial(piece, h, j, n, a0, nr), ("pv", i))
        if i < NQ - 1:
            il.vpu(("pv", i), "end", [(1, lambda hold: None)], _read_back(ctx, ctx_row + zero),
                   until=("pv", i))

    for i in range(2):
        proj_q(i, 0)
        proj_k(i)
        proj_q(i, 1)
    proj_v(0)
    qk(0, True)
    softmax(0, ("v", 1), None)
    for i in range(1, NQ - 1):
        qk(i, True)
        softmax(i, ("v", i + 1), ("qk", i + 1))
        proj_k(i + 1)
        proj_q(i + 1, 0)
        proj_q(i + 1, 1)
        proj_v(i)
        if i < NQ - 2:
            pv(i - 1, False)
    qk(NQ - 1, False)
    softmax(NQ - 1, ("pv", NQ - 1), None)
    pv(NQ - 3, True)
    proj_v(NQ - 1)
    pv(NQ - 2, False)
    pv(NQ - 1, True)
    il.emit(CFG["delay"], CFG["lead"], CFG["period"])


def _transposed_weights(part, mb, w_v, stage):
    r = pl.ds(_aligned(64 * mb, 64), 64)
    for cb in range(8):
        tt = pltpu.bitcast(_halves(w_v[part, r, 128 * cb:128 * cb + 128]).T, U32)
        for hl in range(4):
            o = (4 * cb + hl) * WPITCH
            stage[o:o + 16, :] = tt[16 * hl:16 * hl + 16]
    return jnp.concatenate([stage[pl.ds(j, H, stride=WPITCH), :] for j in range(DH // 2)], axis=0)


def _b_project(il, bx_v, wt, part, row0, nrows, store):
    st = {}

    def rhs(cb, half):
        return _halves(jnp.concatenate(
            [wt[part, mb, 2 * H * cb:2 * H * (cb + 1), :]
             for mb in range(4 * half, 4 * half + 4)], axis=1))

    def first(cb, xx):
        st["y"] = _dot_nt(xx, rhs(cb, 0))
        return st["y"]

    def second(cb, r, xx):
        y = _dot_nt(xx, rhs(cb, 1))
        store(cb, r, st.pop("y") + y)
        return y

    for r in range(0, nrows, 256):
        rr = pl.ds(_half(row0 + r), 128)
        for cb in range(8):
            il.mxu(256, 4, lambda rr=rr: bx_v[rr, 0:512], functools.partial(first, cb), 'p')
            il.mxu(256, 4, lambda rr=rr: bx_v[rr, 512:1024], functools.partial(second, cb, r), 'p')


def _window(buf, cb, row, n):
    half = W // 2
    back = DIL * half
    out = [None] * W
    for w in range(half):
        x = buf[cb, pl.ds(row + (HALO - back - DIL * w), n + back), :]
        out[w], out[w + half] = x[back:], x[:n]
    return out


def _b_prob_steps(row0, nrows, qk_f, prob):
    G = CFG["G"]
    st = {}
    even = lax.broadcasted_iota(jnp.int32, (G, 128), 1) % 2 == 0

    def products(r0, cb, hold):
        q = hold(qk_f[cb, pl.ds(pl.multiple_of(row0 + (HALO + r0), 8), G), :])
        sums = st.get(r0)
        sums = [q * k if cb == 0 else sums[w] + q * k
                for w, k in enumerate(_window(qk_f, 8 + cb, row0 + r0, G))]
        st[r0] = [a + pltpu.roll(a, 64, 1) for a in sums] if cb == 7 else sums

    def finish(r0, hold):
        lg = []
        for w, a in enumerate(st.pop(r0)):
            a = a + jnp.where(even, pltpu.roll(a, 127, 1), pltpu.roll(a, 1, 1))
            if r0 < DIL * w:
                pos = row0 + r0 + lax.broadcasted_iota(jnp.int32, (G, 128), 0)
                a = jnp.where(pos >= DIL * w, a, NEG)
            lg.append(a)
        m = functools.reduce(jnp.maximum, lg)
        ps = [jnp.exp2(a - m) for a in lg]
        inv = _recip(functools.reduce(jnp.add, ps))
        for w in range(W):
            prob[pl.ds(pl.multiple_of(row0 + r0, G), G), 128 * w:128 * w + 128] = ps[w] * inv

    starts = list(range(0, nrows, G))
    fns = []
    for n in range(len(starts) + CFG["LAG"]):
        if n < len(starts):
            fns += [(1, functools.partial(products, starts[n], cb)) for cb in range(8)]
        if n >= CFG["LAG"]:
            fns.append((CFG['fw'], functools.partial(finish, starts[n - CFG["LAG"]])))
    return fns


def _b_mix_steps(row0, nrows, v_f, prob, o_s, dst0):
    half = W // 2
    back = DIL * half
    st = {}

    def step(r0, w, cb, hold):
        if cb == 0:
            r = pl.ds(pl.multiple_of(row0 + r0, 16), 16)
            st["p"] = [hold(prob[r, 128 * u:128 * u + 128]) for u in (w, w + half)]
        v = v_f[cb, pl.ds(row0 + (r0 + HALO - back - DIL * w), 16 + back), :]
        a = st["p"][0] * v[back:] + st["p"][1] * v[:16]
        st[cb] = a if w == 0 else st[cb] + a
        if w == half - 1:
            o_s[pl.ds(_half(dst0 + r0), 8), 128 * cb:128 * cb + 128] = _words(st[cb])

    return [(1, functools.partial(step, r0, w, cb))
            for r0 in range(0, nrows, 16) for w in range(half) for cb in range(8)]


def _branch_b(bx_hbm, wqkv_hbm, bwo_hbm, out_v, a_copies, a_weights,
              bx_v, w_v, bwo_v, stage, wt, bwo_p, qk_f, v_f, prob, o_a, o_b, w_sems, x_sems):
    R0, R1 = CFG["R0"], CFG["R1"]
    bscale = (DH ** -0.5) * LOG2E

    def w_copy(part, mb):
        r = pl.ds(_aligned(64 * mb, 64), 64)
        return pltpu.make_async_copy(
            wqkv_hbm.bitcast(U32).at[r, pl.ds(_aligned(part * M, M), M)], w_v.at[part, r],
            w_sems.at[8 * part + mb])

    def bwo_copy(cb):
        return pltpu.make_async_copy(
            bwo_hbm.bitcast(U32).at[:, pl.ds(_aligned(128 * cb, 128), 128)],
            bwo_v.at[cb, pl.ds(0, M // 2)], w_sems.at[24 + cb])

    def bx_copy(c):
        r = pl.ds(_aligned(c * (R0 // 2), R0 // 2), R0 // 2)
        return pltpu.make_async_copy(bx_hbm.bitcast(U32).at[r, :], bx_v.at[r, :], x_sems.at[c])

    for mb in range(8):
        w_copy(0, mb).start()
    bx_copy(0).start()
    w_copy(1, 0).start()
    bwo_copy(0).start()
    qk_f[8:16, 0:HALO, :] = jnp.zeros((8, HALO, 128), F32)
    v_f[:, 0:HALO, :] = jnp.zeros((8, HALO, 128), F32)
    prob[0:8, 0:128] = jnp.zeros((8, 128), F32)
    o_a[0:8, 0:128] = jnp.zeros((8, 128), U32)
    o_b[0:8, 0:128] = jnp.zeros((8, 128), U32)

    def first_weights(mb, carry):
        w_copy(0, mb).wait()
        wt[0, mb] = _transposed_weights(0, mb, w_v, stage)
        return carry

    with _scope('w0'):
        lax.fori_loop(0, 8, first_weights, 0, unroll=CFG["wunroll"])
    mode = CFG["dmam"]
    for c in range(1, 8 if mode < 2 else 2):
        bx_copy(c).start()
        w_copy(1, c).start()
        bwo_copy(c).start()
    if mode < 2:
        for mb in range(8):
            w_copy(2, mb).start(priority=mode)
    if CFG["astart"] == -1:
        for cp in a_copies:
            cp.start(priority=CFG["aprio"])
    if CFG["astart"] == -3:
        for cp in a_copies[:3]:
            cp.start(priority=CFG["aprio"])

    def store_into(buf, cb0, row0, scale=None):
        def store(cb, r, y):
            buf[cb0 + cb, pl.ds(pl.multiple_of(row0 + (HALO + r), 8), 256), :] = (
                y if scale is None else y * scale)
        return store

    def qk_rows(n, carry):
        part, c = n >> 3, n & 7
        w_copy(part + 1, c).wait()

        @pl.when(part == 0)
        def _():
            bx_copy(c).wait()
            bwo_copy(c).wait()

        if CFG["astart"] >= 0:
            @pl.when(n == CFG["astart"])
            def _():
                for cp in a_copies:
                    cp.start()

        if mode == 2:
            @pl.when(n < 6)
            def _():
                bx_copy(n + 2).start()
                bwo_copy(n + 2).start()

            @pl.when(n < 14)
            def _():
                w_copy(((n + 2) >> 3) + 1, (n + 2) & 7).start()

        il = _Interleaver(None)
        row0 = pl.multiple_of(c * R0, R0)
        _b_project(il, bx_v, wt, part, row0, R0,
                   store_into(qk_f, 8 * part, row0, jnp.where(part == 0, bscale, 1.0)))
        upcoming = _transposed_weights(part + 1, c, w_v, stage)
        il.emit()
        wt[part + 1, c] = upcoming
        for j in range(DH // 4):
            j = part * (DH // 4) + j
            bwo_p[c, pl.ds(pl.multiple_of(H * j, H), H), :] = (
                bwo_v[c, pl.ds(j, H, stride=DH // 2), :])
        return carry

    with _scope('L0'):
        lax.fori_loop(0, 16, qk_rows, 0)

    if CFG["astart"] == -2:
        for cp in a_copies:
            cp.start()
    if CFG["astart"] == -3:
        for cp in a_copies[3:]:
            cp.start()

    def prob_rows(c, carry):
        il = _Interleaver(c < 0)
        row0 = pl.multiple_of(c * R1, R1)
        _b_project(il, bx_v, wt, 2, row0, R1, store_into(v_f, 0, row0))
        il.vpu("begin", "end", _b_prob_steps(row0, R1, qk_f, prob), _read_back(prob, _zero_of(c)))
        il.emit(0, CFG["blead"], CFG["bperiod"])
        return carry

    with _scope('L1'):
        lax.fori_loop(0, S // R1, prob_rows, 0)

    def out_rows(c, carry):
        il = _Interleaver(c < 0)
        st = {}

        def first(n0, oo):
            st["y"] = _dot(oo, _halves(bwo_p[n0 // 128, 0:256, :]))
            return st["y"]

        def second(n0, r, oo):
            y = _dot(oo, _halves(bwo_p[n0 // 128, 256:512, :]))
            out_v[r, M + n0:M + n0 + 128] = _words(st.pop("y") + y)
            return y

        for n, (src, dst) in enumerate(((o_a, o_b), (o_b, o_a))):
            row0 = pl.multiple_of((2 * c + n) * 256, 256)
            for n0 in range(0, M, 128):
                il.mxu(256, 4, lambda src=src: src[0:128, 0:512], functools.partial(first, n0), n)
                il.mxu(256, 4, lambda src=src: src[0:128, 512:1024],
                       functools.partial(second, n0, pl.ds(_half(row0), 128)), n)
            fns = _b_mix_steps(pl.multiple_of(jnp.minimum(row0 + 256, S - 256), 256), 256,
                               v_f, prob, dst, 0)
            fns.append((0, lambda hold, dst=dst: _fence(dst, _zero_of(c))))
            il.vpu(0 if n else "begin", "end" if n else 1, fns, _read_back(dst, _zero_of(c)))
        il.vpu("begin", "end", _regroup_steps(c, S // 512, *a_weights), None)
        il.emit(CFG["bdelay"], CFG["blead"], CFG["bperiod"])
        return carry

    def first_mix(c, carry):
        row0 = pl.multiple_of(c * 64, 64)
        for _, fn in _b_mix_steps(row0, 64, v_f, prob, o_a, row0):
            fn(lambda x: x)
        return carry

    with _scope('m0'):
        lax.fori_loop(0, 256 // 64, first_mix, 0)
    with _scope('w2'):
        for cp in a_copies[:3]:
            cp.wait()
    with _scope('L2'):
        lax.fori_loop(0, S // 512, out_rows, 0)
    with _scope('w4'):
        for cp in a_copies[3:-1]:
            cp.wait()


def _branch_a(x_v, c_v, wq_h, wk_h, wv_h, wo_v, out_v, wo_copy, out_copy,
              q_s, k_s, v_s, s_a, s_b, p_a, p_b, p_c, ctx):
    R3 = CFG["R3"]

    def head_pair(t, carry):
        with _scope('it'):
            _head_pair(t, x_v, c_v, wq_h, wk_h, wv_h, q_s, k_s, v_s,
                       (s_a, s_b), (p_a, p_b, p_c), ctx)
        return carry

    with _scope('LA'):
        lax.fori_loop(0, CFG["na"], head_pair, 0)
    wo_copy.wait()

    NS = CFG["NS"]

    def out_rows(c, carry):
        w0 = pl.multiple_of(c * (R3 // 2), 128)
        for n0 in range(0, M, 128):
            y = None
            for t in range(0, H // 2, 2):
                lhs = jnp.concatenate([ctx[pl.ds(w0 + u * (S // 2), R3 // 2), :]
                                       for u in (t, t + 1)], axis=1)
                part = _dot(_halves(lhs), _halves(wo_v[128 * t:128 * t + 256, n0:n0 + 128]))
                y = part if y is None else y + part
            out_v[pl.ds(w0, R3 // 2), n0:n0 + 128] = _words(y)
            for n in range(NS):
                if n0 == min((n + 1) * (M // NS), M - 128):
                    out_copy(c, n).start()
        return carry

    with _scope('L4'):
        lax.fori_loop(0, S // R3, out_rows, 0)
    with _scope('w3'):
        for c in range(S // R3):
            for n in range(NS):
                out_copy(c, n).wait()


def _kernel(x_hbm, c_hbm, wq_hbm, wuk_hbm, wuv_hbm, wo_hbm, bx_hbm, wqkv_hbm, bwo_hbm,
            out_hbm, x_v, c_v, wq_v, wuk_v, wuv_v, wo_v, wq_h, wk_h, wv_h, out_v, a_sems, o_sems):
    R3, NS = CFG["R3"], CFG["NS"]
    vm = pltpu.VMEM
    a_copies = [
        pltpu.make_async_copy(src.bitcast(U32), dst, a_sems.at[n])
        for n, (src, dst) in enumerate((
            (wuk_hbm, wuk_v.at[pl.ds(0, DC * H // 2)]),
            (wuv_hbm, wuv_v.at[pl.ds(0, DC * H // 2)]),
            (wq_hbm, wq_v.at[pl.ds(0, M * H // 2)]),
            (c_hbm, c_v), (x_hbm, x_v), (wo_hbm, wo_v)))]
    a_weights = ((wq_v, wuk_v, wuv_v), (wq_h, wk_h, wv_h))

    def out_copy(r, cols, n):
        return pltpu.make_async_copy(out_v.at[r, cols], out_hbm.bitcast(U32).at[r, cols],
                                     o_sems.at[n])

    def a_out_copy(c, n):
        return out_copy(pl.ds(_aligned(c * (R3 // 2), R3 // 2), R3 // 2),
                        pl.ds(n * (M // NS), M // NS), 1 + NS * c + n)

    if CFG["only"] == "a":
        for cp in a_copies: cp.start()
        for cp in a_copies[:-1]: cp.wait()
    else: pl.run_scoped(
        functools.partial(_branch_b, bx_hbm, wqkv_hbm, bwo_hbm, out_v, a_copies, a_weights),
        vm((S // 2, M), U32), vm((3, M // 2, M), U32), vm((8, M // 2 + 16, 128), U32),
        vm((H * WPITCH + 16, 128), U32), vm((3, 8, M // 2, 128), U32), vm((8, M // 2, 128), U32),
        vm((16, HALO + S, 128), F32), vm((8, HALO + S, 128), F32),
        vm((S, W * 128), F32), vm((128 + 8, M), U32), vm((128 + 8, M), U32),
        pltpu.SemaphoreType.DMA((32,)), pltpu.SemaphoreType.DMA((8,)))
    b_out_copy = out_copy(pl.ds(0, S // 2), pl.ds(M, M), 0)
    b_out_copy.start()
    if CFG["only"] == "b": a_copies[-1].wait()
    else: pl.run_scoped(
        functools.partial(_branch_a, x_v, c_v, *a_weights[1], wo_v, out_v, a_copies[-1],
                          a_out_copy),
        vm((S // 2, 2 * D), U32), vm((S // 2, 2 * D), U32), vm((S // 2, 2 * D), U32),
        vm((2 * BQ + 8, S), F32), vm((2 * BQ + 8, S), F32),
        vm((BQ + 8, S + 2 * D), U32), vm((BQ + 8, S + 2 * D), U32),
        vm((BQ + 8, S + 2 * D), U32), vm((H // 2 * S // 2, 2 * D), U32))
    b_out_copy.wait()


@jax.jit
def pallas_concat_heads__compressed_kv_cla__sliding_local_dilated__prompt_kernel(
    A_x: jax.Array,
    A_c_kv: jax.Array,
    A_w_q: jax.Array,
    A_w_uk: jax.Array,
    A_w_uv: jax.Array,
    A_w_o: jax.Array,
    B_x: jax.Array,
    B_wqkv: jax.Array,
    B_wo: jax.Array,
):
    vm = pltpu.VMEM
    scratch = [
        vm((S // 2, M), U32), vm((S // 2, DC), U32),
        vm((M * H // 2 + 8, D), U32), vm((DC * H // 2 + 8, D), U32),
        vm((DC * H // 2 + 8, D), U32), vm((H * D // 2, M), U32),
        vm((2, H // 2 * (M // 2 + CFG['pad']), D), U32), vm((2, H // 2 * (DC // 2 + CFG['pad']), D), U32),
        vm((2, H // 2 * (DC // 2 + CFG['pad']), D), U32),
        vm((S // 2, 2 * M), U32),
        pltpu.SemaphoreType.DMA((6,)), pltpu.SemaphoreType.DMA((1 + CFG["NS"] * S // CFG["R3"],)),
    ]
    out = pl.pallas_call(
        _kernel,
        out_shape=jax.ShapeDtypeStruct((S, 2 * M), BF16),
        in_specs=[pl.BlockSpec(memory_space=pl.ANY)] * 9,
        out_specs=pl.BlockSpec(memory_space=pl.ANY),
        scratch_shapes=scratch,
        compiler_params=pltpu.CompilerParams(vmem_limit_bytes=124 * 1024 * 1024,
                                             flags=CFG["flags"]),
        name="fused_ab",
    )(
        A_x.reshape(S, M), A_c_kv.reshape(S, DC),
        A_w_q.reshape(M * H, D), A_w_uk.reshape(DC * H, D), A_w_uv.reshape(DC * H, D),
        A_w_o.reshape(H * D, M),
        B_x.reshape(S, M), B_wqkv, B_wo,
    )
    return out.reshape(1, S, 2 * M)
```

```python
import contextlib
import functools
import math

import jax
import jax.numpy as jnp
from jax import lax
import jax.experimental.pallas as pl
import jax.experimental.pallas.tpu as pltpu

CFG = dict(na=16, R1=512, delay=400, lead=200, period=32, ahead=256, nextra=192, nshift=500,
           pad=8, fw=3, blead=300, bperiod=32, mixat=32, only=None, scopes=False, wpad=16)

S = 2048
M = 1024
H = 32
D = 128
DC = 512
DH = 32
W = 8
DIL = 2
HALO = 16
BQ = 256
NQ = S // BQ
WPITCH = DH // 2 + 1
LOG2E = math.log2(math.e)
NEG = -1e9 * LOG2E

F32 = jnp.float32
BF16 = jnp.bfloat16
U32 = jnp.uint32


def _scope(name):
    return jax.named_scope(name) if CFG["scopes"] else contextlib.nullcontext()


def _dot(a, b):
    return jnp.dot(a, b, preferred_element_type=F32)


def _dot_nt(a, b):
    return lax.dot_general(a, b, (((1,), (1,)), ((), ())), preferred_element_type=F32)


def _words(x):
    return pltpu.bitcast(x.astype(BF16), U32)


def _halves(w):
    return pltpu.bitcast(w, BF16)


def _recip(x):
    r = pl.reciprocal(x, approx=True)
    return r * (2.0 - x * r)


def _rows(r0, n):
    return slice(r0 // 2, (r0 + n) // 2)


def _cols(cb, n=1):
    return slice(128 * cb, 128 * (cb + n))


def _aligned(x, n):
    return x if isinstance(x, int) else pl.multiple_of(x, n)


def _zero(c):
    return pl.multiple_of((c >> 8) * 8, 8)


def _read_back(buf, row):
    return lambda: pltpu.bitcast(buf[pl.ds(row, 8), 0:128], U32)


def _fence(buf, zero):
    buf[pl.ds(zero + (buf.shape[0] - 8), 8), 0:128] = jnp.zeros((8, 128), buf.dtype)


class _Interleaver:
    def __init__(self, counter):
        self.never = counter < 0
        self.steps = []
        self.side = []

    def mxu(self, rows, tiles, lhs, fn, name):
        self.steps.append((rows, tiles, lhs, fn, name))

    def vpu(self, after, before, fns, token=None, until=None, shift=0):
        self.side.append((after, before, fns, token, until, shift))

    def emit(self, delay, lead, period):
        busy, starts, slots = [0] * 4, [], []
        start, end = {}, {"begin": -delay}
        for rows, tiles, _, _, name in self.steps:
            units = sorted(range(4), key=lambda u: busy[u])[:tiles]
            t0 = busy[units[0]]
            starts.append(t0)
            start.setdefault(name, t0)
            for u in units:
                busy[u] += rows
            end[name] = max([end.get(name, 0)] + [busy[u] for u in units])
            slots += [(t, len(starts) - 1) for t in range(t0 + period, t0 + rows + 1, period)
                      if not slots or t > slots[-1][0]]
        start["end"] = max(busy)
        todo = []
        for after, before, fns, token, until, shift in self.side:
            lo = min(end[after] + delay, start[before])
            hi = max(start[before] - lead, lo)
            if until is not None:
                hi = min(hi, end[until] + delay)
            total, done = sum(w for w, _ in fns), 0
            for w, fn in fns:
                when = lo + (hi - lo) * (done + w / 2) / total + shift
                todo.append((when, len(todo), fn, token, None if shift else before))
                done += w
        todo.sort(key=lambda e: e[:2])
        results = []

        def hold_at(now):
            def hold(x, extra=0):
                past = [y for t, y in results if t <= now - CFG["ahead"] - extra]
                if not past:
                    return x
                return jnp.where(
                    self.never, jnp.concatenate([past[-1]] * (x.shape[0] // 8), axis=0), x)

            return hold

        k = 0
        for n, ((rows, _, lhs, fn, name), t0) in enumerate(zip(self.steps, starts)):
            assert all(e[4] != name for e in todo[k:])
            words = lhs()
            slabs = [words[r:r + 8] for r in range(0, rows // 2, 8)]
            for t in [t for t, step in slots if step == n] if todo else []:
                tokens = []
                while k < len(todo) and todo[k][0] < t + period:
                    todo[k][2](hold_at(t))
                    if todo[k][3] is not None and todo[k][3] not in tokens:
                        tokens.append(todo[k][3])
                    k += 1
                u = (t - t0) // 16 - 1
                for token in [x for x in (token() for token in tokens) if x is not None]:
                    head = jnp.where(self.never, token, slabs[u][:, 0:128])
                    slabs[u] = (jnp.concatenate([head, slabs[u][:, 128:]], axis=1)
                                if words.shape[1] > 128 else head)
            y = fn(_halves(jnp.concatenate(slabs, axis=0)))
            results += [(t0 + r + 16, y[r:r + 8, 0:128]) for r in range(0, rows, 16)
                        if todo and (not results or t0 + r + 16 > results[-1][0])]
        for e in todo[k:]:
            e[2](hold_at(start["end"]))


def _regroup_steps(part, nparts, raw, by_head):
    def step(src, dst, r, hold):
        r0 = _aligned(r * H, H)
        src[src.shape[0] - 8:, :] = pltpu.bitcast(hold(jnp.zeros((8, 128), F32)), U32)
        even, odd = src[pl.ds(r0, H // 2), :], src[pl.ds(r0 + H // 2, H // 2), :]
        o = pl.ds(r, H // 2, stride=dst.shape[1] // (H // 2 + 1))
        dst[0, o, :] = (even & jnp.uint32(0xFFFF)) | (odd << 16)
        dst[1, o, :] = (even >> 16) | (odd & jnp.uint32(0xFFFF0000))

    fns = []
    for src, dst in zip(raw, by_head):
        n = (src.shape[0] - 8) // H // nparts
        fns += [(1, functools.partial(step, src, dst, part * n + r)) for r in range(n)]
    return fns


def _head_pair(t, x_v, c_v, wq_h, wk_h, wv_h, q_s, k_s, v_s, s_s, p_s, ctx):
    qscale = (D ** -0.5) * LOG2E
    row = lax.broadcasted_iota(jnp.int32, (128, 128), 0)
    col = lax.broadcasted_iota(jnp.int32, (128, 128), 1)
    tri = col <= row
    zero = _zero(t)
    ctx_row = pl.multiple_of(t * (S // 2), S // 2)
    st = {}
    il = _Interleaver(t)

    def weights(ref, h, r0):
        pitch = ref.shape[1] // (H // 2 + 1)
        return _halves(ref[h, pl.ds(pl.multiple_of(t * pitch + r0, 8), 256), :])

    def proj_kv(w, dst, name, i):
        def step(h, cc):
            y = _dot(cc, weights(w, h, 0))
            dst[_rows(i * BQ, BQ), _cols(h)] = _words(y)
            return y

        for h in range(2):
            il.mxu(BQ, 4, lambda: c_v[_rows(i * BQ, BQ), :], functools.partial(step, h),
                   (name, i))

    proj_k = functools.partial(proj_kv, wk_h, k_s, "k")
    proj_v = functools.partial(proj_kv, wv_h, v_s, "v")

    def proj_q(i, h):
        r = _rows(i * BQ, BQ)

        def first(xx):
            st["q"] = _dot(xx, weights(wq_h, h, 0))
            return st["q"]

        def second(xx):
            y = _dot(xx, weights(wq_h, h, 256))
            q_s[r, _cols(h)] = _words((st.pop("q") + y) * qscale)
            return y

        il.mxu(BQ, 4, lambda: x_v[r, 0:512], first, ("q", i))
        il.mxu(BQ, 4, lambda: x_v[r, 512:1024], second, ("q", i))

    def pieces(i):
        n = 2 * i
        body = [(h, j, 4, 0, BQ) for h in range(2) for j in range(0, n - 3, 4)]
        if n % 4:
            body += [(h, n - 2, 2, 0, BQ) for h in range(2)]
        diag = ([(h, n, 1, 0, BQ) for h in range(2)]
                + [(h, n + 1, 1, 128, 128) for h in range(2)])
        return body, diag

    def scores(i, diag_first):
        left = {}

        def piece(h, j, n, a0, nr, q):
            s = _dot_nt(q, _halves(k_s[_rows(128 * j, 128 * n), _cols(h)]))
            for a in range(a0, a0 + nr, 64):
                m = st.get(("m", i, h, a))
                for u in range(n):
                    tile = s[a - a0:a - a0 + 64, _cols(u)]
                    if j + u == 2 * i + a // 128:
                        tile = jnp.where(tri[a % 128:a % 128 + 64], tile, NEG)
                    s_s[i % 2][BQ * h + a:BQ * h + a + 64, _cols(j + u)] = tile
                    m = tile if m is None else jnp.maximum(m, tile)
                left[h, a] -= n
                if left[h, a] == 0:
                    m = jnp.broadcast_to(jnp.max(m, axis=-1, keepdims=True), (64, 128))
                st["m", i, h, a] = m
            if not any(left[h, a] for a in range(0, BQ, 64)):
                _fence(s_s[i % 2], zero)
            return s

        body, diag = pieces(i)
        for h, j, n, a0, nr in (diag + body[::-1] if diag_first else body[::-1] + diag):
            for a in range(a0, a0 + nr, 64):
                left[h, a] = left.get((h, a), 0) + n
            il.mxu(nr, n, lambda h=h, a0=a0, nr=nr: q_s[_rows(i * BQ + a0, nr), _cols(h)],
                   functools.partial(piece, h, j, n, a0, nr), ("qk", i))

    def softmax(i, before, until):
        sb, pb = s_s[i % 2], p_s[i % 3]

        def unit(h, r0, j, last, hold):
            a = r0 // 64 * 64
            r = BQ * h + r0
            p = jnp.exp2(sb[r:r + 16, _cols(j)] - hold(st["m", i, h, a][r0 - a:r0 - a + 16]))
            l = st["l", i, h, r0] = p if j == 0 else st["l", i, h, r0] + p
            pb[_rows(r, 16), _cols(j)] = _words(p)
            if last:
                pb[r0:r0 + 16, _cols(S // 128 + h)] = pltpu.bitcast(l, U32)
                if r0 + 16 == BQ and h == 0:
                    _fence(pb, zero)

        def normalizer(h, r0, hold):
            l = hold(st.pop(("l", i, h, r0)), CFG["nextra"])
            st["inv", i, h, r0] = st["last", i] = jnp.broadcast_to(
                _recip(jnp.sum(l, axis=-1, keepdims=True)), (16, 128))

        def newest_normalizer():
            inv = st.pop(("last", i), None)
            return None if inv is None else pltpu.bitcast(inv[8:], U32)

        fns, norms = [], []
        for h in (1, 0):
            for r0 in range(0, BQ, 16):
                n = 2 * i + 1 + r0 // 128
                fns += [(1, functools.partial(unit, h, r0, j, j == n - 1)) for j in range(n)]
                norms += [(n, lambda hold: None), (0, functools.partial(normalizer, h, r0))]
        il.vpu(("qk", i), before, fns, _read_back(pb, zero + BQ // 2), until)
        il.vpu(("qk", i), before, norms, newest_normalizer, until, CFG["nshift"])

    def context(i, diag_first):
        left = {}

        def probs(h, j, n, a0, nr):
            return p_s[i % 3][_rows(BQ * h + a0, nr), _cols(j, n)]

        def piece(h, j, n, a0, nr, p):
            o = _dot(p, _halves(v_s[_rows(128 * j, 128 * n), _cols(h)]))
            for a in range(a0, a0 + nr, 64):
                part = o[a - a0:a - a0 + 64]
                prev = st.pop(("o", h, a), None)
                part = part if prev is None else prev + part
                left[h, a] -= n
                if left[h, a] == 0:
                    inv = jnp.concatenate(
                        [st.pop(("inv", i, h, r0)) for r0 in range(a, a + 64, 16)], axis=0)
                    ctx[pl.ds(ctx_row + (i * BQ + a) // 2, 32), _cols(h)] = _words(part * inv)
                else:
                    st["o", h, a] = part
            return o

        body, diag = pieces(i)
        for h, j, n, a0, nr in (diag + body[::-1] if diag_first else body + diag):
            for a in range(a0, a0 + nr, 64):
                left[h, a] = left.get((h, a), 0) + n
            il.mxu(nr, n, functools.partial(probs, h, j, n, a0, nr),
                   functools.partial(piece, h, j, n, a0, nr), ("pv", i))
        if i < NQ - 1:
            il.vpu(("pv", i), "end", [(1, lambda hold: None)],
                   _read_back(ctx, ctx_row + zero), ("pv", i))

    for i in range(2):
        proj_q(i, 0)
        proj_k(i)
        proj_q(i, 1)
    proj_v(0)
    scores(0, True)
    softmax(0, ("v", 1), None)
    for i in range(1, NQ - 1):
        scores(i, True)
        softmax(i, ("v", i + 1), ("qk", i + 1))
        proj_k(i + 1)
        proj_q(i + 1, 0)
        proj_q(i + 1, 1)
        proj_v(i)
        if i < NQ - 2:
            context(i - 1, False)
    scores(NQ - 1, False)
    softmax(NQ - 1, ("pv", NQ - 1), None)
    context(NQ - 3, True)
    proj_v(NQ - 1)
    context(NQ - 2, False)
    context(NQ - 1, True)
    il.emit(CFG["delay"], CFG["lead"], CFG["period"])


def _transposed_weights(group, mb, w_v):
    r = pl.ds(_aligned(64 * mb, 64), 64)
    out = []
    for cb in range(8):
        tt = pltpu.bitcast(_halves(w_v[group, r, _cols(cb)]).T, U32)
        out += [((4 * cb + hl) * WPITCH, tt[16 * hl:16 * hl + 16]) for hl in range(4)]
    return out


def _b_weights(wt, group, cb):
    return _halves(jnp.concatenate(
        [jnp.concatenate([wt[group, mb, pl.ds(j, H, stride=WPITCH), :]
                          for j in (2 * cb, 2 * cb + 1)], axis=0) for mb in range(4)], axis=1))


def _taps(buf, cb, row, w):
    back = DIL * W // 2
    x = buf[cb, pl.ds(row + (HALO - back - DIL * w), 16 + back), :]
    return x[back:], x[:16]


def _prob_steps(row0, nrows, qk_f, prob):
    st = {}
    even = lax.broadcasted_iota(jnp.int32, (16, 128), 1) % 2 == 0

    def products(r0, cb, hold):
        q = hold(qk_f[cb, pl.ds(pl.multiple_of(row0 + (HALO + r0), 8), 16), :])
        near, far = zip(*[_taps(qk_f, 8 + cb, row0 + r0, w) for w in range(W // 2)])
        sums = [q * k if cb == 0 else st[r0][w] + q * k for w, k in enumerate(near + far)]
        st[r0] = [a + pltpu.roll(a, 64, 1) for a in sums] if cb == 7 else sums

    def finish(r0, hold):
        logits = []
        for w, a in enumerate(st.pop(r0)):
            a = a + jnp.where(even, pltpu.roll(a, 127, 1), pltpu.roll(a, 1, 1))
            if r0 < DIL * w:
                pos = row0 + r0 + lax.broadcasted_iota(jnp.int32, (16, 128), 0)
                a = jnp.where(pos >= DIL * w, a, NEG)
            logits.append(a)
        m = functools.reduce(jnp.maximum, logits)
        ps = [jnp.exp2(a - m) for a in logits]
        inv = _recip(functools.reduce(jnp.add, ps))
        for w in range(W):
            prob[pl.ds(pl.multiple_of(row0 + r0, 16), 16), _cols(w)] = ps[w] * inv

    fns = []
    for r0 in range(0, nrows + 16, 16):
        if r0 < nrows:
            fns += [(1, functools.partial(products, r0, cb)) for cb in range(8)]
        if r0:
            fns.append((CFG["fw"], functools.partial(finish, r0 - 16)))
    return fns


def _mix_steps(row0, v_f, prob, o_s):
    st = {}

    def step(r0, w, cb, hold):
        if cb == 0:
            r = pl.ds(pl.multiple_of(row0 + r0, 16), 16)
            st["p"] = [hold(prob[r, _cols(u)]) for u in (w, w + W // 2)]
        near, far = _taps(v_f, cb, row0 + r0, w)
        a = st["p"][0] * near + st["p"][1] * far
        st[cb] = a if w == 0 else st[cb] + a
        if w == W // 2 - 1:
            o_s[_rows(r0, 16), _cols(cb)] = _words(st[cb])

    return [(1, functools.partial(step, r0, w, cb))
            for r0 in range(0, BQ, 16) for w in range(W // 2) for cb in range(8)]


def _project_b(bx_hbm, wqkv_hbm, raw_hbm, start_other_copies, v_f, prob, by_head,
               bx_v, w_v, wt, qk_f, wq_v, wk_v, wv_v, w_sems, x_sems, raw_sems):
    R1 = CFG["R1"]
    bscale = (DH ** -0.5) * LOG2E
    raw = (wq_v, wk_v, wv_v)

    def w_copy(group, r0, n, sem):
        src = wqkv_hbm.bitcast(U32).at[pl.ds(_aligned((group & 1) * 256 + r0, 64), n),
                                       pl.ds(_aligned((group >> 1) * M, M), M)]
        return pltpu.make_async_copy(src, w_v.at[group, pl.ds(_aligned(r0, 64), n)],
                                     w_sems.at[sem])

    def x_copy(n):
        r = pl.ds(_aligned((n & 1) * 512, 512), 512)
        src = bx_hbm.bitcast(U32).at[r, pl.ds(_aligned((n >> 1) * 512, 512), 512)]
        return pltpu.make_async_copy(src, bx_v.at[n >> 1, r], x_sems.at[n])

    raw_copies = [
        pltpu.make_async_copy(src.bitcast(U32), dst.at[pl.ds(0, dst.shape[0] - 8)],
                              raw_sems.at[n])
        for n, (src, dst) in enumerate(zip(raw_hbm, raw))]

    for mb in range(4):
        w_copy(0, 64 * mb, 64, mb).start()
    for n in range(6):
        if n < 4:
            x_copy(n).start()
        if n:
            w_copy(n, 0, 256, 3 + n).start()
    for cp in raw_copies:
        cp.start()
    start_other_copies()
    qk_f[8:16, 0:HALO, :] = jnp.zeros((8, HALO, 128), F32)
    v_f[:, 0:HALO, :] = jnp.zeros((8, HALO, 128), F32)
    prob[0:8, 0:128] = jnp.zeros((8, 128), F32)

    def first_weights(mb, carry):
        w_copy(0, 64 * mb, 64, mb).wait()
        for r, x in _transposed_weights(0, mb, w_v):
            wt[0, mb, r:r + 16, :] = x
        return carry

    with _scope('w0'):
        lax.fori_loop(0, 4, first_weights, 0)

    def qk_rows(n, carry):
        upcoming = jnp.minimum(n, 5)

        @pl.when(n < 4)
        def _():
            x_copy(n).wait()

        @pl.when((n >= 1) & (n <= 5))
        def _():
            w_copy(n, 0, 256, 3 + n).wait()

        scale = jnp.where(n < 4, bscale, 1.0)
        for r0 in range(0, S // 2, BQ):
            row = pl.multiple_of((n & 1) * (S // 2) + r0, BQ)
            x = _halves(bx_v[(n >> 1) & 1, pl.ds(pl.multiple_of(row >> 1, 128), 128), :])
            r = pl.ds(pl.multiple_of(row + HALO, 8), BQ)
            for cb in range(8):
                o = 8 * (n >> 2) + cb
                y = _dot_nt(x, _b_weights(wt, n >> 1, cb)) * scale
                qk_f[o, r, :] = jnp.where((n & 2) != 0, qk_f[o, r, :], 0.0) + y
        for mb, tiles in [(mb, _transposed_weights(upcoming, mb, w_v)) for mb in range(4)]:
            for r, x in tiles:
                wt[upcoming, mb, r:r + 16, :] = x
        return carry

    with _scope('L0'):
        lax.fori_loop(0, 8, qk_rows, 0)
    with _scope('w1'):
        for cp in raw_copies:
            cp.wait()

    def v_rows(c, carry):
        il = _Interleaver(c)
        row0 = pl.multiple_of(c * R1, R1)
        st = {}

        def first(cb, xx):
            st["y"] = _dot_nt(xx, _b_weights(wt, 4, cb))
            return st["y"]

        def second(cb, r, xx):
            y = _dot_nt(xx, _b_weights(wt, 5, cb))
            v_f[cb, r, :] = st.pop("y") + y
            return y

        for r0 in range(0, R1, BQ):
            rw = pl.ds(pl.multiple_of((row0 + r0) >> 1, 128), 128)
            r = pl.ds(pl.multiple_of(row0 + (HALO + r0), 8), BQ)
            for cb in range(8):
                il.mxu(BQ, 4, lambda rw=rw: bx_v[0, rw, :], functools.partial(first, cb), "v")
                il.mxu(BQ, 4, lambda rw=rw: bx_v[1, rw, :], functools.partial(second, cb, r),
                       "v")
        il.vpu("begin", "end", _prob_steps(row0, R1, qk_f, prob), _read_back(prob, _zero(c)))
        il.vpu("begin", "end", _regroup_steps(c, S // R1, raw, by_head))
        il.emit(0, CFG["blead"], CFG["bperiod"])
        return carry

    with _scope('L1'):
        lax.fori_loop(0, S // R1, v_rows, 0)


def _attend_and_project(x_v, c_v, by_head, wo_v, bwo_v, v_f, prob, wait_for_output_weights,
                        out_hbm, q_s, k_s, v_s, s_a, s_b, p_a, p_b, p_c, ctx, o_s, out_v, sems):
    def head_pair(t, carry):
        with _scope('it'):
            _head_pair(t, x_v, c_v, *by_head, q_s, k_s, v_s, (s_a, s_b), (p_a, p_b, p_c), ctx)
        return carry

    o_s[0:8, 0:128] = jnp.zeros((8, 128), U32)
    with _scope('LA'):
        lax.fori_loop(0, CFG["na"], head_pair, 0)
    wait_for_output_weights()

    def out_copy(c):
        r = pl.ds(_aligned(c * (BQ // 2), BQ // 2), BQ // 2)
        return pltpu.make_async_copy(out_v.at[r], out_hbm.bitcast(U32).at[r], sems.at[c])

    def out_rows(c, carry):
        il = _Interleaver(c)
        w0 = pl.multiple_of(c * (BQ // 2), BQ // 2)
        st = {}

        def step(rhs, first, cb, lhs):
            y = _dot(lhs, _halves(rhs()))
            st["y"] = y if first else st["y"] + y
            if cb is not None:
                out_v[pl.ds(w0, BQ // 2), _cols(cb)] = _words(st["y"])
            return y

        def ctx_rows(t):
            return jnp.concatenate([ctx[pl.ds(w0 + u * (S // 2), BQ // 2), :]
                                    for u in (t, t + 1)], axis=1)

        def bwo_rows(cb, half):
            return jnp.concatenate([bwo_v[cb, pl.ds(j, H, stride=DH // 2), :]
                                    for j in range(8 * half, 8 * half + 8)], axis=0)

        for cb in range(8):
            for t in range(0, H // 2, 2):
                il.mxu(BQ, 4, functools.partial(ctx_rows, t), functools.partial(
                    step, lambda t=t, cb=cb: wo_v[128 * t:128 * t + 256, _cols(cb)],
                    t == 0, cb if t == H // 2 - 2 else None), "a")
        for cb in range(8):
            for half in range(2):
                il.mxu(BQ, 4, lambda half=half: o_s[0:BQ // 2, _cols(4 * half, 4)],
                       functools.partial(step, functools.partial(bwo_rows, cb, half),
                                         half == 0, 8 + cb if half else None), "b")
        fns = _mix_steps(pl.multiple_of(c * BQ, BQ), v_f, prob, o_s)
        fns.append((0, lambda hold: _fence(o_s, _zero(c))))
        il.vpu("begin", "b", fns, _read_back(o_s, _zero(c)))
        il.emit(0, CFG["blead"], CFG["mixat"])
        out_copy(c).start()
        return carry

    with _scope('L4'):
        lax.fori_loop(0, NQ, out_rows, 0)
    with _scope('w3'):
        for c in range(NQ):
            out_copy(c).wait()


def _kernel(x_hbm, c_hbm, wq_hbm, wuk_hbm, wuv_hbm, wo_hbm, bx_hbm, wqkv_hbm, bwo_hbm, out_hbm,
            x_v, c_v, wo_v, bwo_v, wq_h, wk_h, wv_h, v_f, prob, sems):
    vm = pltpu.VMEM
    copies = [pltpu.make_async_copy(src.bitcast(U32), dst, sems.at[n])
              for n, (src, dst) in enumerate(((x_hbm, x_v), (c_hbm, c_v), (wo_hbm, wo_v)))]
    copies += [pltpu.make_async_copy(bwo_hbm.bitcast(U32).at[:, pl.ds(128 * cb, 128)],
                                     bwo_v.at[cb, pl.ds(0, M // 2)], sems.at[3 + cb])
               for cb in range(8)]
    by_head = (wq_h, wk_h, wv_h)

    def start(cps):
        for cp in cps:
            cp.start()

    def wait(cps):
        for cp in cps:
            cp.wait()

    if CFG["only"] == "a": start(copies)
    else: pl.run_scoped(
        functools.partial(_project_b, bx_hbm, wqkv_hbm, (wq_hbm, wuk_hbm, wuv_hbm),
                          functools.partial(start, copies), v_f, prob, by_head),
        vm((2, S // 2, M // 2), U32), vm((6, M // 4, M), U32),
        vm((6, 4, H * WPITCH + CFG["wpad"], 128), U32), vm((16, HALO + S, 128), F32),
        vm((M * H // 2 + 8, D), U32), vm((DC * H // 2 + 8, D), U32),
        vm((DC * H // 2 + 8, D), U32), pltpu.SemaphoreType.DMA((9,)),
        pltpu.SemaphoreType.DMA((4,)), pltpu.SemaphoreType.DMA((3,)))
    with _scope('w2'):
        wait(copies[:2])
    pl.run_scoped(
        functools.partial(_attend_and_project, x_v, c_v, by_head, wo_v, bwo_v, v_f, prob,
                          functools.partial(wait, copies[2:]), out_hbm),
        vm((S // 2, 2 * D), U32), vm((S // 2, 2 * D), U32), vm((S // 2, 2 * D), U32),
        vm((2 * BQ + 8, S), F32), vm((2 * BQ + 8, S), F32),
        vm((BQ + 8, S + 2 * D), U32), vm((BQ + 8, S + 2 * D), U32),
        vm((BQ + 8, S + 2 * D), U32), vm((H // 2 * S // 2, 2 * D), U32),
        vm((BQ // 2 + 8, M), U32), vm((S // 2, 2 * M), U32), pltpu.SemaphoreType.DMA((NQ,)))


@jax.jit
def pallas_concat_heads__compressed_kv_cla__sliding_local_dilated__prompt_kernel(
    A_x: jax.Array,
    A_c_kv: jax.Array,
    A_w_q: jax.Array,
    A_w_uk: jax.Array,
    A_w_uv: jax.Array,
    A_w_o: jax.Array,
    B_x: jax.Array,
    B_wqkv: jax.Array,
    B_wo: jax.Array,
):
    vm = pltpu.VMEM
    slots = H // 2 + 1
    pad = CFG["pad"]
    out = pl.pallas_call(
        _kernel,
        out_shape=jax.ShapeDtypeStruct((S, 2 * M), BF16),
        in_specs=[pl.BlockSpec(memory_space=pl.ANY)] * 9,
        out_specs=pl.BlockSpec(memory_space=pl.ANY),
        scratch_shapes=[
            vm((S // 2, M), U32), vm((S // 2, DC), U32), vm((H * D // 2, M), U32),
            vm((8, M // 2 + 16, 128), U32), vm((2, slots * (M // 2 + pad), D), U32),
            vm((2, slots * (DC // 2 + pad), D), U32), vm((2, slots * (DC // 2 + pad), D), U32),
            vm((8, HALO + S, 128), F32), vm((S, W * 128), F32),
            pltpu.SemaphoreType.DMA((11,)),
        ],
        compiler_params=pltpu.CompilerParams(vmem_limit_bytes=124 * 1024 * 1024),
        name="concat_heads_attention",
    )(
        A_x.reshape(S, M), A_c_kv.reshape(S, DC),
        A_w_q.reshape(M * H, D), A_w_uk.reshape(DC * H, D), A_w_uv.reshape(DC * H, D),
        A_w_o.reshape(H * D, M), B_x.reshape(S, M), B_wqkv, B_wo,
    )
    return out.reshape(1, S, 2 * M)
```

```python
import contextlib
import functools
import math

import jax
import jax.numpy as jnp
from jax import lax
import jax.experimental.pallas as pl
import jax.experimental.pallas.tpu as pltpu

CFG = dict(na=16, R1=512, delay=400, lead=200, period=32, ahead=256, nextra=192, nshift=500,
           pad=8, fw=4, hp=16, pp=256, rp=32, xp=0, kp=8, vp=0, qp=0, blead=300, bperiod=16, mixat=32, only=None, scopes=False, wpad=16)

S = 2048
M = 1024
H = 32
D = 128
DC = 512
DH = 32
W = 8
DIL = 2
HALO = 16
BQ = 256
NQ = S // BQ
WPITCH = DH // 2 + 1
LOG2E = math.log2(math.e)
NEG = -1e9 * LOG2E

F32 = jnp.float32
BF16 = jnp.bfloat16
U32 = jnp.uint32


def _scope(name):
    return jax.named_scope(name) if CFG["scopes"] else contextlib.nullcontext()


def _dot(a, b):
    return jnp.dot(a, b, preferred_element_type=F32)


def _dot_nt(a, b):
    return lax.dot_general(a, b, (((1,), (1,)), ((), ())), preferred_element_type=F32)


def _words(x):
    return pltpu.bitcast(x.astype(BF16), U32)


def _halves(w):
    return pltpu.bitcast(w, BF16)


def _recip(x):
    r = pl.reciprocal(x, approx=True)
    return r * (2.0 - x * r)


def _rows(r0, n):
    return slice(r0 // 2, (r0 + n) // 2)


def _cols(cb, n=1):
    return slice(128 * cb, 128 * (cb + n))


def _aligned(x, n):
    return x if isinstance(x, int) else pl.multiple_of(x, n)


def _zero(c):
    return pl.multiple_of((c >> 8) * 8, 8)


def _read_back(buf, row):
    return lambda: pltpu.bitcast(buf[pl.ds(row, 8), 0:128], U32)


def _fence(buf, zero):
    buf[pl.ds(zero + (buf.shape[0] - 8), 8), 0:128] = jnp.zeros((8, 128), buf.dtype)


class _Interleaver:
    def __init__(self, counter):
        self.never = counter < 0
        self.steps = []
        self.side = []

    def mxu(self, rows, tiles, lhs, fn, name):
        self.steps.append((rows, tiles, lhs, fn, name))

    def vpu(self, after, before, fns, token=None, until=None, shift=0):
        self.side.append((after, before, fns, token, until, shift))

    def emit(self, delay, lead, period):
        busy, starts, slots = [0] * 4, [], []
        start, end = {}, {"begin": -delay}
        for rows, tiles, _, _, name in self.steps:
            units = sorted(range(4), key=lambda u: busy[u])[:tiles]
            t0 = busy[units[0]]
            starts.append(t0)
            start.setdefault(name, t0)
            for u in units:
                busy[u] += rows
            end[name] = max([end.get(name, 0)] + [busy[u] for u in units])
            slots += [(t, len(starts) - 1) for t in range(t0 + period, t0 + rows + 1, period)
                      if not slots or t > slots[-1][0]]
        start["end"] = max(busy)
        todo = []
        for after, before, fns, token, until, shift in self.side:
            lo = min(end[after] + delay, start[before])
            hi = max(start[before] - lead, lo)
            if until is not None:
                hi = min(hi, end[until] + delay)
            total, done = sum(w for w, _ in fns), 0
            for w, fn in fns:
                when = lo + (hi - lo) * (done + w / 2) / total + shift
                todo.append((when, len(todo), fn, token, None if shift else before))
                done += w
        todo.sort(key=lambda e: e[:2])
        results = []

        def hold_at(now):
            def hold(x, extra=0):
                past = [y for t, y in results if t <= now - CFG["ahead"] - extra]
                if not past:
                    return x
                return jnp.where(
                    self.never, jnp.concatenate([past[-1]] * (x.shape[0] // 8), axis=0), x)

            return hold

        k = 0
        for n, ((rows, _, lhs, fn, name), t0) in enumerate(zip(self.steps, starts)):
            assert all(e[4] != name for e in todo[k:])
            words = lhs()
            slabs = [words[r:r + 8] for r in range(0, rows // 2, 8)]
            for t in [t for t, step in slots if step == n] if todo else []:
                tokens = []
                while k < len(todo) and todo[k][0] < t + period:
                    todo[k][2](hold_at(t))
                    if todo[k][3] is not None and todo[k][3] not in tokens:
                        tokens.append(todo[k][3])
                    k += 1
                u = (t - t0) // 16 - 1
                for token in [x for x in (token() for token in tokens) if x is not None]:
                    head = jnp.where(self.never, token, slabs[u][:, 0:128])
                    slabs[u] = (jnp.concatenate([head, slabs[u][:, 128:]], axis=1)
                                if words.shape[1] > 128 else head)
            y = fn(_halves(jnp.concatenate(slabs, axis=0)))
            results += [(t0 + r + 16, y[r:r + 8, 0:128]) for r in range(0, rows, 16)
                        if todo and (not results or t0 + r + 16 > results[-1][0])]
        for e in todo[k:]:
            e[2](hold_at(start["end"]))


def _regroup_steps(part, nparts, raw, by_head):
    def step(src, dst, r, hold):
        r0 = _aligned(r * H, H)
        src[src.shape[0] - 8:, :] = pltpu.bitcast(hold(jnp.zeros((8, 128), F32)), U32)
        even, odd = src[pl.ds(r0, H // 2), :], src[pl.ds(r0 + H // 2, H // 2), :]
        o = pl.ds(r, H // 2, stride=dst.shape[1] // (H // 2 + 1) // 8 * 8)
        dst[0, o, :] = (even & jnp.uint32(0xFFFF)) | (odd << 16)
        dst[1, o, :] = (even >> 16) | (odd & jnp.uint32(0xFFFF0000))

    fns = []
    for src, dst in zip(raw, by_head):
        n = (src.shape[0] - CFG['rp']) // H // nparts
        fns += [(1, functools.partial(step, src, dst, part * n + r)) for r in range(n)]
    return fns


def _head_pair(t, x_v, c_v, wq_h, wk_h, wv_h, q_s, k_s, v_s, s_s, p_s, ctx):
    qscale = (D ** -0.5) * LOG2E
    row = lax.broadcasted_iota(jnp.int32, (128, 128), 0)
    col = lax.broadcasted_iota(jnp.int32, (128, 128), 1)
    tri = col <= row
    zero = _zero(t)
    ctx_row = pl.multiple_of(t * (S // 2), S // 2)
    st = {}
    il = _Interleaver(t)

    def weights(ref, h, r0):
        pitch = ref.shape[1] // (H // 2 + 1) // 8 * 8
        return _halves(ref[h, pl.ds(pl.multiple_of(t * pitch + r0, 8), 256), :])

    def proj_kv(w, dst, name, i):
        def step(h, cc):
            y = _dot(cc, weights(w, h, 0))
            dst[_rows(i * BQ, BQ), _cols(h)] = _words(y)
            return y

        for h in range(2):
            il.mxu(BQ, 4, lambda: c_v[_rows(i * BQ, BQ), :], functools.partial(step, h),
                   (name, i))

    proj_k = functools.partial(proj_kv, wk_h, k_s, "k")
    proj_v = functools.partial(proj_kv, wv_h, v_s, "v")

    def proj_q(i, h):
        r = _rows(i * BQ, BQ)

        def first(xx):
            st["q"] = _dot(xx, weights(wq_h, h, 0))
            return st["q"]

        def second(xx):
            y = _dot(xx, weights(wq_h, h, 256))
            q_s[r, _cols(h)] = _words((st.pop("q") + y) * qscale)
            return y

        il.mxu(BQ, 4, lambda: x_v[r, 0:512], first, ("q", i))
        il.mxu(BQ, 4, lambda: x_v[r, 512:1024], second, ("q", i))

    def pieces(i):
        n = 2 * i
        body = [(h, j, 4, 0, BQ) for h in range(2) for j in range(0, n - 3, 4)]
        if n % 4:
            body += [(h, n - 2, 2, 0, BQ) for h in range(2)]
        diag = ([(h, n, 1, 0, BQ) for h in range(2)]
                + [(h, n + 1, 1, 128, 128) for h in range(2)])
        return body, diag

    def scores(i, diag_first):
        left = {}

        def piece(h, j, n, a0, nr, q):
            s = _dot_nt(q, _halves(k_s[_rows(128 * j, 128 * n), _cols(h)]))
            for a in range(a0, a0 + nr, 64):
                m = st.get(("m", i, h, a))
                for u in range(n):
                    tile = s[a - a0:a - a0 + 64, _cols(u)]
                    if j + u == 2 * i + a // 128:
                        tile = jnp.where(tri[a % 128:a % 128 + 64], tile, NEG)
                    s_s[i % 2][BQ * h + a:BQ * h + a + 64, _cols(j + u)] = tile
                    m = tile if m is None else jnp.maximum(m, tile)
                left[h, a] -= n
                if left[h, a] == 0:
                    m = jnp.broadcast_to(jnp.max(m, axis=-1, keepdims=True), (64, 128))
                st["m", i, h, a] = m
            if not any(left[h, a] for a in range(0, BQ, 64)):
                _fence(s_s[i % 2], zero)
            return s

        body, diag = pieces(i)
        for h, j, n, a0, nr in (diag + body[::-1] if diag_first else body[::-1] + diag):
            for a in range(a0, a0 + nr, 64):
                left[h, a] = left.get((h, a), 0) + n
            il.mxu(nr, n, lambda h=h, a0=a0, nr=nr: q_s[_rows(i * BQ + a0, nr), _cols(h)],
                   functools.partial(piece, h, j, n, a0, nr), ("qk", i))

    def softmax(i, before, until):
        sb, pb = s_s[i % 2], p_s[i % 3]

        def unit(h, r0, j, last, hold):
            a = r0 // 64 * 64
            r = BQ * h + r0
            p = jnp.exp2(sb[r:r + 16, _cols(j)] - hold(st["m", i, h, a][r0 - a:r0 - a + 16]))
            l = st["l", i, h, r0] = p if j == 0 else st["l", i, h, r0] + p
            pb[_rows(r, 16), _cols(j)] = _words(p)
            if last:
                pb[r0:r0 + 16, _cols(S // 128 + h)] = pltpu.bitcast(l, U32)
                if r0 + 16 == BQ and h == 0:
                    _fence(pb, zero)

        def normalizer(h, r0, hold):
            l = hold(st.pop(("l", i, h, r0)), CFG["nextra"])
            st["inv", i, h, r0] = st["last", i] = jnp.broadcast_to(
                _recip(jnp.sum(l, axis=-1, keepdims=True)), (16, 128))

        def newest_normalizer():
            inv = st.pop(("last", i), None)
            return None if inv is None else pltpu.bitcast(inv[8:], U32)

        fns, norms = [], []
        for h in (1, 0):
            for r0 in range(0, BQ, 16):
                n = 2 * i + 1 + r0 // 128
                fns += [(1, functools.partial(unit, h, r0, j, j == n - 1)) for j in range(n)]
                norms += [(n, lambda hold: None), (0, functools.partial(normalizer, h, r0))]
        il.vpu(("qk", i), before, fns, _read_back(pb, zero + BQ // 2), until)
        il.vpu(("qk", i), before, norms, newest_normalizer, until, CFG["nshift"])

    def context(i, diag_first):
        left = {}

        def probs(h, j, n, a0, nr):
            return p_s[i % 3][_rows(BQ * h + a0, nr), _cols(j, n)]

        def piece(h, j, n, a0, nr, p):
            o = _dot(p, _halves(v_s[_rows(128 * j, 128 * n), _cols(h)]))
            for a in range(a0, a0 + nr, 64):
                part = o[a - a0:a - a0 + 64]
                prev = st.pop(("o", h, a), None)
                part = part if prev is None else prev + part
                left[h, a] -= n
                if left[h, a] == 0:
                    inv = jnp.concatenate(
                        [st.pop(("inv", i, h, r0)) for r0 in range(a, a + 64, 16)], axis=0)
                    ctx[pl.ds(ctx_row + (i * BQ + a) // 2, 32), _cols(h)] = _words(part * inv)
                else:
                    st["o", h, a] = part
            return o

        body, diag = pieces(i)
        for h, j, n, a0, nr in (diag + body[::-1] if diag_first else body + diag):
            for a in range(a0, a0 + nr, 64):
                left[h, a] = left.get((h, a), 0) + n
            il.mxu(nr, n, functools.partial(probs, h, j, n, a0, nr),
                   functools.partial(piece, h, j, n, a0, nr), ("pv", i))
        if i < NQ - 1:
            il.vpu(("pv", i), "end", [(1, lambda hold: None)],
                   _read_back(ctx, ctx_row + zero), ("pv", i))

    for i in range(2):
        proj_q(i, 0)
        proj_k(i)
        proj_q(i, 1)
    proj_v(0)
    scores(0, True)
    softmax(0, ("v", 1), None)
    for i in range(1, NQ - 1):
        scores(i, True)
        softmax(i, ("v", i + 1), ("qk", i + 1))
        proj_k(i + 1)
        proj_q(i + 1, 0)
        proj_q(i + 1, 1)
        proj_v(i)
        if i < NQ - 2:
            context(i - 1, False)
    scores(NQ - 1, False)
    softmax(NQ - 1, ("pv", NQ - 1), None)
    context(NQ - 3, True)
    proj_v(NQ - 1)
    context(NQ - 2, False)
    context(NQ - 1, True)
    il.emit(CFG["delay"], CFG["lead"], CFG["period"])


def _transposed_weights(group, mb, w_v):
    r = pl.ds(_aligned(64 * mb, 64), 64)
    out = []
    for cb in range(8):
        tt = pltpu.bitcast(_halves(w_v[group, r, _cols(cb)]).T, U32)
        out += [((4 * cb + hl) * WPITCH, tt[16 * hl:16 * hl + 16]) for hl in range(4)]
    return out


def _b_weights(wt, group, cb):
    return _halves(jnp.concatenate(
        [jnp.concatenate([wt[group, mb, pl.ds(j, H, stride=WPITCH), :]
                          for j in (2 * cb, 2 * cb + 1)], axis=0) for mb in range(4)], axis=1))


def _taps(buf, cb, row, w):
    back = DIL * W // 2
    x = buf[cb, pl.ds(row + (HALO - back - DIL * w), 16 + back), :]
    return x[back:], x[:16]


def _prob_steps(row0, nrows, qk_f, prob):
    st = {}
    even = lax.broadcasted_iota(jnp.int32, (16, 128), 1) % 2 == 0

    def products(r0, cb, hold):
        q = hold(qk_f[cb, pl.ds(pl.multiple_of(row0 + (HALO + r0), 8), 16), :])
        near, far = zip(*[_taps(qk_f, 8 + cb, row0 + r0, w) for w in range(W // 2)])
        sums = [q * k if cb == 0 else st[r0][w] + q * k for w, k in enumerate(near + far)]
        st[r0] = [a + pltpu.roll(a, 64, 1) for a in sums] if cb == 7 else sums

    def finish(r0, hold):
        logits = []
        for w, a in enumerate(st.pop(r0)):
            a = a + jnp.where(even, pltpu.roll(a, 127, 1), pltpu.roll(a, 1, 1))
            if r0 < DIL * w:
                pos = row0 + r0 + lax.broadcasted_iota(jnp.int32, (16, 128), 0)
                a = jnp.where(pos >= DIL * w, a, NEG)
            logits.append(a)
        m = functools.reduce(jnp.maximum, logits)
        ps = [jnp.exp2(a - m) for a in logits]
        inv = _recip(functools.reduce(jnp.add, ps))
        for w in range(W):
            prob[pl.ds(pl.multiple_of(row0 + r0, 16), 16), _cols(w)] = ps[w] * inv

    fns = []
    for r0 in range(0, nrows + 16, 16):
        if r0 < nrows:
            fns += [(1, functools.partial(products, r0, cb)) for cb in range(8)]
        if r0:
            fns.append((CFG["fw"], functools.partial(finish, r0 - 16)))
    return fns


def _mix_steps(row0, v_f, prob, o_s):
    st = {}

    def step(r0, w, cb, hold):
        if cb == 0:
            r = pl.ds(pl.multiple_of(row0 + r0, 16), 16)
            st["p"] = [hold(prob[r, _cols(u)]) for u in (w, w + W // 2)]
        near, far = _taps(v_f, cb, row0 + r0, w)
        a = st["p"][0] * near + st["p"][1] * far
        st[cb] = a if w == 0 else st[cb] + a
        if w == W // 2 - 1:
            o_s[_rows(r0, 16), _cols(cb)] = _words(st[cb])

    return [(1, functools.partial(step, r0, w, cb))
            for r0 in range(0, BQ, 16) for w in range(W // 2) for cb in range(8)]


def _project_b(bx_hbm, wqkv_hbm, raw_hbm, start_other_copies, v_f, prob, by_head,
               bx_v, w_v, wt, qk_f, wq_v, wk_v, wv_v, w_sems, x_sems, raw_sems):
    R1 = CFG["R1"]
    bscale = (DH ** -0.5) * LOG2E
    raw = (wq_v, wk_v, wv_v)

    def w_copy(group, r0, n, sem):
        src = wqkv_hbm.bitcast(U32).at[pl.ds(_aligned((group & 1) * 256 + r0, 64), n),
                                       pl.ds(_aligned((group >> 1) * M, M), M)]
        return pltpu.make_async_copy(src, w_v.at[group, pl.ds(_aligned(r0, 64), n)],
                                     w_sems.at[sem])

    def x_copy(n):
        r = pl.ds(_aligned((n & 1) * 512, 512), 512)
        src = bx_hbm.bitcast(U32).at[r, pl.ds(_aligned((n >> 1) * 512, 512), 512)]
        return pltpu.make_async_copy(src, bx_v.at[n >> 1, r], x_sems.at[n])

    raw_copies = [
        pltpu.make_async_copy(src.bitcast(U32), dst.at[pl.ds(0, dst.shape[0] - CFG['rp'])],
                              raw_sems.at[n])
        for n, (src, dst) in enumerate(zip(raw_hbm, raw))]

    for mb in range(4):
        w_copy(0, 64 * mb, 64, mb).start()
    for n in range(6):
        if n < 4:
            x_copy(n).start()
        if n:
            w_copy(n, 0, 256, 3 + n).start()
    for cp in raw_copies:
        cp.start()
    start_other_copies()
    qk_f[8:16, 0:HALO, :] = jnp.zeros((8, HALO, 128), F32)
    v_f[:, 0:HALO, :] = jnp.zeros((8, HALO, 128), F32)
    prob[0:8, 0:128] = jnp.zeros((8, 128), F32)

    def first_weights(mb, carry):
        w_copy(0, 64 * mb, 64, mb).wait()
        for r, x in _transposed_weights(0, mb, w_v):
            wt[0, mb, r:r + 16, :] = x
        return carry

    with _scope('w0'):
        lax.fori_loop(0, 4, first_weights, 0)

    def qk_rows(n, carry):
        upcoming = jnp.minimum(n, 5)

        @pl.when(n < 4)
        def _():
            x_copy(n).wait()

        @pl.when((n >= 1) & (n <= 5))
        def _():
            w_copy(n, 0, 256, 3 + n).wait()

        scale = jnp.where(n < 4, bscale, 1.0)
        for r0 in range(0, S // 2, BQ):
            row = pl.multiple_of((n & 1) * (S // 2) + r0, BQ)
            x = _halves(bx_v[(n >> 1) & 1, pl.ds(pl.multiple_of(row >> 1, 128), 128), :])
            r = pl.ds(pl.multiple_of(row + HALO, 8), BQ)
            for cb in range(8):
                o = 8 * (n >> 2) + cb
                y = _dot_nt(x, _b_weights(wt, n >> 1, cb)) * scale
                qk_f[o, r, :] = jnp.where((n & 2) != 0, qk_f[o, r, :], 0.0) + y
        for mb, tiles in [(mb, _transposed_weights(upcoming, mb, w_v)) for mb in range(4)]:
            for r, x in tiles:
                wt[upcoming, mb, r:r + 16, :] = x
        return carry

    with _scope('L0'):
        lax.fori_loop(0, 8, qk_rows, 0)
    with _scope('w1'):
        for cp in raw_copies:
            cp.wait()

    def v_rows(c, carry):
        il = _Interleaver(c)
        row0 = pl.multiple_of(c * R1, R1)
        st = {}

        def first(cb, xx):
            st["y"] = _dot_nt(xx, _b_weights(wt, 4, cb))
            return st["y"]

        def second(cb, r, xx):
            y = _dot_nt(xx, _b_weights(wt, 5, cb))
            v_f[cb, r, :] = st.pop("y") + y
            return y

        for r0 in range(0, R1, BQ):
            rw = pl.ds(pl.multiple_of((row0 + r0) >> 1, 128), 128)
            r = pl.ds(pl.multiple_of(row0 + (HALO + r0), 8), BQ)
            for cb in range(8):
                il.mxu(BQ, 4, lambda rw=rw: bx_v[0, rw, :], functools.partial(first, cb), "v")
                il.mxu(BQ, 4, lambda rw=rw: bx_v[1, rw, :], functools.partial(second, cb, r),
                       "v")
        il.vpu("begin", "end", _prob_steps(row0, R1, qk_f, prob), _read_back(prob, _zero(c)))
        il.vpu("begin", "end", _regroup_steps(c, S // R1, raw, by_head))
        il.emit(0, CFG["blead"], CFG["bperiod"])
        return carry

    with _scope('L1'):
        lax.fori_loop(0, S // R1, v_rows, 0)


def _attend_and_project(x_v, c_v, by_head, wo_v, bwo_v, v_f, prob, wait_for_output_weights,
                        out_hbm, ctx, out_v, o_s, q_s, k_s, v_s, s_a, s_b, p_a, p_b, p_c, sems):
    def head_pair(t, carry):
        with _scope('it'):
            _head_pair(t, x_v, c_v, *by_head, q_s, k_s, v_s, (s_a, s_b), (p_a, p_b, p_c), ctx)
        return carry

    o_s[0:8, 0:128] = jnp.zeros((8, 128), U32)
    with _scope('LA'):
        lax.fori_loop(0, CFG["na"], head_pair, 0)
    wait_for_output_weights()

    def out_copy(c):
        r = pl.ds(_aligned(c * (BQ // 2), BQ // 2), BQ // 2)
        return pltpu.make_async_copy(out_v.at[r], out_hbm.bitcast(U32).at[r], sems.at[c])

    def out_rows(c, carry):
        il = _Interleaver(c)
        w0 = pl.multiple_of(c * (BQ // 2), BQ // 2)
        st = {}

        def step(rhs, first, cb, lhs):
            y = _dot(lhs, _halves(rhs()))
            st["y"] = y if first else st["y"] + y
            if cb is not None:
                out_v[pl.ds(w0, BQ // 2), _cols(cb)] = _words(st["y"])
            return y

        def ctx_rows(t):
            return jnp.concatenate([ctx[pl.ds(w0 + u * (S // 2), BQ // 2), :]
                                    for u in (t, t + 1)], axis=1)

        def bwo_rows(cb, half):
            return jnp.concatenate([bwo_v[cb, pl.ds(j, H, stride=DH // 2), :]
                                    for j in range(8 * half, 8 * half + 8)], axis=0)

        for cb in range(8):
            for t in range(0, H // 2, 2):
                il.mxu(BQ, 4, functools.partial(ctx_rows, t), functools.partial(
                    step, lambda t=t, cb=cb: wo_v[128 * t:128 * t + 256, _cols(cb)],
                    t == 0, cb if t == H // 2 - 2 else None), "a")
        for cb in range(8):
            for half in range(2):
                il.mxu(BQ, 4, lambda half=half: o_s[0:BQ // 2, _cols(4 * half, 4)],
                       functools.partial(step, functools.partial(bwo_rows, cb, half),
                                         half == 0, 8 + cb if half else None), "b")
        fns = _mix_steps(pl.multiple_of(c * BQ, BQ), v_f, prob, o_s)
        fns.append((0, lambda hold: _fence(o_s, _zero(c))))
        il.vpu("begin", "b", fns, _read_back(o_s, _zero(c)))
        il.emit(0, CFG["blead"], CFG["mixat"])
        out_copy(c).start()
        return carry

    with _scope('L4'):
        lax.fori_loop(0, NQ, out_rows, 0)
    with _scope('w3'):
        for c in range(NQ):
            out_copy(c).wait()


def _kernel(x_hbm, c_hbm, wq_hbm, wuk_hbm, wuv_hbm, wo_hbm, bx_hbm, wqkv_hbm, bwo_hbm, out_hbm,
            x_v, c_v, wo_v, bwo_v, v_f, prob, wq_h, wk_h, wv_h, sems):
    vm = pltpu.VMEM
    copies = [pltpu.make_async_copy(src.bitcast(U32), dst, sems.at[n])
              for n, (src, dst) in enumerate(((x_hbm, x_v), (c_hbm, c_v), (wo_hbm, wo_v)))]
    copies += [pltpu.make_async_copy(bwo_hbm.bitcast(U32).at[:, pl.ds(128 * cb, 128)],
                                     bwo_v.at[cb, pl.ds(0, M // 2)], sems.at[3 + cb])
               for cb in range(8)]
    by_head = (wq_h, wk_h, wv_h)

    def start(cps):
        for cp in cps:
            cp.start()

    def wait(cps):
        for cp in cps:
            cp.wait()

    if CFG["only"] == "a": start(copies)
    else: pl.run_scoped(
        functools.partial(_project_b, bx_hbm, wqkv_hbm, (wq_hbm, wuk_hbm, wuv_hbm),
                          functools.partial(start, copies), v_f, prob, by_head),
        vm((2, S // 2, M // 2), U32), vm((6, M // 4, M), U32),
        vm((6, 4, H * WPITCH + CFG["wpad"], 128), U32), vm((16, HALO + S + CFG['kp'], 128), F32),
        vm((M * H // 2 + CFG['rp'], D), U32), vm((DC * H // 2 + CFG['rp'], D), U32),
        vm((DC * H // 2 + CFG['rp'], D), U32), pltpu.SemaphoreType.DMA((9,)),
        pltpu.SemaphoreType.DMA((4,)), pltpu.SemaphoreType.DMA((3,)))
    with _scope('w2'):
        wait(copies[:2])
    if CFG["only"] == "b":
        wait(copies[2:])
        def fin(o, sem):
            o[...] = wq_h[0, 0:8] ^ wk_h[0, 0:8] ^ wv_h[0, 0:8] ^ pltpu.bitcast(v_f[0, 0:8] + prob[0:8, 0:128], U32)
            cp = pltpu.make_async_copy(o, out_hbm.bitcast(U32).at[0:8, 0:128], sem); cp.start(); cp.wait()
        pl.run_scoped(fin, vm((8, 128), U32), pltpu.SemaphoreType.DMA(()))
    else: pl.run_scoped(
        functools.partial(_attend_and_project, x_v, c_v, by_head, wo_v, bwo_v, v_f, prob,
                          functools.partial(wait, copies[2:]), out_hbm),
        vm((H // 2 * S // 2, 2 * D), U32), vm((S // 2, 2 * M), U32), vm((BQ // 2 + 8, M), U32),
        vm((S // 2, 2 * D), U32), vm((S // 2, 2 * D), U32), vm((S // 2, 2 * D), U32),
        vm((2 * BQ + 8, S), F32), vm((2 * BQ + 8, S), F32),
        vm((BQ + 8, S + 2 * D), U32), vm((BQ + 8, S + 2 * D), U32),
        vm((BQ + 8, S + 2 * D), U32), pltpu.SemaphoreType.DMA((NQ,)))


@jax.jit
def pallas_concat_heads__compressed_kv_cla__sliding_local_dilated__prompt_kernel(
    A_x: jax.Array,
    A_c_kv: jax.Array,
    A_w_q: jax.Array,
    A_w_uk: jax.Array,
    A_w_uv: jax.Array,
    A_w_o: jax.Array,
    B_x: jax.Array,
    B_wqkv: jax.Array,
    B_wo: jax.Array,
):
    vm = pltpu.VMEM
    slots = H // 2 + 1
    pad = CFG["pad"]
    out = pl.pallas_call(
        _kernel,
        out_shape=jax.ShapeDtypeStruct((S, 2 * M), BF16),
        in_specs=[pl.BlockSpec(memory_space=pl.ANY)] * 9,
        out_specs=pl.BlockSpec(memory_space=pl.ANY),
        scratch_shapes=[
            vm((S // 2, M), U32), vm((S // 2, DC), U32), vm((H * D // 2, M), U32),
            vm((8, M // 2 + 16, 128), U32), vm((8, HALO + S, 128), F32), vm((S, W * 128), F32),
            vm((2, slots * (M // 2 + pad) + 24, D), U32),
            vm((2, slots * (DC // 2 + pad) + 24, D), U32),
            vm((2, slots * (DC // 2 + pad) + CFG['hp'], D), U32),
            pltpu.SemaphoreType.DMA((11,)),
        ],
        compiler_params=pltpu.CompilerParams(vmem_limit_bytes=124 * 1024 * 1024),
        name="concat_heads_attention",
    )(
        A_x.reshape(S, M), A_c_kv.reshape(S, DC),
        A_w_q.reshape(M * H, D), A_w_uk.reshape(DC * H, D), A_w_uv.reshape(DC * H, D),
        A_w_o.reshape(H * D, M), B_x.reshape(S, M), B_wqkv, B_wo,
    )
    return out.reshape(1, S, 2 * M)
```

```python
import contextlib
import functools
import math

import jax
import jax.numpy as jnp
from jax import lax
import jax.experimental.pallas as pl
import jax.experimental.pallas.tpu as pltpu

CFG = dict(na=16, R1=512, delay=400, lead=200, period=32, ahead=256, nextra=192, nshift=500,
           pad=8, fw=4, hp=16, pp=256, rp=32, xp=0, kp=0, op=256, vp=0, qp=0, blead=300, bperiod=16, mixat=32, only=None, scopes=False, wpad=16)

S = 2048
M = 1024
H = 32
D = 128
DC = 512
DH = 32
W = 8
DIL = 2
HALO = 16
BQ = 256
NQ = S // BQ
WPITCH = DH // 2 + 1
HPITCH = H + 8
LOG2E = math.log2(math.e)
NEG = -1e9 * LOG2E

F32 = jnp.float32
BF16 = jnp.bfloat16
U32 = jnp.uint32


def _scope(name):
    return jax.named_scope(name) if CFG["scopes"] else contextlib.nullcontext()


def _dot(a, b):
    return jnp.dot(a, b, preferred_element_type=F32)


def _dot_nt(a, b):
    return lax.dot_general(a, b, (((1,), (1,)), ((), ())), preferred_element_type=F32)


def _words(x):
    return pltpu.bitcast(x.astype(BF16), U32)


def _halves(w):
    return pltpu.bitcast(w, BF16)


def _recip(x):
    r = pl.reciprocal(x, approx=True)
    return r * (2.0 - x * r)


def _rows(r0, n):
    return slice(r0 // 2, (r0 + n) // 2)


def _cols(cb, n=1):
    return slice(128 * cb, 128 * (cb + n))


def _aligned(x, n):
    return x if isinstance(x, int) else pl.multiple_of(x, n)


def _zero(c):
    return pl.multiple_of((c >> 8) * 8, 8)


def _read_back(buf, row):
    return lambda: pltpu.bitcast(buf[pl.ds(row, 8), 0:128], U32)


def _fence(buf, zero):
    buf[pl.ds(zero + (buf.shape[0] - 8), 8), 0:128] = jnp.zeros((8, 128), buf.dtype)


class _Interleaver:
    def __init__(self, counter):
        self.never = counter < 0
        self.steps = []
        self.side = []

    def mxu(self, rows, tiles, lhs, fn, name):
        self.steps.append((rows, tiles, lhs, fn, name))

    def vpu(self, after, before, fns, token=None, until=None, shift=0):
        self.side.append((after, before, fns, token, until, shift))

    def emit(self, delay, lead, period):
        busy, starts, slots = [0] * 4, [], []
        start, end = {}, {"begin": -delay}
        for rows, tiles, _, _, name in self.steps:
            units = sorted(range(4), key=lambda u: busy[u])[:tiles]
            t0 = busy[units[0]]
            starts.append(t0)
            start.setdefault(name, t0)
            for u in units:
                busy[u] += rows
            end[name] = max([end.get(name, 0)] + [busy[u] for u in units])
            slots += [(t, len(starts) - 1) for t in range(t0 + period, t0 + rows + 1, period)
                      if not slots or t > slots[-1][0]]
        start["end"] = max(busy)
        todo = []
        for after, before, fns, token, until, shift in self.side:
            lo = min(end[after] + delay, start[before])
            hi = max(start[before] - lead, lo)
            if until is not None:
                hi = min(hi, end[until] + delay)
            total, done = sum(w for w, _ in fns), 0
            for w, fn in fns:
                when = lo + (hi - lo) * (done + w / 2) / total + shift
                todo.append((when, len(todo), fn, token, None if shift else before))
                done += w
        todo.sort(key=lambda e: e[:2])
        results = []

        def hold_at(now):
            def hold(x, extra=0):
                past = [y for t, y in results if t <= now - CFG["ahead"] - extra]
                if not past:
                    return x
                return jnp.where(
                    self.never, jnp.concatenate([past[-1]] * (x.shape[0] // 8), axis=0), x)

            return hold

        k = 0
        for n, ((rows, _, lhs, fn, name), t0) in enumerate(zip(self.steps, starts)):
            assert all(e[4] != name for e in todo[k:])
            words = lhs()
            slabs = [words[r:r + 8] for r in range(0, rows // 2, 8)]
            for t in [t for t, step in slots if step == n] if todo else []:
                tokens = []
                while k < len(todo) and todo[k][0] < t + period:
                    todo[k][2](hold_at(t))
                    if todo[k][3] is not None and todo[k][3] not in tokens:
                        tokens.append(todo[k][3])
                    k += 1
                u = (t - t0) // 16 - 1
                for token in [x for x in (token() for token in tokens) if x is not None]:
                    head = jnp.where(self.never, token, slabs[u][:, 0:128])
                    slabs[u] = (jnp.concatenate([head, slabs[u][:, 128:]], axis=1)
                                if words.shape[1] > 128 else head)
            y = fn(_halves(jnp.concatenate(slabs, axis=0)))
            results += [(t0 + r + 16, y[r:r + 8, 0:128]) for r in range(0, rows, 16)
                        if todo and (not results or t0 + r + 16 > results[-1][0])]
        for e in todo[k:]:
            e[2](hold_at(start["end"]))


def _regroup_steps(part, nparts, raw, by_head):
    def step(src, dst, r, t, hold):
        src[src.shape[0] - 8:, :] = pltpu.bitcast(hold(jnp.zeros((8, 128), F32)), U32)
        even, odd = (src[pl.ds(r * HPITCH + t + o, 8, stride=HPITCH), :] for o in (0, H // 2))
        dst[0, t, pl.ds(_aligned(r, 8), 8), :] = (even & jnp.uint32(0xFFFF)) | (odd << 16)
        dst[1, t, pl.ds(_aligned(r, 8), 8), :] = (even >> 16) | (odd & jnp.uint32(0xFFFF0000))

    fns = []
    for src, dst in zip(raw, by_head):
        n = dst.shape[2] // nparts
        src = src.reshape(src.shape[0] * HPITCH, D)
        fns += [(1, functools.partial(step, src, dst, part * n + r, t))
                for r in range(0, n, 8) for t in range(H // 2)]
    return fns


def _head_pair(t, x_v, c_v, wq_h, wk_h, wv_h, q_s, k_s, v_s, s_s, p_s, ctx):
    qscale = (D ** -0.5) * LOG2E
    row = lax.broadcasted_iota(jnp.int32, (128, 128), 0)
    col = lax.broadcasted_iota(jnp.int32, (128, 128), 1)
    tri = col <= row
    zero = _zero(t)
    ctx_row = pl.multiple_of(t * (S // 2), S // 2)
    st = {}
    il = _Interleaver(t)

    def weights(ref, h, r0):
        return _halves(ref[h, t, r0:r0 + 256, :])

    def proj_kv(w, dst, name, i):
        def step(h, cc):
            y = _dot(cc, weights(w, h, 0))
            dst[_rows(i * BQ, BQ), _cols(h)] = _words(y)
            return y

        for h in range(2):
            il.mxu(BQ, 4, lambda: c_v[_rows(i * BQ, BQ), :], functools.partial(step, h),
                   (name, i))

    proj_k = functools.partial(proj_kv, wk_h, k_s, "k")
    proj_v = functools.partial(proj_kv, wv_h, v_s, "v")

    def proj_q(i, h):
        r = _rows(i * BQ, BQ)

        def first(xx):
            st["q"] = _dot(xx, weights(wq_h, h, 0))
            return st["q"]

        def second(xx):
            y = _dot(xx, weights(wq_h, h, 256))
            q_s[r, _cols(h)] = _words((st.pop("q") + y) * qscale)
            return y

        il.mxu(BQ, 4, lambda: x_v[r, 0:512], first, ("q", i))
        il.mxu(BQ, 4, lambda: x_v[r, 512:1024], second, ("q", i))

    def pieces(i):
        n = 2 * i
        body = [(h, j, 4, 0, BQ) for h in range(2) for j in range(0, n - 3, 4)]
        if n % 4:
            body += [(h, n - 2, 2, 0, BQ) for h in range(2)]
        diag = ([(h, n, 1, 0, BQ) for h in range(2)]
                + [(h, n + 1, 1, 128, 128) for h in range(2)])
        return body, diag

    def scores(i, diag_first):
        left = {}

        def piece(h, j, n, a0, nr, q):
            s = _dot_nt(q, _halves(k_s[_rows(128 * j, 128 * n), _cols(h)]))
            for a in range(a0, a0 + nr, 64):
                m = st.get(("m", i, h, a))
                for u in range(n):
                    tile = s[a - a0:a - a0 + 64, _cols(u)]
                    if j + u == 2 * i + a // 128:
                        tile = jnp.where(tri[a % 128:a % 128 + 64], tile, NEG)
                    s_s[i % 2][BQ * h + a:BQ * h + a + 64, _cols(j + u)] = tile
                    m = tile if m is None else jnp.maximum(m, tile)
                left[h, a] -= n
                if left[h, a] == 0:
                    m = jnp.broadcast_to(jnp.max(m, axis=-1, keepdims=True), (64, 128))
                st["m", i, h, a] = m
            if not any(left[h, a] for a in range(0, BQ, 64)):
                _fence(s_s[i % 2], zero)
            return s

        body, diag = pieces(i)
        for h, j, n, a0, nr in (diag + body[::-1] if diag_first else body[::-1] + diag):
            for a in range(a0, a0 + nr, 64):
                left[h, a] = left.get((h, a), 0) + n
            il.mxu(nr, n, lambda h=h, a0=a0, nr=nr: q_s[_rows(i * BQ + a0, nr), _cols(h)],
                   functools.partial(piece, h, j, n, a0, nr), ("qk", i))

    def softmax(i, before, until):
        sb, pb = s_s[i % 2], p_s[i % 3]

        def unit(h, r0, j, last, hold):
            a = r0 // 64 * 64
            r = BQ * h + r0
            p = jnp.exp2(sb[r:r + 16, _cols(j)] - hold(st["m", i, h, a][r0 - a:r0 - a + 16]))
            l = st["l", i, h, r0] = p if j == 0 else st["l", i, h, r0] + p
            pb[_rows(r, 16), _cols(j)] = _words(p)
            if last:
                pb[r0:r0 + 16, _cols(S // 128 + h)] = pltpu.bitcast(l, U32)
                if r0 + 16 == BQ and h == 0:
                    _fence(pb, zero)

        def normalizer(h, r0, hold):
            l = hold(st.pop(("l", i, h, r0)), CFG["nextra"])
            st["inv", i, h, r0] = st["last", i] = jnp.broadcast_to(
                _recip(jnp.sum(l, axis=-1, keepdims=True)), (16, 128))

        def newest_normalizer():
            inv = st.pop(("last", i), None)
            return None if inv is None else pltpu.bitcast(inv[8:], U32)

        fns, norms = [], []
        for h in (1, 0):
            for r0 in range(0, BQ, 16):
                n = 2 * i + 1 + r0 // 128
                fns += [(1, functools.partial(unit, h, r0, j, j == n - 1)) for j in range(n)]
                norms += [(n, lambda hold: None), (0, functools.partial(normalizer, h, r0))]
        il.vpu(("qk", i), before, fns, _read_back(pb, zero + BQ // 2), until)
        il.vpu(("qk", i), before, norms, newest_normalizer, until, CFG["nshift"])

    def context(i, diag_first):
        left = {}

        def probs(h, j, n, a0, nr):
            return p_s[i % 3][_rows(BQ * h + a0, nr), _cols(j, n)]

        def piece(h, j, n, a0, nr, p):
            o = _dot(p, _halves(v_s[_rows(128 * j, 128 * n), _cols(h)]))
            for a in range(a0, a0 + nr, 64):
                part = o[a - a0:a - a0 + 64]
                prev = st.pop(("o", h, a), None)
                part = part if prev is None else prev + part
                left[h, a] -= n
                if left[h, a] == 0:
                    inv = jnp.concatenate(
                        [st.pop(("inv", i, h, r0)) for r0 in range(a, a + 64, 16)], axis=0)
                    ctx[pl.ds(ctx_row + (i * BQ + a) // 2, 32), _cols(h)] = _words(part * inv)
                else:
                    st["o", h, a] = part
            return o

        body, diag = pieces(i)
        for h, j, n, a0, nr in (diag + body[::-1] if diag_first else body + diag):
            for a in range(a0, a0 + nr, 64):
                left[h, a] = left.get((h, a), 0) + n
            il.mxu(nr, n, functools.partial(probs, h, j, n, a0, nr),
                   functools.partial(piece, h, j, n, a0, nr), ("pv", i))
        if i < NQ - 1:
            il.vpu(("pv", i), "end", [(1, lambda hold: None)],
                   _read_back(ctx, ctx_row + zero), ("pv", i))

    for i in range(2):
        proj_q(i, 0)
        proj_k(i)
        proj_q(i, 1)
    proj_v(0)
    scores(0, True)
    softmax(0, ("v", 1), None)
    for i in range(1, NQ - 1):
        scores(i, True)
        softmax(i, ("v", i + 1), ("qk", i + 1))
        proj_k(i + 1)
        proj_q(i + 1, 0)
        proj_q(i + 1, 1)
        proj_v(i)
        if i < NQ - 2:
            context(i - 1, False)
    scores(NQ - 1, False)
    softmax(NQ - 1, ("pv", NQ - 1), None)
    context(NQ - 3, True)
    proj_v(NQ - 1)
    context(NQ - 2, False)
    context(NQ - 1, True)
    il.emit(CFG["delay"], CFG["lead"], CFG["period"])


def _transposed_weights(group, mb, w_v):
    r = pl.ds(_aligned(64 * mb, 64), 64)
    out = []
    for cb in range(8):
        tt = pltpu.bitcast(_halves(w_v[group, r, _cols(cb)]).T, U32)
        out += [((4 * cb + hl) * WPITCH, tt[16 * hl:16 * hl + 16]) for hl in range(4)]
    return out


def _b_weights(wt, group, cb):
    return _halves(jnp.concatenate(
        [jnp.concatenate([wt[group, mb, pl.ds(j, H, stride=WPITCH), :]
                          for j in (2 * cb, 2 * cb + 1)], axis=0) for mb in range(4)], axis=1))


def _taps(buf, cb, row, w):
    back = DIL * W // 2
    x = buf[cb, pl.ds(row + (HALO - back - DIL * w), 16 + back), :]
    return x[back:], x[:16]


def _prob_steps(row0, nrows, qk_f, prob):
    st = {}
    even = lax.broadcasted_iota(jnp.int32, (16, 128), 1) % 2 == 0

    def products(r0, cb, hold):
        q = hold(qk_f[cb, pl.ds(pl.multiple_of(row0 + (HALO + r0), 8), 16), :])
        near, far = zip(*[_taps(qk_f, 8 + cb, row0 + r0, w) for w in range(W // 2)])
        sums = [q * k if cb == 0 else st[r0][w] + q * k for w, k in enumerate(near + far)]
        st[r0] = [a + pltpu.roll(a, 64, 1) for a in sums] if cb == 7 else sums

    def finish(r0, hold):
        logits = []
        for w, a in enumerate(st.pop(r0)):
            a = a + jnp.where(even, pltpu.roll(a, 127, 1), pltpu.roll(a, 1, 1))
            if r0 < DIL * w:
                pos = row0 + r0 + lax.broadcasted_iota(jnp.int32, (16, 128), 0)
                a = jnp.where(pos >= DIL * w, a, NEG)
            logits.append(a)
        m = functools.reduce(jnp.maximum, logits)
        ps = [jnp.exp2(a - m) for a in logits]
        inv = _recip(functools.reduce(jnp.add, ps))
        for w in range(W):
            prob[pl.ds(pl.multiple_of(row0 + r0, 16), 16), _cols(w)] = ps[w] * inv

    fns = []
    for r0 in range(0, nrows + 16, 16):
        if r0 < nrows:
            fns += [(1, functools.partial(products, r0, cb)) for cb in range(8)]
        if r0:
            fns.append((CFG["fw"], functools.partial(finish, r0 - 16)))
    return fns


def _mix_steps(row0, v_f, prob, o_s):
    st = {}

    def step(r0, w, cb, hold):
        if cb == 0:
            r = pl.ds(pl.multiple_of(row0 + r0, 16), 16)
            st["p"] = [hold(prob[r, _cols(u)]) for u in (w, w + W // 2)]
        near, far = _taps(v_f, cb, row0 + r0, w)
        a = st["p"][0] * near + st["p"][1] * far
        st[cb] = a if w == 0 else st[cb] + a
        if w == W // 2 - 1:
            o_s[_rows(r0, 16), _cols(cb)] = _words(st[cb])

    return [(1, functools.partial(step, r0, w, cb))
            for r0 in range(0, BQ, 16) for w in range(W // 2) for cb in range(8)]


def _project_b(bx_hbm, wqkv_hbm, raw_hbm, start_other_copies, v_f, prob, by_head,
               bx_v, w_v, wt, qk_f, wq_v, wk_v, wv_v, w_sems, x_sems, raw_sems):
    R1 = CFG["R1"]
    bscale = (DH ** -0.5) * LOG2E
    raw = (wq_v, wk_v, wv_v)

    def w_copy(group, r0, n, sem):
        src = wqkv_hbm.bitcast(U32).at[pl.ds(_aligned((group & 1) * 256 + r0, 64), n),
                                       pl.ds(_aligned((group >> 1) * M, M), M)]
        return pltpu.make_async_copy(src, w_v.at[group, pl.ds(_aligned(r0, 64), n)],
                                     w_sems.at[sem])

    def x_copy(n):
        r = pl.ds(_aligned((n & 1) * 512, 512), 512)
        src = bx_hbm.bitcast(U32).at[r, pl.ds(_aligned((n >> 1) * 512, 512), 512)]
        return pltpu.make_async_copy(src, bx_v.at[n >> 1, r], x_sems.at[n])

    raw_copies = [
        pltpu.make_async_copy(src.bitcast(U32), dst.at[pl.ds(0, src.shape[0]), pl.ds(0, H)],
                              raw_sems.at[n])
        for n, (src, dst) in enumerate(zip(raw_hbm, raw))]

    for mb in range(4):
        w_copy(0, 64 * mb, 64, mb).start()
    for n in range(6):
        if n < 4:
            x_copy(n).start()
        if n:
            w_copy(n, 0, 256, 3 + n).start()
    for cp in raw_copies:
        cp.start()
    start_other_copies()
    qk_f[8:16, 0:HALO, :] = jnp.zeros((8, HALO, 128), F32)
    v_f[:, 0:HALO, :] = jnp.zeros((8, HALO, 128), F32)
    prob[0:8, 0:128] = jnp.zeros((8, 128), F32)

    def first_weights(mb, carry):
        w_copy(0, 64 * mb, 64, mb).wait()
        for r, x in _transposed_weights(0, mb, w_v):
            wt[0, mb, r:r + 16, :] = x
        return carry

    with _scope('w0'):
        lax.fori_loop(0, 4, first_weights, 0)

    def qk_rows(n, carry):
        upcoming = jnp.minimum(n, 5)

        @pl.when(n < 4)
        def _():
            x_copy(n).wait()

        @pl.when((n >= 1) & (n <= 5))
        def _():
            w_copy(n, 0, 256, 3 + n).wait()

        scale = jnp.where(n < 4, bscale, 1.0)
        for r0 in range(0, S // 2, BQ):
            row = pl.multiple_of((n & 1) * (S // 2) + r0, BQ)
            x = _halves(bx_v[(n >> 1) & 1, pl.ds(pl.multiple_of(row >> 1, 128), 128), :])
            r = pl.ds(pl.multiple_of(row + HALO, 8), BQ)
            for cb in range(8):
                o = 8 * (n >> 2) + cb
                y = _dot_nt(x, _b_weights(wt, n >> 1, cb)) * scale
                qk_f[o, r, :] = jnp.where((n & 2) != 0, qk_f[o, r, :], 0.0) + y
        for mb, tiles in [(mb, _transposed_weights(upcoming, mb, w_v)) for mb in range(4)]:
            for r, x in tiles:
                wt[upcoming, mb, r:r + 16, :] = x
        return carry

    with _scope('L0'):
        lax.fori_loop(0, 8, qk_rows, 0)
    with _scope('w1'):
        for cp in raw_copies:
            cp.wait()

    def v_rows(c, carry):
        il = _Interleaver(c)
        row0 = pl.multiple_of(c * R1, R1)
        st = {}

        def first(cb, xx):
            st["y"] = _dot_nt(xx, _b_weights(wt, 4, cb))
            return st["y"]

        def second(cb, r, xx):
            y = _dot_nt(xx, _b_weights(wt, 5, cb))
            v_f[cb, r, :] = st.pop("y") + y
            return y

        for r0 in range(0, R1, BQ):
            rw = pl.ds(pl.multiple_of((row0 + r0) >> 1, 128), 128)
            r = pl.ds(pl.multiple_of(row0 + (HALO + r0), 8), BQ)
            for cb in range(8):
                il.mxu(BQ, 4, lambda rw=rw: bx_v[0, rw, :], functools.partial(first, cb), "v")
                il.mxu(BQ, 4, lambda rw=rw: bx_v[1, rw, :], functools.partial(second, cb, r),
                       "v")
        il.vpu("begin", "end", _prob_steps(row0, R1, qk_f, prob), _read_back(prob, _zero(c)))
        il.vpu("begin", "end", _regroup_steps(c, S // R1, raw, by_head))
        il.emit(0, CFG["blead"], CFG["bperiod"])
        return carry

    with _scope('L1'):
        lax.fori_loop(0, S // R1, v_rows, 0)


def _attend_and_project(x_v, c_v, by_head, wo_v, bwo_v, v_f, prob, wait_for_output_weights,
                        out_hbm, o_s, ctx, out_v, q_s, k_s, v_s, s_a, s_b, p_a, p_b, p_c, sems):
    def head_pair(t, carry):
        with _scope('it'):
            _head_pair(t, x_v, c_v, *by_head, q_s, k_s, v_s, (s_a, s_b), (p_a, p_b, p_c), ctx)
        return carry

    o_s[0:8, 0:128] = jnp.zeros((8, 128), U32)
    with _scope('LA'):
        lax.fori_loop(0, CFG["na"], head_pair, 0)
    wait_for_output_weights()

    def out_copy(c):
        r = pl.ds(_aligned(c * (BQ // 2), BQ // 2), BQ // 2)
        return pltpu.make_async_copy(out_v.at[r], out_hbm.bitcast(U32).at[r], sems.at[c])

    def out_rows(c, carry):
        il = _Interleaver(c)
        w0 = pl.multiple_of(c * (BQ // 2), BQ // 2)
        st = {}

        def step(rhs, first, cb, lhs):
            y = _dot(lhs, _halves(rhs()))
            st["y"] = y if first else st["y"] + y
            if cb is not None:
                out_v[pl.ds(w0, BQ // 2), _cols(cb)] = _words(st["y"])
            return y

        def ctx_rows(t):
            return jnp.concatenate([ctx[pl.ds(w0 + u * (S // 2), BQ // 2), :]
                                    for u in (t, t + 1)], axis=1)

        def bwo_rows(cb, half):
            return jnp.concatenate([bwo_v[cb, pl.ds(j, H, stride=DH // 2), :]
                                    for j in range(8 * half, 8 * half + 8)], axis=0)

        for cb in range(8):
            for t in range(0, H // 2, 2):
                il.mxu(BQ, 4, functools.partial(ctx_rows, t), functools.partial(
                    step, lambda t=t, cb=cb: wo_v[128 * t:128 * t + 256, _cols(cb)],
                    t == 0, cb if t == H // 2 - 2 else None), "a")
        for cb in range(8):
            for half in range(2):
                il.mxu(BQ, 4, lambda half=half: o_s[0:BQ // 2, _cols(4 * half, 4)],
                       functools.partial(step, functools.partial(bwo_rows, cb, half),
                                         half == 0, 8 + cb if half else None), "b")
        fns = _mix_steps(pl.multiple_of(c * BQ, BQ), v_f, prob, o_s)
        fns.append((0, lambda hold: _fence(o_s, _zero(c))))
        il.vpu("begin", "b", fns, _read_back(o_s, _zero(c)))
        il.emit(0, CFG["blead"], CFG["mixat"])
        out_copy(c).start()
        return carry

    with _scope('L4'):
        lax.fori_loop(0, NQ, out_rows, 0)
    with _scope('w3'):
        for c in range(NQ):
            out_copy(c).wait()


def _kernel(x_hbm, c_hbm, wq_hbm, wuk_hbm, wuv_hbm, wo_hbm, bx_hbm, wqkv_hbm, bwo_hbm, out_hbm,
            x_v, c_v, wo_v, bwo_v, v_f, prob, wq_h, wk_h, wv_h, o_s, sems):
    vm = pltpu.VMEM
    copies = [pltpu.make_async_copy(src.bitcast(U32), dst, sems.at[n])
              for n, (src, dst) in enumerate(((x_hbm, x_v), (c_hbm, c_v), (wo_hbm, wo_v)))]
    copies += [pltpu.make_async_copy(bwo_hbm.bitcast(U32).at[:, pl.ds(128 * cb, 128)],
                                     bwo_v.at[cb, pl.ds(0, M // 2)], sems.at[3 + cb])
               for cb in range(8)]
    by_head = (wq_h, wk_h, wv_h)

    def start(cps):
        for cp in cps:
            cp.start()

    def wait(cps):
        for cp in cps:
            cp.wait()

    if CFG["only"] == "a": start(copies)
    else: pl.run_scoped(
        functools.partial(_project_b, bx_hbm, wqkv_hbm, (wq_hbm, wuk_hbm, wuv_hbm),
                          functools.partial(start, copies), v_f, prob, by_head),
        vm((2, S // 2, M // 2), U32), vm((6, M // 4, M), U32),
        vm((6, 4, H * WPITCH + CFG["wpad"], 128), U32), vm((16, HALO + S + CFG['kp'], 128), F32),
        vm((M // 2 + 4, HPITCH, D), U32), vm((DC // 2 + 4, HPITCH, D), U32),
        vm((DC // 2 + 4, HPITCH, D), U32), pltpu.SemaphoreType.DMA((9,)),
        pltpu.SemaphoreType.DMA((4,)), pltpu.SemaphoreType.DMA((3,)))
    with _scope('w2'):
        wait(copies[:2])
    if CFG["only"] == "b":
        wait(copies[2:])
        def fin(o, sem):
            o[...] = wq_h[0, 0, 0:8] ^ wk_h[0, 0, 0:8] ^ wv_h[0, 0, 0:8] ^ pltpu.bitcast(v_f[0, 0:8] + prob[0:8, 0:128], U32)
            cp = pltpu.make_async_copy(o, out_hbm.bitcast(U32).at[0:8, 0:128], sem); cp.start(); cp.wait()
        pl.run_scoped(fin, vm((8, 128), U32), pltpu.SemaphoreType.DMA(()))
    else: pl.run_scoped(
        functools.partial(_attend_and_project, x_v, c_v, by_head, wo_v, bwo_v, v_f, prob,
                          functools.partial(wait, copies[2:]), out_hbm, o_s),
        vm((H // 2 * S // 2, 2 * D), U32), vm((S // 2, 2 * M), U32),
        vm((S // 2, 2 * D), U32), vm((S // 2, 2 * D), U32), vm((S // 2, 2 * D), U32),
        vm((2 * BQ + 8, S), F32), vm((2 * BQ + 8, S), F32),
        vm((BQ + 8, S + 2 * D), U32), vm((BQ + 8, S + 2 * D), U32),
        vm((BQ + 8, S + 2 * D), U32), pltpu.SemaphoreType.DMA((NQ,)))


@jax.jit
def pallas_concat_heads__compressed_kv_cla__sliding_local_dilated__prompt_kernel(
    A_x: jax.Array,
    A_c_kv: jax.Array,
    A_w_q: jax.Array,
    A_w_uk: jax.Array,
    A_w_uv: jax.Array,
    A_w_o: jax.Array,
    B_x: jax.Array,
    B_wqkv: jax.Array,
    B_wo: jax.Array,
):
    vm = pltpu.VMEM
    out = pl.pallas_call(
        _kernel,
        out_shape=jax.ShapeDtypeStruct((S, 2 * M), BF16),
        in_specs=[pl.BlockSpec(memory_space=pl.ANY)] * 9,
        out_specs=pl.BlockSpec(memory_space=pl.ANY),
        scratch_shapes=[
            vm((S // 2, M), U32), vm((S // 2, DC), U32), vm((H * D // 2, M), U32),
            vm((8, M // 2 + 16, 128), U32), vm((8, HALO + S, 128), F32), vm((S, W * 128), F32),
            vm((2, H // 2, M // 2, D), U32), vm((2, H // 2, DC // 2, D), U32),
            vm((2, H // 2, DC // 2, D), U32), vm((BQ // 2 + 8, M + CFG['op']), U32),
            pltpu.SemaphoreType.DMA((11,)),
        ],
        compiler_params=pltpu.CompilerParams(vmem_limit_bytes=124 * 1024 * 1024),
        name="concat_heads_attention",
    )(
        A_x.reshape(S, M), A_c_kv.reshape(S, DC),
        A_w_q.reshape(M // 2, 2 * H, D), A_w_uk.reshape(DC // 2, 2 * H, D),
        A_w_uv.reshape(DC // 2, 2 * H, D),
        A_w_o.reshape(H * D, M), B_x.reshape(S, M), B_wqkv, B_wo,
    )
    return out.reshape(1, S, 2 * M)
```

```python
import functools
import math

import jax
import jax.numpy as jnp
from jax import lax
import jax.experimental.pallas as pl
import jax.experimental.pallas.tpu as pltpu

S = 2048
M = 1024
H = 32
D = 128
DC = 512
DH = 32
W = 8
DIL = 2
HALO = 16
BQ = 256
NQ = S // BQ
RV = 512
RB = S // (H // 2)
WPITCH = DH // 2 + 1
HPITCH = H + 8
LOG2E = math.log2(math.e)
NEG = -1e9 * LOG2E

F32 = jnp.float32
BF16 = jnp.bfloat16
U32 = jnp.uint32


def _dot(a, b):
    return jnp.dot(a, b, preferred_element_type=F32)


def _dot_nt(a, b):
    return lax.dot_general(a, b, (((1,), (1,)), ((), ())), preferred_element_type=F32)


def _words(x):
    return pltpu.bitcast(x.astype(BF16), U32)


def _halves(w):
    return pltpu.bitcast(w, BF16)


def _recip(x):
    r = pl.reciprocal(x, approx=True)
    return r * (2.0 - x * r)


def _rows(r0, n):
    return slice(r0 // 2, (r0 + n) // 2)


def _cols(cb, n=1):
    return slice(128 * cb, 128 * (cb + n))


def _aligned(x, n):
    return x if isinstance(x, int) else pl.multiple_of(x, n)


def _zero(c):
    return pl.multiple_of((c >> 8) * 8, 8)


def _read_back(buf, row):
    return lambda: pltpu.bitcast(buf[pl.ds(row, 8), 0:128], U32)


def _fence(buf, zero):
    buf[pl.ds(zero + (buf.shape[0] - 8), 8), 0:128] = jnp.zeros((8, 128), buf.dtype)


class _Interleaver:
    def __init__(self, counter):
        self.never = counter < 0
        self.steps = []
        self.side = []

    def mxu(self, rows, tiles, lhs, fn, name):
        self.steps.append((rows, tiles, lhs, fn, name))

    def vpu(self, after, before, fns, token=None, until=None, shift=0):
        self.side.append((after, before, fns, token, until, shift))

    def emit(self, delay, lead, period):
        busy, starts, slots = [0] * 4, [], []
        start, end = {}, {"begin": -delay}
        for rows, tiles, _, _, name in self.steps:
            units = sorted(range(4), key=lambda u: busy[u])[:tiles]
            t0 = busy[units[0]]
            starts.append(t0)
            start.setdefault(name, t0)
            for u in units:
                busy[u] += rows
            end[name] = max([end.get(name, 0)] + [busy[u] for u in units])
            slots += [(t, len(starts) - 1) for t in range(t0 + period, t0 + rows + 1, period)
                      if not slots or t > slots[-1][0]]
        start["end"] = max(busy)
        todo = []
        for after, before, fns, token, until, shift in self.side:
            lo = min(end[after] + delay, start[before])
            hi = max(start[before] - lead, lo)
            if until is not None:
                hi = min(hi, end[until] + delay)
            total, done = sum(w for w, _ in fns), 0
            for w, fn in fns:
                when = lo + (hi - lo) * (done + w / 2) / total + shift
                todo.append((when, len(todo), fn, token, None if shift else before))
                done += w
        todo.sort(key=lambda e: e[:2])
        results = []

        def hold_at(now):
            def hold(x, extra=0):
                past = [y for t, y in results if t <= now - 256 - extra]
                if not past:
                    return x
                return jnp.where(
                    self.never, jnp.concatenate([past[-1]] * (x.shape[0] // 8), axis=0), x)

            return hold

        k = 0
        for n, ((rows, _, lhs, fn, name), t0) in enumerate(zip(self.steps, starts)):
            assert all(e[4] != name for e in todo[k:])
            words = lhs()
            slabs = [words[r:r + 8] for r in range(0, rows // 2, 8)]
            for t in [t for t, step in slots if step == n] if todo else []:
                tokens = []
                while k < len(todo) and todo[k][0] < t + period:
                    todo[k][2](hold_at(t))
                    if todo[k][3] is not None and todo[k][3] not in tokens:
                        tokens.append(todo[k][3])
                    k += 1
                u = (t - t0) // 16 - 1
                for token in [x for x in (token() for token in tokens) if x is not None]:
                    head = jnp.where(self.never, token, slabs[u][:, 0:128])
                    slabs[u] = (jnp.concatenate([head, slabs[u][:, 128:]], axis=1)
                                if words.shape[1] > 128 else head)
            y = fn(_halves(jnp.concatenate(slabs, axis=0)))
            results += [(t0 + r + 16, y[r:r + 8, 0:128]) for r in range(0, rows, 16)
                        if todo and (not results or t0 + r + 16 > results[-1][0])]
        for e in todo[k:]:
            e[2](hold_at(start["end"]))


def _regroup_steps(part, nparts, raw, by_head):
    def step(src, dst, r, t, hold):
        src[src.shape[0] - 8:, :] = pltpu.bitcast(hold(jnp.zeros((8, 128), F32)), U32)
        even, odd = (src[pl.ds(r * HPITCH + t + o, 8, stride=HPITCH), :] for o in (0, H // 2))
        dst[0, t, pl.ds(_aligned(r, 8), 8), :] = (even & jnp.uint32(0xFFFF)) | (odd << 16)
        dst[1, t, pl.ds(_aligned(r, 8), 8), :] = (even >> 16) | (odd & jnp.uint32(0xFFFF0000))

    fns = []
    for src, dst in zip(raw, by_head):
        n = dst.shape[2] // nparts
        src = src.reshape(src.shape[0] * HPITCH, D)
        fns += [(1, functools.partial(step, src, dst, part * n + r, t))
                for r in range(0, n, 8) for t in range(H // 2)]
    return fns


def _head_pair(t, il, x_v, c_v, wq_h, wk_h, wv_h, q_s, k_s, v_s, s_s, p_s, ctx, other_steps):
    qscale = (D ** -0.5) * LOG2E
    row = lax.broadcasted_iota(jnp.int32, (128, 128), 0)
    col = lax.broadcasted_iota(jnp.int32, (128, 128), 1)
    tri = col <= row
    zero = _zero(t)
    ctx_row = pl.multiple_of(t * (S // 2), S // 2)
    st = {}

    def weights(ref, h, r0):
        return _halves(ref[h, t, r0:r0 + 256, :])

    def proj_kv(w, dst, name, i):
        def step(h, cc):
            y = _dot(cc, weights(w, h, 0))
            dst[_rows(i * BQ, BQ), _cols(h)] = _words(y)
            return y

        for h in range(2):
            il.mxu(BQ, 4, lambda: c_v[_rows(i * BQ, BQ), :], functools.partial(step, h),
                   (name, i))

    proj_k = functools.partial(proj_kv, wk_h, k_s, "k")
    proj_v = functools.partial(proj_kv, wv_h, v_s, "v")

    def proj_q(i, h):
        r = _rows(i * BQ, BQ)

        def first(xx):
            st["q"] = _dot(xx, weights(wq_h, h, 0))
            return st["q"]

        def second(xx):
            y = _dot(xx, weights(wq_h, h, 256))
            q_s[r, _cols(h)] = _words((st.pop("q") + y) * qscale)
            return y

        il.mxu(BQ, 4, lambda: x_v[r, 0:512], first, ("q", i))
        il.mxu(BQ, 4, lambda: x_v[r, 512:1024], second, ("q", i))

    def pieces(i):
        n = 2 * i
        body = [(h, j, 4, 0, BQ) for h in range(2) for j in range(0, n - 3, 4)]
        if n % 4:
            body += [(h, n - 2, 2, 0, BQ) for h in range(2)]
        diag = ([(h, n, 1, 0, BQ) for h in range(2)]
                + [(h, n + 1, 1, 128, 128) for h in range(2)])
        return body, diag

    def scores(i, diag_first):
        left = {}

        def piece(h, j, n, a0, nr, q):
            s = _dot_nt(q, _halves(k_s[_rows(128 * j, 128 * n), _cols(h)]))
            for a in range(a0, a0 + nr, 64):
                m = st.get(("m", i, h, a))
                for u in range(n):
                    tile = s[a - a0:a - a0 + 64, _cols(u)]
                    if j + u == 2 * i + a // 128:
                        tile = jnp.where(tri[a % 128:a % 128 + 64], tile, NEG)
                    s_s[i % 2][BQ * h + a:BQ * h + a + 64, _cols(j + u)] = tile
                    m = tile if m is None else jnp.maximum(m, tile)
                left[h, a] -= n
                if left[h, a] == 0:
                    m = jnp.broadcast_to(jnp.max(m, axis=-1, keepdims=True), (64, 128))
                st["m", i, h, a] = m
            if not any(left[h, a] for a in range(0, BQ, 64)):
                _fence(s_s[i % 2], zero)
            return s

        body, diag = pieces(i)
        for h, j, n, a0, nr in (diag + body[::-1] if diag_first else body[::-1] + diag):
            for a in range(a0, a0 + nr, 64):
                left[h, a] = left.get((h, a), 0) + n
            il.mxu(nr, n, lambda h=h, a0=a0, nr=nr: q_s[_rows(i * BQ + a0, nr), _cols(h)],
                   functools.partial(piece, h, j, n, a0, nr), ("qk", i))

    def softmax(i, before, until):
        sb, pb = s_s[i % 2], p_s[i % 3]

        def unit(h, r0, j, last, hold):
            a = r0 // 64 * 64
            r = BQ * h + r0
            p = jnp.exp2(sb[r:r + 16, _cols(j)] - hold(st["m", i, h, a][r0 - a:r0 - a + 16]))
            l = st["l", i, h, r0] = p if j == 0 else st["l", i, h, r0] + p
            pb[_rows(r, 16), _cols(j)] = _words(p)
            if last:
                pb[r0:r0 + 16, _cols(S // 128 + h)] = pltpu.bitcast(l, U32)
                if r0 + 16 == BQ and h == 0:
                    _fence(pb, zero)

        def normalizer(h, r0, hold):
            l = hold(st.pop(("l", i, h, r0)), 192)
            st["inv", i, h, r0] = st["last", i] = jnp.broadcast_to(
                _recip(jnp.sum(l, axis=-1, keepdims=True)), (16, 128))

        def newest_normalizer():
            inv = st.pop(("last", i), None)
            return None if inv is None else pltpu.bitcast(inv[8:], U32)

        fns, norms = [], []
        for h in (1, 0):
            for r0 in range(0, BQ, 16):
                n = 2 * i + 1 + r0 // 128
                fns += [(1, functools.partial(unit, h, r0, j, j == n - 1)) for j in range(n)]
                norms += [(n, lambda hold: None), (0, functools.partial(normalizer, h, r0))]
        il.vpu(("qk", i), before, fns, _read_back(pb, zero + BQ // 2), until)
        il.vpu(("qk", i), before, norms, newest_normalizer, until, 500)

    def context(i, diag_first):
        left = {}

        def probs(h, j, n, a0, nr):
            return p_s[i % 3][_rows(BQ * h + a0, nr), _cols(j, n)]

        def piece(h, j, n, a0, nr, p):
            o = _dot(p, _halves(v_s[_rows(128 * j, 128 * n), _cols(h)]))
            for a in range(a0, a0 + nr, 64):
                part = o[a - a0:a - a0 + 64]
                prev = st.pop(("o", h, a), None)
                part = part if prev is None else prev + part
                left[h, a] -= n
                if left[h, a] == 0:
                    inv = jnp.concatenate(
                        [st.pop(("inv", i, h, r0)) for r0 in range(a, a + 64, 16)], axis=0)
                    ctx[pl.ds(ctx_row + (i * BQ + a) // 2, 32), _cols(h)] = _words(part * inv)
                else:
                    st["o", h, a] = part
            return o

        body, diag = pieces(i)
        for h, j, n, a0, nr in (diag + body[::-1] if diag_first else body + diag):
            for a in range(a0, a0 + nr, 64):
                left[h, a] = left.get((h, a), 0) + n
            il.mxu(nr, n, functools.partial(probs, h, j, n, a0, nr),
                   functools.partial(piece, h, j, n, a0, nr), ("pv", i))
        if i < NQ - 1:
            il.vpu(("pv", i), "end", [(1, lambda hold: None)],
                   _read_back(ctx, ctx_row + zero), ("pv", i))

    for i in range(2):
        proj_q(i, 0)
        proj_k(i)
        proj_q(i, 1)
    proj_v(0)
    scores(0, True)
    softmax(0, ("v", 1), None)
    for i in range(1, NQ - 1):
        scores(i, True)
        softmax(i, ("v", i + 1), ("qk", i + 1))
        proj_k(i + 1)
        proj_q(i + 1, 0)
        proj_q(i + 1, 1)
        proj_v(i)
        if i == NQ - 2:
            other_steps()
        if i < NQ - 2:
            context(i - 1, False)
    scores(NQ - 1, False)
    softmax(NQ - 1, ("pv", NQ - 1), None)
    context(NQ - 3, True)
    proj_v(NQ - 1)
    context(NQ - 2, False)
    context(NQ - 1, True)


def _transposed_weights(group, mb, w_v):
    r = pl.ds(_aligned(64 * mb, 64), 64)
    out = []
    for cb in range(8):
        tt = pltpu.bitcast(_halves(w_v[group, r, _cols(cb)]).T, U32)
        out += [((4 * cb + hl) * WPITCH, tt[16 * hl:16 * hl + 16]) for hl in range(4)]
    return out


def _b_weights(wt, group, cb):
    return _halves(jnp.concatenate(
        [jnp.concatenate([wt[group, mb, pl.ds(j, H, stride=WPITCH), :]
                          for j in (2 * cb, 2 * cb + 1)], axis=0) for mb in range(4)], axis=1))


def _taps(buf, cb, row, w):
    back = DIL * W // 2
    x = buf[cb, pl.ds(row + (HALO - back - DIL * w), 16 + back), :]
    return x[back:], x[:16]


def _prob_steps(row0, nrows, qk_f, prob):
    st = {}
    even = lax.broadcasted_iota(jnp.int32, (16, 128), 1) % 2 == 0

    def products(r0, cb, hold):
        q = hold(qk_f[cb, pl.ds(pl.multiple_of(row0 + (HALO + r0), 8), 16), :])
        near, far = zip(*[_taps(qk_f, 8 + cb, row0 + r0, w) for w in range(W // 2)])
        sums = [q * k if cb == 0 else st[r0][w] + q * k for w, k in enumerate(near + far)]
        st[r0] = [a + pltpu.roll(a, 64, 1) for a in sums] if cb == 7 else sums

    def finish(r0, hold):
        logits = []
        for w, a in enumerate(st.pop(r0)):
            a = a + jnp.where(even, pltpu.roll(a, 127, 1), pltpu.roll(a, 1, 1))
            if r0 < DIL * w:
                pos = row0 + r0 + lax.broadcasted_iota(jnp.int32, (16, 128), 0)
                a = jnp.where(pos >= DIL * w, a, NEG)
            logits.append(a)
        m = functools.reduce(jnp.maximum, logits)
        ps = [jnp.exp2(a - m) for a in logits]
        inv = _recip(functools.reduce(jnp.add, ps))
        for w in range(W):
            prob[pl.ds(pl.multiple_of(row0 + r0, 16), 16), _cols(w)] = ps[w] * inv

    fns = []
    for r0 in range(0, nrows + 16, 16):
        if r0 < nrows:
            fns += [(1, functools.partial(products, r0, cb)) for cb in range(8)]
        if r0:
            fns.append((4, functools.partial(finish, r0 - 16)))
    return fns


def _mix_steps(row0, nrows, v_f, prob, o_s):
    st = {}

    def step(r0, w, cb, hold):
        if cb == 0:
            r = pl.ds(pl.multiple_of(row0 + r0, 16), 16)
            st["p"] = [hold(prob[r, _cols(u)]) for u in (w, w + W // 2)]
        near, far = _taps(v_f, cb, row0 + r0, w)
        a = st["p"][0] * near + st["p"][1] * far
        st[cb] = a if w == 0 else st[cb] + a
        if w == W // 2 - 1:
            o_s[_rows(r0, 16), _cols(cb)] = _words(st[cb])

    return [(1, functools.partial(step, r0, w, cb))
            for r0 in range(0, nrows, 16) for w in range(W // 2) for cb in range(8)]


def _project_b(bx_hbm, wqkv_hbm, raw_hbm, start_other_copies, v_f, prob, by_head,
               bx_v, w_v, wt, qk_f, wq_v, wk_v, wv_v, w_sems, x_sems, raw_sems):
    bscale = (DH ** -0.5) * LOG2E
    raw = (wq_v, wk_v, wv_v)

    def w_copy(group, r0, n, sem):
        src = wqkv_hbm.bitcast(U32).at[pl.ds(_aligned((group & 1) * 256 + r0, 64), n),
                                       pl.ds(_aligned((group >> 1) * M, M), M)]
        return pltpu.make_async_copy(src, w_v.at[group, pl.ds(_aligned(r0, 64), n)],
                                     w_sems.at[sem])

    def x_copy(n):
        r = pl.ds(_aligned((n & 1) * 512, 512), 512)
        src = bx_hbm.bitcast(U32).at[r, pl.ds(_aligned((n >> 1) * 512, 512), 512)]
        return pltpu.make_async_copy(src, bx_v.at[n >> 1, r], x_sems.at[n])

    raw_copies = [
        pltpu.make_async_copy(src.bitcast(U32), dst.at[pl.ds(0, src.shape[0]), pl.ds(0, H)],
                              raw_sems.at[n])
        for n, (src, dst) in enumerate(zip(raw_hbm, raw))]

    for mb in range(4):
        w_copy(0, 64 * mb, 64, mb).start()
    for n in range(6):
        if n < 4:
            x_copy(n).start()
        if n:
            w_copy(n, 0, 256, 3 + n).start()
    for cp in raw_copies:
        cp.start()
    start_other_copies()
    qk_f[8:16, 0:HALO, :] = jnp.zeros((8, HALO, 128), F32)
    v_f[:, 0:HALO, :] = jnp.zeros((8, HALO, 128), F32)
    prob[0:8, 0:128] = jnp.zeros((8, 128), F32)

    def first_weights(mb, carry):
        w_copy(0, 64 * mb, 64, mb).wait()
        for r, x in _transposed_weights(0, mb, w_v):
            wt[0, mb, r:r + 16, :] = x
        return carry

    lax.fori_loop(0, 4, first_weights, 0)

    def qk_rows(n, carry):
        upcoming = jnp.minimum(n, 5)

        @pl.when(n < 4)
        def _():
            x_copy(n).wait()

        @pl.when((n >= 1) & (n <= 5))
        def _():
            w_copy(n, 0, 256, 3 + n).wait()

        scale = jnp.where(n < 4, bscale, 1.0)
        for r0 in range(0, S // 2, BQ):
            row = pl.multiple_of((n & 1) * (S // 2) + r0, BQ)
            x = _halves(bx_v[(n >> 1) & 1, pl.ds(pl.multiple_of(row >> 1, 128), 128), :])
            r = pl.ds(pl.multiple_of(row + HALO, 8), BQ)
            for cb in range(8):
                o = 8 * (n >> 2) + cb
                y = _dot_nt(x, _b_weights(wt, n >> 1, cb)) * scale
                qk_f[o, r, :] = jnp.where((n & 2) != 0, qk_f[o, r, :], 0.0) + y
        for mb, tiles in [(mb, _transposed_weights(upcoming, mb, w_v)) for mb in range(4)]:
            for r, x in tiles:
                wt[upcoming, mb, r:r + 16, :] = x
        return carry

    lax.fori_loop(0, 8, qk_rows, 0)
    for cp in raw_copies:
        cp.wait()

    def v_rows(c, carry):
        il = _Interleaver(c)
        row0 = pl.multiple_of(c * RV, RV)
        st = {}

        def first(cb, xx):
            st["y"] = _dot_nt(xx, _b_weights(wt, 4, cb))
            return st["y"]

        def second(cb, r, xx):
            y = _dot_nt(xx, _b_weights(wt, 5, cb))
            v_f[cb, r, :] = st.pop("y") + y
            return y

        for r0 in range(0, RV, BQ):
            rw = pl.ds(pl.multiple_of((row0 + r0) >> 1, 128), 128)
            r = pl.ds(pl.multiple_of(row0 + (HALO + r0), 8), BQ)
            for cb in range(8):
                il.mxu(BQ, 4, lambda rw=rw: bx_v[0, rw, :], functools.partial(first, cb), "v")
                il.mxu(BQ, 4, lambda rw=rw: bx_v[1, rw, :], functools.partial(second, cb, r),
                       "v")
        il.vpu("begin", "end", _prob_steps(row0, RV, qk_f, prob), _read_back(prob, _zero(c)))
        il.vpu("begin", "end", _regroup_steps(c, S // RV, raw, by_head))
        il.emit(delay=0, lead=300, period=16)
        return carry

    lax.fori_loop(0, S // RV, v_rows, 0)


def _attend_and_project(x_v, c_v, by_head, wo_v, bwo_v, v_f, prob, wait_for_wo, out_hbm, o_s,
                        ctx, out_v, q_s, k_s, v_s, s_a, s_b, p_a, p_b, p_c, sems):
    def head_pair(t, carry):
        il = _Interleaver(t)
        st = {}

        def step(cb, half, lhs):
            y = _dot(lhs, _halves(jnp.concatenate(
                [bwo_v[cb, pl.ds(j, H, stride=DH // 2), :]
                 for j in range(8 * half, 8 * half + 8)], axis=0)))
            if half:
                out_v[pl.ds(pl.multiple_of(t * (RB // 2), RB // 2), RB // 2), _cols(8 + cb)] = (
                    _words(st["y"] + y))
            st["y"] = y
            return y

        def b_rows():
            for cb in range(8):
                for half in range(2):
                    il.mxu(RB, 4, lambda half=half: o_s[0:RB // 2, _cols(4 * half, 4)],
                           functools.partial(step, cb, half), "b")

        _head_pair(t, il, x_v, c_v, *by_head, q_s, k_s, v_s, (s_a, s_b), (p_a, p_b, p_c), ctx,
                   b_rows)
        fns = _mix_steps(pl.multiple_of(t * RB, RB), RB, v_f, prob, o_s)
        fns.append((0, lambda hold: _fence(o_s, _zero(t))))
        il.vpu("begin", ("qk", 0), fns, _read_back(o_s, _zero(t)))
        il.emit(delay=400, lead=200, period=32)
        return carry

    def out_copy(r, half, n):
        cols = pl.ds(half * M, M)
        return pltpu.make_async_copy(out_v.at[r, cols], out_hbm.bitcast(U32).at[r, cols],
                                     sems.at[n])

    def a_copy(c):
        return out_copy(pl.ds(_aligned(c * (BQ // 2), BQ // 2), BQ // 2), 0, c)

    o_s[0:8, 0:128] = jnp.zeros((8, 128), U32)
    lax.fori_loop(0, H // 2, head_pair, 0)
    b_copy = out_copy(pl.ds(0, S // 2), 1, NQ)
    b_copy.start()
    wait_for_wo()

    def out_rows(c, carry):
        w0 = pl.multiple_of(c * (BQ // 2), BQ // 2)
        for cb in range(8):
            y = None
            for t in range(0, H // 2, 2):
                lhs = jnp.concatenate([ctx[pl.ds(w0 + u * (S // 2), BQ // 2), :]
                                       for u in (t, t + 1)], axis=1)
                part = _dot(_halves(lhs), _halves(wo_v[128 * t:128 * t + 256, _cols(cb)]))
                y = part if y is None else y + part
            out_v[pl.ds(w0, BQ // 2), _cols(cb)] = _words(y)
        a_copy(c).start()
        return carry

    lax.fori_loop(0, NQ, out_rows, 0)
    b_copy.wait()
    for c in range(NQ):
        a_copy(c).wait()


def _kernel(x_hbm, c_hbm, wq_hbm, wuk_hbm, wuv_hbm, wo_hbm, bx_hbm, wqkv_hbm, bwo_hbm, out_hbm,
            x_v, c_v, wo_v, bwo_v, v_f, prob, wq_h, wk_h, wv_h, o_s, sems):
    vm = pltpu.VMEM
    copies = [pltpu.make_async_copy(src.bitcast(U32), dst, sems.at[n])
              for n, (src, dst) in enumerate(((wo_hbm, wo_v), (x_hbm, x_v), (c_hbm, c_v)))]
    copies += [pltpu.make_async_copy(bwo_hbm.bitcast(U32).at[:, pl.ds(128 * cb, 128)],
                                     bwo_v.at[cb, pl.ds(0, M // 2)], sems.at[3 + cb])
               for cb in range(8)]
    by_head = (wq_h, wk_h, wv_h)

    def start(cps):
        for cp in cps:
            cp.start()

    def wait(cps):
        for cp in cps:
            cp.wait()

    pl.run_scoped(
        functools.partial(_project_b, bx_hbm, wqkv_hbm, (wq_hbm, wuk_hbm, wuv_hbm),
                          functools.partial(start, copies[1:] + copies[:1]), v_f, prob, by_head),
        vm((2, S // 2, M // 2), U32), vm((6, M // 4, M), U32),
        vm((6, 4, H * WPITCH + 16, 128), U32), vm((16, HALO + S, 128), F32),
        vm((M // 2 + 4, HPITCH, D), U32), vm((DC // 2 + 4, HPITCH, D), U32),
        vm((DC // 2 + 4, HPITCH, D), U32), pltpu.SemaphoreType.DMA((9,)),
        pltpu.SemaphoreType.DMA((4,)), pltpu.SemaphoreType.DMA((3,)))
    wait(copies[1:])
    pl.run_scoped(
        functools.partial(_attend_and_project, x_v, c_v, by_head, wo_v, bwo_v, v_f, prob,
                          functools.partial(wait, copies[:1]), out_hbm, o_s),
        vm((H // 2 * S // 2, 2 * D), U32), vm((S // 2, 2 * M), U32),
        vm((S // 2, 2 * D), U32), vm((S // 2, 2 * D), U32), vm((S // 2, 2 * D), U32),
        vm((2 * BQ + 8, S), F32), vm((2 * BQ + 8, S), F32),
        vm((BQ + 8, S + 2 * D), U32), vm((BQ + 8, S + 2 * D), U32),
        vm((BQ + 8, S + 2 * D), U32), pltpu.SemaphoreType.DMA((NQ + 1,)))


@jax.jit
def pallas_concat_heads__compressed_kv_cla__sliding_local_dilated__prompt_kernel(
    A_x: jax.Array,
    A_c_kv: jax.Array,
    A_w_q: jax.Array,
    A_w_uk: jax.Array,
    A_w_uv: jax.Array,
    A_w_o: jax.Array,
    B_x: jax.Array,
    B_wqkv: jax.Array,
    B_wo: jax.Array,
):
    vm = pltpu.VMEM
    out = pl.pallas_call(
        _kernel,
        out_shape=jax.ShapeDtypeStruct((S, 2 * M), BF16),
        in_specs=[pl.BlockSpec(memory_space=pl.ANY)] * 9,
        out_specs=pl.BlockSpec(memory_space=pl.ANY),
        scratch_shapes=[
            vm((S // 2, M), U32), vm((S // 2, DC), U32), vm((H * D // 2, M), U32),
            vm((8, M // 2 + 16, 128), U32), vm((8, HALO + S, 128), F32), vm((S, W * 128), F32),
            vm((2, H // 2, M // 2, D), U32), vm((2, H // 2, DC // 2, D), U32),
            vm((2, H // 2, DC // 2, D), U32),
            vm((RB // 2 + 8, M + 256), U32),
            pltpu.SemaphoreType.DMA((11,)),
        ],
        compiler_params=pltpu.CompilerParams(vmem_limit_bytes=124 * 1024 * 1024),
        name="concat_heads_attention",
    )(
        A_x.reshape(S, M), A_c_kv.reshape(S, DC),
        A_w_q.reshape(M // 2, 2 * H, D), A_w_uk.reshape(DC // 2, 2 * H, D),
        A_w_uv.reshape(DC // 2, 2 * H, D),
        A_w_o.reshape(H * D, M), B_x.reshape(S, M), B_wqkv, B_wo,
    )
    return out.reshape(1, S, 2 * M)
```
